```python
import jax
import jax.numpy as jnp

def _softmax(x, axis=-1):
    return jax.nn.softmax(x, axis=axis)

def _gelu(x):
    return jax.nn.gelu(x, approximate=True)

def _silu(x):
    return jax.nn.silu(x)

def _sigmoid(x):
    return jax.nn.sigmoid(x)

def _layernorm(x, axis=-1, eps=1e-05):
    m = jnp.mean(x, axis=axis, keepdims=True)
    v = jnp.var(x, axis=axis, keepdims=True)
    return (x - m) / jnp.sqrt(v + eps)

def _scatter_add(tgt, idx, src, axis=0):
    return tgt.at[idx].add(src)

def _segment_sum(src, seg, n):
    return jax.ops.segment_sum(src, seg, n)

class _Rng:

    def __init__(self, key):
        self._k = key

    def _next(self):
        self._k, sub = jax.random.split(self._k)
        return sub

    def normal(self, shape):
        return jax.random.normal(self._next(), shape, dtype=jnp.bfloat16)

    def randint(self, lo, hi, shape):
        return jax.random.randint(self._next(), shape, lo, hi, dtype=jnp.int32)

    def uniform(self, shape, lo=0.0, hi=1.0):
        return jax.random.uniform(self._next(), shape, jnp.bfloat16, lo, hi)

    def permutation(self, n):
        return jax.random.permutation(self._next(), n)
kernel_name = 'adaLN_cond__memory_aug_recurrent_mem_tr__glu_gated_swiglu__prompt'

def setup_inputs():
    _rng = _Rng(jax.random.key(int.from_bytes(__import__("os").urandom(4), "little")))
    _w = lambda a: (lambda t: t.astype(jnp.bfloat16) if jnp.issubdtype(t.dtype, jnp.floating) else t)(jnp.asarray(a))

    def _A_setup():
        B, S, Dm = (1, 2048, 1024)
        H, Dh = (32, 128)
        M, seg = (8, 32)
        seg = min(seg, S)
        S = S // seg * seg
        return {'x': _w((lambda *s: _rng.normal(s) * 0.05)(B, S, Dm)), 'mem0': _w((lambda *s: _rng.normal(s) * 0.05)(B, M, Dm)), 'Wq': _w((lambda *s: _rng.normal(s) * 0.05)(Dm, H, Dh) * Dm ** (-0.5)), 'Wk': _w((lambda *s: _rng.normal(s) * 0.05)(Dm, H, Dh) * Dm ** (-0.5)), 'Wv': _w((lambda *s: _rng.normal(s) * 0.05)(Dm, H, Dh) * Dm ** (-0.5)), 'Wo': _w((lambda *s: _rng.normal(s) * 0.05)(H, Dh, Dm) * (H * Dh) ** (-0.5)), 'seg_len': seg}
    _A_in = _A_setup()

    def _B_setup():
        B, S, D, F = (1, 2048, 1024, 3584)
        return {'x': _w((lambda *s: _rng.normal(s) * 0.05)(B, S, D)), 'w1': _w((lambda *s: _rng.normal(s) * 0.05)(D, F) * (2.0 / D) ** 0.5), 'w3': _w((lambda *s: _rng.normal(s) * 0.05)(D, F) * (2.0 / D) ** 0.5), 'w2': _w((lambda *s: _rng.normal(s) * 0.05)(F, D) * (2.0 / F) ** 0.5)}
    _B_in = _B_setup()
    return {'A_x': _A_in['x'], 'A_mem0': _A_in['mem0'], 'A_Wq': _A_in['Wq'], 'A_Wk': _A_in['Wk'], 'A_Wv': _A_in['Wv'], 'A_Wo': _A_in['Wo'], 'A_seg_len': _A_in['seg_len'], 'B_x': _B_in['x'], 'B_w1': _B_in['w1'], 'B_w3': _B_in['w3'], 'B_w2': _B_in['w2'], 'c': _w((lambda *s: _rng.normal(s) * 0.05)(1, 1024)), 'w_mod': _w((lambda *s: _rng.normal(s) * 0.05)(1024, 6 * 1024) * 1024 ** (-0.5))}

def reference(A_x, A_mem0, A_Wq, A_Wk, A_Wv, A_Wo, A_seg_len, B_x, B_w1, B_w3, B_w2, c, w_mod):

    def _A_ref(x, mem0, Wq, Wk, Wv, Wo, seg_len):
        B, S, Dm = x.shape
        H, Dh = (Wq.shape[1], Wq.shape[2])
        M = mem0.shape[1]
        scale = Dh ** (-0.5)
        n_seg = S // seg_len
        L = M + seg_len
        idx = jnp.arange(L)
        mask = (idx[:, None] < M) | (idx[:, None] >= idx[None, :])
        mem = mem0
        outs = []
        for s in range(n_seg):
            xs = x[:, s * seg_len:(s + 1) * seg_len, :].copy()
            h = jnp.concatenate([mem, xs], axis=1)
            q = jnp.einsum('btd,dhe->bhte', h, Wq)
            k = jnp.einsum('btd,dhe->bhte', h, Wk)
            v = jnp.einsum('btd,dhe->bhte', h, Wv)
            scores = jnp.einsum('bhqe,bhke->bhqk', q, k) * scale
            scores = jnp.where(mask[None, None], scores, -1000000000.0)
            p = _softmax(scores, axis=-1)
            o = jnp.einsum('bhqk,bhke->bhqe', p, v)
            o = jnp.einsum('bhte,hed->btd', o, Wo)
            mem = o[:, :M, :].copy()
            outs.append(o[:, M:, :])
        return jnp.concatenate(outs, axis=1)

    def _B_ref(x, w1, w3, w2):
        gate = jnp.einsum('bsd,df->bsf', x, w1)
        up = jnp.einsum('bsd,df->bsf', x, w3)
        h = _silu(gate) * up
        out = jnp.einsum('bsf,fd->bsd', h, w2)
        return out
    x = A_x
    mod = (_silu(c) @ w_mod).reshape(c.shape[0], 6, 1, -1)
    sa, ca, ga, sb, cb, gb = (mod[:, 0].copy(), mod[:, 1].copy(), mod[:, 2].copy(), mod[:, 3].copy(), mod[:, 4].copy(), mod[:, 5].copy())
    h = _layernorm(x, axis=-1) * (1 + ca) + sa
    x = x + ga * _A_ref(h, A_mem0, A_Wq, A_Wk, A_Wv, A_Wo, A_seg_len)
    h = _layernorm(x, axis=-1) * (1 + cb) + sb
    x = x + gb * _B_ref(h, B_w1, B_w3, B_w2)
    return x
```

```python
import functools

import jax
import jax.numpy as jnp
from jax import lax
import jax.experimental.pallas as pl
import jax.experimental.pallas.tpu as pltpu

F32 = jnp.float32
BF16 = jnp.bfloat16
U32 = jnp.uint32

LANE = 128
SEG = 32
MEM = 8
PAIR = 2 * SEG
EPS = 1e-5


def _dot(a, b):
    return jnp.dot(a, b, preferred_element_type=F32)


def _cat_lanes(ref, n):
    return jnp.concatenate([ref[k] for k in range(n)], axis=1)


def _layernorm(x):
    m = jnp.mean(x, axis=-1, keepdims=True)
    xc = x - m
    v = jnp.mean(xc * xc, axis=-1, keepdims=True)
    return xc * lax.rsqrt(v + EPS)


def _kernel(x_hbm, mem0_ref, wq_hbm, wk_hbm, wv_hbm, wo_hbm, w1_hbm, w3_hbm,
            w2_hbm, c_ref, wmod_hbm, out_hbm,
            x_v, wqkv, wo_v, w1_v, w3_v, w2_v, wmod_v, mod_v, mem_v,
            lhsa_v, lhsb_v, sv_v, oa_v, ob_v, x1_v, h2_v, act_v, stage_v,
            sem_x, sem_mod, sem_qkv, sem_wo, sem_ffn, sem_out,
            *, S, D, H, F):
    KD = D // LANE
    NF = F // LANE
    NP = S // PAIR
    L = SEG + MEM
    scale = float(LANE) ** -0.5

    def mod_copy(j):
        return pltpu.make_async_copy(
            wmod_hbm.at[:, pl.ds(j * LANE, LANE)], wmod_v.at[j], sem_mod.at[0])

    def qkv_copy(w, j, p):
        src = (wq_hbm, wk_hbm, wv_hbm)[w].bitcast(U32)
        return pltpu.make_async_copy(
            src.at[:, p, j, 0, :], wqkv.at[w, j, p], sem_qkv.at[j])

    def wo_copy(j):
        return pltpu.make_async_copy(
            wo_hbm.at[:, pl.ds(j * LANE, LANE)], wo_v.at[j], sem_wo.at[0])

    def ffn_copies():
        cps = []
        for f in range(NF):
            cps.append(pltpu.make_async_copy(
                w1_hbm.at[:, pl.ds(f * LANE, LANE)], w1_v.at[f], sem_ffn.at[0]))
            cps.append(pltpu.make_async_copy(
                w3_hbm.at[:, pl.ds(f * LANE, LANE)], w3_v.at[f], sem_ffn.at[0]))
        for j in range(KD):
            cps.append(pltpu.make_async_copy(
                w2_hbm.at[:, pl.ds(j * LANE, LANE)], w2_v.at[j], sem_ffn.at[0]))
        return cps

    x_copy = pltpu.make_async_copy(x_hbm, x_v, sem_x.at[0])

    def out_copy(i, slot):
        return pltpu.make_async_copy(
            stage_v.at[slot], out_hbm.at[pl.ds(i * PAIR, PAIR), :],
            sem_out.at[slot])

    for j in range(6 * KD):
        mod_copy(j).start()
    x_copy.start()
    for j in range(H // 2):
        for w in range(3):
            for p in range(2):
                qkv_copy(w, j, p).start()
    for j in range(KD):
        wo_copy(j).start()
    for cp in ffn_copies():
        cp.start()

    for j in range(6 * KD):
        mod_copy(j).wait()
    c = c_ref[...].astype(F32)
    sc = (c * jax.nn.sigmoid(c)).astype(BF16)
    sc = jnp.broadcast_to(sc, (16, D))
    for j in range(6 * KD):
        r = _dot(sc, wmod_v[j])[0:8]
        if j // KD in (1, 4):
            r = r + 1.0
        mod_v[:, j * LANE:(j + 1) * LANE] = r

    def mod_row(k):
        return mod_v[0:1, k * D:(k + 1) * D]

    for j in range(H // 2):
        for w in range(3):
            for p in range(2):
                qkv_copy(w, j, p).wait()

    def relayout(j, carry):
        for w in range(3):
            for r in range(0, D // 2, 64):
                a = wqkv[w, j, 0, r:r + 64, :]
                b = wqkv[w, j, 1, r:r + 64, :]
                wqkv[w, j, 0, r:r + 64, :] = (a & U32(0xFFFF)) | (b << 16)
                wqkv[w, j, 1, r:r + 64, :] = (a >> 16) | (b & U32(0xFFFF0000))
        return carry

    lax.fori_loop(0, H // 2, relayout, 0)

    def w_head(w, h):
        return pltpu.bitcast(wqkv[w, h // 2, h % 2], BF16)

    def ln1(i):
        x = x_v[pl.ds(pl.multiple_of(i * PAIR, PAIR), PAIR), :].astype(F32)
        h = _layernorm(x) * mod_row(1) + mod_row(0)
        for k in range(KD):
            hk = h[:, k * LANE:(k + 1) * LANE]
            lhsa_v[k, 0:SEG, :] = hk[0:SEG].astype(BF16)
            lhsa_v[k, L:L + 8, :] = hk[SEG:SEG + 8].astype(BF16)
            lhsb_v[k, 0:24, :] = hk[SEG + 8:PAIR].astype(BF16)

    rr = lax.broadcasted_iota(jnp.int32, (L, L), 0)
    cc = lax.broadcasted_iota(jnp.int32, (L, L), 1)
    mask = (rr >= SEG) | (cc >= SEG) | (cc <= rr)

    def attend(q, k, v):
        s = lax.dot_general(q.astype(BF16), k.astype(BF16),
                            (((1,), (1,)), ((), ())),
                            preferred_element_type=F32)
        s = jnp.where(mask, s * scale, -1000000000.0)
        m = jnp.max(s, axis=-1, keepdims=True)
        e = jnp.exp(s - m)
        p = e / jnp.sum(e, axis=-1, keepdims=True)
        return _dot(p.astype(BF16), v.astype(BF16))

    def ffn_pieces(i_prev, slot):
        def ln2():
            x1 = x1_v[...]
            h = _layernorm(x1) * mod_row(4) + mod_row(3)
            for k in range(KD):
                h2_v[k] = h[:, k * LANE:(k + 1) * LANE].astype(BF16)

        def up(f):
            h2 = _cat_lanes(h2_v, KD)
            g = _dot(h2, w1_v[f])
            u = _dot(h2, w3_v[f])
            act_v[f] = (g * jax.nn.sigmoid(g) * u).astype(BF16)

        def down(j):
            a = _cat_lanes(act_v, NF)
            y = _dot(a, w2_v[j])
            sl = slice(j * LANE, (j + 1) * LANE)
            gb = mod_v[0:1, 5 * D + j * LANE:5 * D + (j + 1) * LANE]
            stage_v[slot, :, sl] = (x1_v[:, sl] + gb * y).astype(BF16)

        ups = [functools.partial(up, f) for f in range(NF)]
        downs = [functools.partial(down, j) for j in range(KD)]
        return ln2, ups, downs

    def attn_pair(i, fill_a, fill_wa, fill_b, fill_wb):
        row0 = pl.multiple_of(i * PAIR, PAIR)
        mem = mem_v[...]
        for k in range(KD):
            lhsa_v[k, SEG:L, :] = mem[:, k * LANE:(k + 1) * LANE].astype(BF16)
        for h in range(H):
            lhs = _cat_lanes(lhsa_v, KD)
            q = _dot(lhs, w_head(0, h))
            k_ = _dot(lhs, w_head(1, h))
            v = _dot(lhs, w_head(2, h))
            sv_v[0, h] = q[L:L + 8]
            sv_v[1, h] = k_[L:L + 8]
            sv_v[2, h] = v[L:L + 8]
            o = attend(q[0:L], k_[0:L], v[0:L])
            oa_v[h] = jnp.concatenate([o[0:24], o[SEG:L]], axis=0).astype(BF16)
            ob_v[h, 0:8, :] = o[24:SEG].astype(BF16)
            for fn in fill_a.get(h, ()):
                fn()
        for fn in fill_wa:
            fn()
        oa = _cat_lanes(oa_v, H)
        ya = []
        for j in range(KD):
            y = _dot(oa, wo_v[j])
            ya.append(y[0:24])
            lhsb_v[j, 24:SEG, :] = y[24:SEG].astype(BF16)
        for h in range(H):
            lhs = _cat_lanes(lhsb_v, KD)
            q = jnp.concatenate([sv_v[0, h], _dot(lhs, w_head(0, h))], axis=0)
            k_ = jnp.concatenate([sv_v[1, h], _dot(lhs, w_head(1, h))], axis=0)
            v = jnp.concatenate([sv_v[2, h], _dot(lhs, w_head(2, h))], axis=0)
            o = attend(q, k_, v)
            ob_v[h, 8:8 + L, :] = o.astype(BF16)
            for fn in fill_b.get(h, ()):
                fn()
        for fn in fill_wb:
            fn()
        ob = _cat_lanes(ob_v, H)
        for j in range(KD):
            sl = slice(j * LANE, (j + 1) * LANE)
            y = _dot(ob, wo_v[j])
            att = jnp.concatenate([ya[j], y[0:L]], axis=0)
            ga = mod_v[0:1, 2 * D + j * LANE:2 * D + (j + 1) * LANE]
            x1_v[:, sl] = x_v[pl.ds(row0, PAIR), sl].astype(F32) + ga * att
            mem_v[:, sl] = y[L:L + 8]

    x_copy.wait()
    mem_v[...] = mem0_ref[...].astype(F32)
    ln1(0)
    for j in range(KD):
        wo_copy(j).wait()
    attn_pair(0, {}, [], {}, [lambda: ln1(1)])
    for cp in ffn_copies():
        cp.wait()

    def body(i, carry):
        slot = i % 2

        @pl.when(i >= 3)
        def _():
            out_copy(i - 3, slot).wait()

        ln2, ups, downs = ffn_pieces(i - 1, slot)
        fill_a = {0: [ln2]}
        for f in range(24):
            fill_a.setdefault(4 + f, []).append(ups[f])
        fill_wa = ups[24:]
        fill_b = {}
        for j in range(6):
            fill_b.setdefault(2 + 4 * j, []).append(downs[j])
        nxt = jnp.minimum(i + 1, NP - 1)
        fill_b.setdefault(28, []).append(lambda: None)
        fill_wb = downs[6:] + [lambda: ln1(nxt)]
        attn_pair(i, fill_a, fill_wa, fill_b, fill_wb)
        out_copy(i - 1, slot).start()
        return carry

    lax.fori_loop(1, NP, body, 0)

    slot = NP % 2
    out_copy(NP - 3, slot).wait()
    ln2, ups, downs = ffn_pieces(NP - 1, slot)
    ln2()
    for fn in ups:
        fn()
    for fn in downs:
        fn()
    out_copy(NP - 1, slot).start()
    out_copy(NP - 2, 1 - slot).wait()
    out_copy(NP - 1, slot).wait()


@functools.partial(jax.jit, static_argnames=("A_seg_len",))
def pallas_adaLN_cond__memory_aug_recurrent_mem_tr__glu_gated_swiglu__prompt_kernel(
    A_x: jax.Array,
    A_mem0: jax.Array,
    A_Wq: jax.Array,
    A_Wk: jax.Array,
    A_Wv: jax.Array,
    A_Wo: jax.Array,
    A_seg_len,
    B_x: jax.Array,
    B_w1: jax.Array,
    B_w3: jax.Array,
    B_w2: jax.Array,
    c: jax.Array,
    w_mod: jax.Array,
):
    B, S, D = A_x.shape
    H, Dh = A_Wq.shape[1], A_Wq.shape[2]
    F = B_w1.shape[1]
    assert B == 1 and Dh == LANE and A_seg_len == SEG and A_mem0.shape[1] == MEM
    assert S % PAIR == 0 and S // PAIR >= 4 and D % LANE == 0 and F % LANE == 0
    KD, NF = D // LANE, F // LANE
    L = SEG + MEM

    def split(w):
        return w.reshape(D // 2, 2, H // 2, 2, Dh)

    any_spec = pl.BlockSpec(memory_space=pl.ANY)
    vmem_spec = pl.BlockSpec(memory_space=pltpu.VMEM)
    out = pl.pallas_call(
        functools.partial(_kernel, S=S, D=D, H=H, F=F),
        out_shape=jax.ShapeDtypeStruct((S, D), A_x.dtype),
        in_specs=[any_spec, vmem_spec, any_spec, any_spec, any_spec, any_spec,
                  any_spec, any_spec, any_spec, vmem_spec, any_spec],
        out_specs=any_spec,
        scratch_shapes=[
            pltpu.VMEM((S, D), BF16),
            pltpu.VMEM((3, H // 2, 2, D // 2, LANE), U32),
            pltpu.VMEM((KD, H * Dh, LANE), BF16),
            pltpu.VMEM((NF, D, LANE), BF16),
            pltpu.VMEM((NF, D, LANE), BF16),
            pltpu.VMEM((KD, F, LANE), BF16),
            pltpu.VMEM((6 * KD, D, LANE), BF16),
            pltpu.VMEM((8, 6 * D), F32),
            pltpu.VMEM((MEM, D), F32),
            pltpu.VMEM((KD, L + 8, LANE), BF16),
            pltpu.VMEM((KD, SEG, LANE), BF16),
            pltpu.VMEM((3, H, 8, LANE), F32),
            pltpu.VMEM((H, SEG, LANE), BF16),
            pltpu.VMEM((H, L + 8, LANE), BF16),
            pltpu.VMEM((PAIR, D), F32),
            pltpu.VMEM((KD, PAIR, LANE), BF16),
            pltpu.VMEM((NF, PAIR, LANE), BF16),
            pltpu.VMEM((2, PAIR, D), BF16),
            pltpu.SemaphoreType.DMA((1,)),
            pltpu.SemaphoreType.DMA((1,)),
            pltpu.SemaphoreType.DMA((H // 2,)),
            pltpu.SemaphoreType.DMA((1,)),
            pltpu.SemaphoreType.DMA((1,)),
            pltpu.SemaphoreType.DMA((2,)),
        ],
        compiler_params=pltpu.CompilerParams(
            vmem_limit_bytes=110 * 1024 * 1024),
        name="rmt_block",
    )(A_x.reshape(S, D), A_mem0.reshape(MEM, D), split(A_Wq), split(A_Wk),
      split(A_Wv), A_Wo.reshape(H * Dh, D), B_w1, B_w3, B_w2, c, w_mod)
    return out.reshape(B, S, D)
```

```python
import functools

import jax
import jax.numpy as jnp
from jax import lax
import jax.experimental.pallas as pl
import jax.experimental.pallas.tpu as pltpu

F32 = jnp.float32
BF16 = jnp.bfloat16
U32 = jnp.uint32

LANE = 128
SEG = 32
MEM = 8
PAIR = 2 * SEG
EPS = 1e-5


def _dot(a, b):
    return jnp.dot(a, b, preferred_element_type=F32)


def _cat_lanes(ref, n):
    return jnp.concatenate([ref[k] for k in range(n)], axis=1)


def _layernorm(x):
    m = jnp.mean(x, axis=-1, keepdims=True)
    xc = x - m
    v = jnp.mean(xc * xc, axis=-1, keepdims=True)
    return xc * lax.rsqrt(v + EPS)


def _pk(x):
    return pltpu.bitcast(x.astype(BF16), U32)


def _unpk(x):
    return pltpu.bitcast(x, BF16)


def _cat_pk(ref, ks):
    return jnp.concatenate([_unpk(ref[k]) for k in ks], axis=1)


def _kernel(x_hbm, mem0_ref, wq_hbm, wk_hbm, wv_hbm, wo_hbm, w1_hbm, w3_hbm,
            w2_hbm, c_ref, wmod_hbm, out_hbm,
            x_v, wqkv, wo_v, w1_v, w3_v, w2_v, wmod_v, mod_v,
            hs_v, lhsa_v, lhsb_v, sv_v, so_v, oa_v, ob_v, acc_v, ya_v,
            x1_v, h2_v, act_v, stage_v,
            sem_x, sem_mod, sem_qkv, sem_wo, sem_ffn, sem_out,
            *, S, D, H, F):
    KD = D // LANE
    NF = F // LANE
    NP = S // PAIR
    L = SEG + MEM
    scale = float(LANE) ** -0.5

    def col_copy(src, dst, j, sem):
        return pltpu.make_async_copy(
            src.bitcast(U32).at[:, pl.ds(j * LANE, LANE)], dst.at[j], sem)

    def mod_copy(j):
        return col_copy(wmod_hbm, wmod_v, j, sem_mod.at[0])

    def qkv_copy(w, j, p):
        src = (wq_hbm, wk_hbm, wv_hbm)[w].bitcast(U32)
        return pltpu.make_async_copy(
            src.at[:, p, j, 0, :], wqkv.at[w, j, p], sem_qkv.at[j])

    def wo_copy(j):
        return col_copy(wo_hbm, wo_v, j, sem_wo.at[0])

    def ffn_copies():
        cps = []
        for f in range(NF):
            cps.append(col_copy(w1_hbm, w1_v, f, sem_ffn.at[0]))
            cps.append(col_copy(w3_hbm, w3_v, f, sem_ffn.at[0]))
        for j in range(KD):
            cps.append(col_copy(w2_hbm, w2_v, j, sem_ffn.at[0]))
        return cps

    x_copy = pltpu.make_async_copy(x_hbm, x_v, sem_x.at[0])

    def out_copy(i, slot):
        return pltpu.make_async_copy(
            stage_v.at[slot], out_hbm.at[pl.ds(i * PAIR, PAIR), :],
            sem_out.at[slot])

    for j in range(6 * KD):
        mod_copy(j).start()
    x_copy.start()
    for j in range(H // 2):
        for w in range(3):
            for p in range(2):
                qkv_copy(w, j, p).start()
    for j in range(KD):
        wo_copy(j).start()
    for cp in ffn_copies():
        cp.start()

    for j in range(6 * KD):
        mod_copy(j).wait()
    c = c_ref[...].astype(F32)
    sc = (c * jax.nn.sigmoid(c)).astype(BF16)
    sc = jnp.broadcast_to(sc, (16, D))
    for j in range(6 * KD):
        r = _dot(sc, _unpk(wmod_v[j]))[0:8]
        if j // KD in (1, 4):
            r = r + 1.0
        mod_v[:, j * LANE:(j + 1) * LANE] = r

    def mod_row(k):
        return mod_v[0:1, k * D:(k + 1) * D]

    def mod_blk(k, j):
        return mod_v[0:1, k * D + j * LANE:k * D + (j + 1) * LANE]

    for j in range(H // 2):
        for w in range(3):
            for p in range(2):
                qkv_copy(w, j, p).wait()

    def relayout(j, carry):
        for w in range(3):
            for r in range(0, D // 2, 64):
                a = wqkv[w, j, 0, r:r + 64, :]
                b = wqkv[w, j, 1, r:r + 64, :]
                wqkv[w, j, 0, r:r + 64, :] = (a & U32(0xFFFF)) | (b << 16)
                wqkv[w, j, 1, r:r + 64, :] = (a >> 16) | (b & U32(0xFFFF0000))
        return carry

    lax.fori_loop(0, H // 2, relayout, 0)

    def w_head(w, h):
        return _unpk(wqkv[w, h // 2, h % 2])

    def ln1(i):
        x = x_v[pl.ds(pl.multiple_of(i * PAIR, PAIR), PAIR), :].astype(F32)
        h = _layernorm(x) * mod_row(1) + mod_row(0)
        for k in range(KD):
            hk = h[:, k * LANE:(k + 1) * LANE]
            lhsa_v[k, 0:16, :] = _pk(hk[0:32])
            lhsb_v[k, 0:8, :] = _pk(hk[40:56])
            hs_v[0, k] = hk[32:40]
            hs_v[1, k] = hk[56:64]

    rr = lax.broadcasted_iota(jnp.int32, (L, L), 0)
    cc = lax.broadcasted_iota(jnp.int32, (L, L), 1)
    mask = (rr >= SEG) | (cc >= SEG) | (cc <= rr)

    def scores(q, k):
        s = lax.dot_general(q, k, (((1,), (1,)), ((), ())),
                            preferred_element_type=F32)
        s = jnp.where(mask, s * scale, -1000000000.0)
        m = jnp.max(s, axis=-1, keepdims=True)
        e = jnp.exp(s - m)
        p = e / jnp.sum(e, axis=-1, keepdims=True)
        return p.astype(BF16)

    def ffn_pieces(slot):
        def ln2():
            x1 = x1_v[...]
            h = _layernorm(x1) * mod_row(4) + mod_row(3)
            for k in range(KD):
                h2_v[k] = _pk(h[:, k * LANE:(k + 1) * LANE])

        def up(f):
            h2 = _cat_pk(h2_v, range(KD))
            g = _dot(h2, _unpk(w1_v[f]))
            u = _dot(h2, _unpk(w3_v[f]))
            act_v[f] = _pk(g * jax.nn.sigmoid(g) * u)

        def down(j):
            a = _cat_pk(act_v, range(NF))
            y = _dot(a, _unpk(w2_v[j]))
            sl = slice(j * LANE, (j + 1) * LANE)
            stage_v[slot, :, sl] = (x1_v[:, sl] + mod_blk(5, j) * y).astype(BF16)

        ups = [functools.partial(up, f) for f in range(NF)]
        downs = [functools.partial(down, j) for j in range(KD)]
        return ln2, ups, downs

    HG = 2
    NG = H // HG
    TAIL = 4

    def segment(is_a, fill, finish):
        lhs_v = lhsa_v if is_a else lhsb_v
        o_v = oa_v if is_a else ob_v
        qk, vs, ps = {}, {}, {}

        def proj(h):
            lhs = _cat_pk(lhs_v, range(KD))
            r = [_dot(lhs, w_head(w, h)) for w in range(3)]
            if is_a:
                for w in range(3):
                    sv_v[w, h] = r[w][L:L + 8]
                r = [t[0:L] for t in r]
            else:
                r = [jnp.concatenate([sv_v[w, h], r[w]], axis=0)
                     for w in range(3)]
            r = [t.astype(BF16) for t in r]
            qk[h] = r[0:2]
            vs[h] = r[2]

        def pv(h):
            o = _dot(ps.pop(h), vs.pop(h))
            if is_a:
                o_v[h] = _pk(jnp.concatenate([o[0:24], o[SEG:L]], axis=0))
                so_v[h] = o[24:SEG]
            else:
                o_v[h] = _pk(jnp.concatenate([so_v[h], o], axis=0))

        def wo_part(hs, j):
            lo, hi = hs[0] * (LANE // 2), (hs[-1] + 1) * (LANE // 2)
            return _dot(_cat_pk(o_v, hs), _unpk(wo_v[j, lo:hi, :]))

        rows = SEG if is_a else L + 8
        head_hs = list(range(H - TAIL))
        tail_hs = list(range(H - TAIL, H))
        for g in range(NG + 2):
            if g < NG:
                for h in range(g * HG, (g + 1) * HG):
                    proj(h)
            if g == NG:
                for j in range(0, 2):
                    acc_v[j, 0:rows, :] = wo_part(head_hs, j)
            if g == NG + 1:
                for j in range(2, 5):
                    acc_v[j, 0:rows, :] = wo_part(head_hs, j)
            if 1 <= g <= NG:
                for h in range((g - 1) * HG, g * HG):
                    ps[h] = scores(*qk.pop(h))
            if g >= 2:
                for h in range((g - 2) * HG, (g - 1) * HG):
                    pv(h)
            for fn in fill.get(g, ()):
                fn()
        for j in range(5, KD):
            acc_v[j, 0:rows, :] = wo_part(head_hs, j)
        for j in range(KD):
            finish(j, acc_v[j, 0:rows, :] + wo_part(tail_hs, j))
        for fn in fill.get(NG + 2, ()):
            fn()

    def attn_pair(i, fill_a, fill_b):
        row0 = pl.multiple_of(i * PAIR, PAIR)

        def finish_a(j, y):
            ya_v[j] = y[0:24]
            lhsb_v[j, 8:16, :] = _pk(
                jnp.concatenate([hs_v[1, j], y[24:SEG]], axis=0))

        def finish_b(j, y):
            sl = slice(j * LANE, (j + 1) * LANE)
            att = jnp.concatenate([ya_v[j], y[0:L]], axis=0)
            x1_v[:, sl] = (x_v[pl.ds(row0, PAIR), sl].astype(F32)
                           + mod_blk(2, j) * att)
            lhsa_v[j, 16:24, :] = _pk(
                jnp.concatenate([y[L:L + 8], hs_v[0, j]], axis=0))

        segment(True, fill_a, finish_a)
        segment(False, fill_b, finish_b)

    x_copy.wait()
    ln1(0)
    mem0 = mem0_ref[...].astype(F32)
    for k in range(KD):
        lhsa_v[k, 16:24, :] = _pk(jnp.concatenate(
            [mem0[:, k * LANE:(k + 1) * LANE], hs_v[0, k]], axis=0))
    for j in range(KD):
        wo_copy(j).wait()
    attn_pair(0, {}, {NG: [lambda: ln1(1)]})
    for cp in ffn_copies():
        cp.wait()

    def body(i, carry):
        slot = i % 2

        @pl.when(i >= 3)
        def _():
            out_copy(i - 3, slot).wait()

        ln2, ups, downs = ffn_pieces(slot)
        fill_a, fill_b = {0: [ln2]}, {}
        for f in range(NF - 2):
            fill_a.setdefault(2 + f // 2, []).append(ups[f])
        fill_a[NG + 2] = ups[NF - 2:]
        for j in range(KD):
            fill_b.setdefault(2 + 2 * j - (j == KD - 1), []).append(downs[j])
        nxt = jnp.minimum(i + 1, NP - 1)
        fill_b.setdefault(NG, []).append(lambda: ln1(nxt))
        attn_pair(i, fill_a, fill_b)
        out_copy(i - 1, slot).start()
        return carry

    lax.fori_loop(1, NP, body, 0)

    slot = NP % 2
    out_copy(NP - 3, slot).wait()
    ln2, ups, downs = ffn_pieces(slot)
    ln2()
    for fn in ups:
        fn()
    for fn in downs:
        fn()
    out_copy(NP - 1, slot).start()
    out_copy(NP - 2, 1 - slot).wait()
    out_copy(NP - 1, slot).wait()


@functools.partial(jax.jit, static_argnames=("A_seg_len",))
def pallas_adaLN_cond__memory_aug_recurrent_mem_tr__glu_gated_swiglu__prompt_kernel(
    A_x: jax.Array,
    A_mem0: jax.Array,
    A_Wq: jax.Array,
    A_Wk: jax.Array,
    A_Wv: jax.Array,
    A_Wo: jax.Array,
    A_seg_len,
    B_x: jax.Array,
    B_w1: jax.Array,
    B_w3: jax.Array,
    B_w2: jax.Array,
    c: jax.Array,
    w_mod: jax.Array,
):
    B, S, D = A_x.shape
    H, Dh = A_Wq.shape[1], A_Wq.shape[2]
    F = B_w1.shape[1]
    assert B == 1 and Dh == LANE and A_seg_len == SEG and A_mem0.shape[1] == MEM
    assert S % PAIR == 0 and S // PAIR >= 4 and D % LANE == 0 and F % LANE == 0
    KD, NF = D // LANE, F // LANE
    L = SEG + MEM

    def split(w):
        return w.reshape(D // 2, 2, H // 2, 2, Dh)

    any_spec = pl.BlockSpec(memory_space=pl.ANY)
    vmem_spec = pl.BlockSpec(memory_space=pltpu.VMEM)
    out = pl.pallas_call(
        functools.partial(_kernel, S=S, D=D, H=H, F=F),
        out_shape=jax.ShapeDtypeStruct((S, D), A_x.dtype),
        in_specs=[any_spec, vmem_spec, any_spec, any_spec, any_spec, any_spec,
                  any_spec, any_spec, any_spec, vmem_spec, any_spec],
        out_specs=any_spec,
        scratch_shapes=[
            pltpu.VMEM((S, D), BF16),
            pltpu.VMEM((3, H // 2, 2, D // 2, LANE), U32),
            pltpu.VMEM((KD, H * Dh // 2, LANE), U32),
            pltpu.VMEM((NF, D // 2, LANE), U32),
            pltpu.VMEM((NF, D // 2, LANE), U32),
            pltpu.VMEM((KD, F // 2, LANE), U32),
            pltpu.VMEM((6 * KD, D // 2, LANE), U32),
            pltpu.VMEM((8, 6 * D), F32),
            pltpu.VMEM((2, KD, 8, LANE), F32),
            pltpu.VMEM((KD, 24, LANE), U32),
            pltpu.VMEM((KD, 16, LANE), U32),
            pltpu.VMEM((3, H, 8, LANE), F32),
            pltpu.VMEM((H, 8, LANE), F32),
            pltpu.VMEM((H, 16, LANE), U32),
            pltpu.VMEM((H, 24, LANE), U32),
            pltpu.VMEM((KD, 48, LANE), F32),
            pltpu.VMEM((KD, 24, LANE), F32),
            pltpu.VMEM((PAIR, D), F32),
            pltpu.VMEM((KD, PAIR // 2, LANE), U32),
            pltpu.VMEM((NF, PAIR // 2, LANE), U32),
            pltpu.VMEM((2, PAIR, D), BF16),
            pltpu.SemaphoreType.DMA((1,)),
            pltpu.SemaphoreType.DMA((1,)),
            pltpu.SemaphoreType.DMA((H // 2,)),
            pltpu.SemaphoreType.DMA((1,)),
            pltpu.SemaphoreType.DMA((1,)),
            pltpu.SemaphoreType.DMA((2,)),
        ],
        compiler_params=pltpu.CompilerParams(
            vmem_limit_bytes=110 * 1024 * 1024),
        name="rmt_block",
    )(A_x.reshape(S, D), A_mem0.reshape(MEM, D), split(A_Wq), split(A_Wk),
      split(A_Wv), A_Wo.reshape(H * Dh, D), B_w1, B_w3, B_w2, c, w_mod)
    return out.reshape(B, S, D)
```

```python
import functools

import jax
import jax.numpy as jnp
from jax import lax
import jax.experimental.pallas as pl
import jax.experimental.pallas.tpu as pltpu

F32 = jnp.float32
BF16 = jnp.bfloat16
U32 = jnp.uint32

LANE = 128
SEG = 32
MEM = 8
PAIR = 2 * SEG
EPS = 1e-5


def _dot(a, b):
    return jnp.dot(a, b, preferred_element_type=F32)


def _cat_lanes(ref, n):
    return jnp.concatenate([ref[k] for k in range(n)], axis=1)


def _layernorm(x):
    m = jnp.mean(x, axis=-1, keepdims=True)
    xc = x - m
    v = jnp.mean(xc * xc, axis=-1, keepdims=True)
    return xc * lax.rsqrt(v + EPS)


def _pk(x):
    return pltpu.bitcast(x.astype(BF16), U32)


def _unpk(x):
    return pltpu.bitcast(x, BF16)


def _cat_pk(ref, ks):
    return jnp.concatenate([_unpk(ref[k]) for k in ks], axis=1)


def _kernel(x_hbm, mem0_ref, wq_hbm, wk_hbm, wv_hbm, wo_hbm, w1_hbm, w3_hbm,
            w2_hbm, c_ref, wmod_hbm, out_hbm,
            x_v, xpre_v, hpre_v, pre_v, wqkv, wo_v, w1_v, w3_v, w2_v, wmod_v,
            mod_v, hs_v, lhs_v, so_v, oa_v, ob_v, acc_v, ya_v,
            x1_v, h2_v, act_v, stage_v,
            sem_x, sem_mod, sem_qkv, sem_w, sem_out,
            *, S, D, H, F):
    KD = D // LANE
    NF = F // LANE
    NP = S // PAIR
    NSEG = S // SEG
    NJ = H // 2
    L = SEG + MEM
    scale = float(LANE) ** -0.5

    def blk(j):
        return slice(j * LANE, (j + 1) * LANE)

    MODC = 4 * LANE

    def mod_copy(c0, n, sem):
        return pltpu.make_async_copy(
            wmod_hbm.bitcast(U32).at[:, pl.ds(c0, n)],
            wmod_v.at[:, pl.ds(c0, n)], sem)

    n_early = 2 * D // MODC
    early_mod = [mod_copy(k * MODC, MODC, sem_mod.at[k]) for k in range(n_early)]
    late_mod = mod_copy(2 * D, 4 * D, sem_mod.at[n_early])

    def qkv_copies(j):
        return [pltpu.make_async_copy(
            w.bitcast(U32).at[:, p, j, 0, :],
            wqkv.at[n, j, p], sem_qkv.at[j])
            for n, w in enumerate((wq_hbm, wk_hbm, wv_hbm)) for p in range(2)]

    def w_copy(src, dst, k):
        return pltpu.make_async_copy(src.bitcast(U32), dst, sem_w.at[k])

    wo_copy = w_copy(wo_hbm, wo_v, 0)
    ffn_copies = [w_copy(w1_hbm, w1_v, 1), w_copy(w3_hbm, w3_v, 2),
                  w_copy(w2_hbm, w2_v, 3)]
    xpre_copy = pltpu.make_async_copy(
        x_hbm.at[:, pl.ds(0, 8), :], xpre_v, sem_x.at[0])
    x_copy = pltpu.make_async_copy(x_hbm, x_v, sem_x.at[1])

    def out_copy(i, slot):
        return pltpu.make_async_copy(
            stage_v.at[slot], out_hbm.at[pl.ds(i * PAIR, PAIR), :],
            sem_out.at[slot])

    NQ0 = 8
    xpre_copy.start()
    for cp in early_mod:
        cp.start()
    for j in range(NQ0):
        for cp in qkv_copies(j):
            cp.start()

    c = c_ref[...].astype(F32)
    sc = (c * jax.nn.sigmoid(c)).astype(BF16)
    sc = jnp.broadcast_to(sc, (16, D))

    def mod_cols(j0, j1):
        for j in range(j0, j1):
            r = _dot(sc, _unpk(wmod_v[:, blk(j)]))[0:8]
            if j // KD in (1, 4):
                r = r + 1.0
            mod_v[:, blk(j)] = r

    for k, cp in enumerate(early_mod):
        cp.wait()
        mod_cols(k * MODC // LANE, (k + 1) * MODC // LANE)

    def mod_row(k):
        return mod_v[0:1, k * D:(k + 1) * D]

    def mod_blk(k, j):
        return mod_v[0:1, k * D + j * LANE:k * D + (j + 1) * LANE]

    xpre_copy.wait()

    def ln_pre(b, carry):
        x = xpre_v[pl.ds(b * 8, 8)].astype(F32).reshape(64, D)
        h = _layernorm(x) * mod_row(1) + mod_row(0)
        r0 = pl.multiple_of(b * 32, 32)
        for k in range(KD):
            hpre_v[k, pl.ds(r0, 32), :] = _pk(h[:, blk(k)])
        return carry

    lax.fori_loop(0, NSEG // 8, ln_pre, 0)

    def pre_body(j, carry):
        @pl.when(j < (NJ - NQ0) // 2)
        def _():
            for t in range(2):
                for cp in qkv_copies(NQ0 + 2 * j + t):
                    cp.start()

        @pl.when(j == (NJ - NQ0) // 2)
        def _():
            wo_copy.start()
            x_copy.start()
            late_mod.start()
            for cp in ffn_copies:
                cp.start()

        for cp in qkv_copies(j):
            cp.wait()
        for w in range(3):
            for r in range(0, D // 2, 64):
                a = wqkv[w, j, 0, r:r + 64, :]
                b = wqkv[w, j, 1, r:r + 64, :]
                wqkv[w, j, 0, r:r + 64, :] = (a & U32(0xFFFF)) | (b << 16)
                wqkv[w, j, 1, r:r + 64, :] = (a >> 16) | (b & U32(0xFFFF0000))
            for p in range(2):
                hp = _cat_pk(hpre_v, range(KD))
                pre_v[w, j, p] = _pk(_dot(hp, _unpk(wqkv[w, j, p])))
        return carry

    lax.fori_loop(0, NJ, pre_body, 0)

    def w_head(w, h):
        return _unpk(wqkv[w, h // 2, h % 2])

    def ln1(i):
        for sg in range(2):
            x = x_v[2 * i + sg].astype(F32)[8:SEG]
            h = _layernorm(x) * mod_row(1) + mod_row(0)
            for k in range(KD):
                lhs_v[sg, k, 0:8, :] = _pk(h[0:16, blk(k)])
                hs_v[sg, k] = h[16:24, blk(k)]

    L2 = 2 * L
    rr = lax.broadcasted_iota(jnp.int32, (L2, L2), 0)
    cc = lax.broadcasted_iota(jnp.int32, (L2, L2), 1)
    same = (rr >= L) == (cc >= L)
    rr = jnp.where(rr >= L, rr - L, rr)
    cc = jnp.where(cc >= L, cc - L, cc)
    mask = same & ((rr >= SEG) | (cc >= SEG) | (cc <= rr))
    fill_val = jnp.where(same, -1000000000.0, -jnp.inf).astype(F32)

    def scores(q, k):
        s = lax.dot_general(q, k, (((1,), (1,)), ((), ())),
                            preferred_element_type=F32)
        s = jnp.where(mask, s * scale, fill_val)
        m = jnp.max(s, axis=-1, keepdims=True)
        e = jnp.exp(s - m)
        p = e / jnp.sum(e, axis=-1, keepdims=True)
        return p.astype(BF16)

    def ffn_pieces(xs, slot):
        def ln2():
            h = _layernorm(x1_v[xs]) * mod_row(4) + mod_row(3)
            for k in range(KD):
                h2_v[k] = _pk(h[:, blk(k)])

        def up(f):
            h2 = _cat_pk(h2_v, range(KD))
            g = _dot(h2, _unpk(w1_v[:, blk(f)]))
            u = _dot(h2, _unpk(w3_v[:, blk(f)]))
            act_v[f] = _pk(g * jax.nn.sigmoid(g) * u)

        def down(j):
            a = _cat_pk(act_v, range(NF))
            y = _dot(a, _unpk(w2_v[:, blk(j)]))
            stage_v[slot, :, blk(j)] = (
                x1_v[xs, :, blk(j)] + mod_blk(5, j) * y).astype(BF16)

        ups = [functools.partial(up, f) for f in range(NF)]
        downs = [functools.partial(down, j) for j in range(KD)]
        return ln2, ups, downs

    LS, LP = 1, 2
    TAIL = 4

    def segment(i, sg, fill, finish):
        o_v = ob_v if sg else oa_v
        prow = pl.multiple_of(i * 8, 8)
        qk, vs, ps = {}, {}, {}

        def proj(g):
            r = []
            for w in range(3):
                parts = []
                for p in range(2):
                    lhs = _cat_pk(lhs_v.at[sg], range(KD))
                    pre = _unpk(pre_v[w, g, p, pl.ds(prow, 8), :]).astype(F32)
                    parts += [pre[8 * sg:8 * sg + 8],
                              _dot(lhs, w_head(w, 2 * g + p))]
                r.append(jnp.concatenate(parts, axis=0).astype(BF16))
            qk[g] = r[0:2]
            vs[g] = r[2]

        def pv(g):
            o2 = _dot(ps.pop(g), vs.pop(g))
            for p in range(2):
                h = 2 * g + p
                o = o2[p * L:(p + 1) * L]
                if sg == 0:
                    o_v[h] = _pk(jnp.concatenate([o[0:24], o[SEG:L]], axis=0))
                    so_v[h] = o[24:SEG]
                else:
                    o_v[h] = _pk(jnp.concatenate([so_v[h], o], axis=0))

        def wo_part(hs, j):
            lo, hi = hs[0] * (LANE // 2), (hs[-1] + 1) * (LANE // 2)
            return _dot(_cat_pk(o_v, hs), _unpk(wo_v[lo:hi, blk(j)]))

        rows = L + 8 if sg else SEG
        head_hs = list(range(H - TAIL))
        tail_hs = list(range(H - TAIL, H))
        wo_at = {NJ: range(0, 2), NJ + 1: range(2, 5)}
        for g in range(NJ + LP):
            if g < NJ:
                proj(g)
            for j in wo_at.get(g, ()):
                acc_v[j, 0:rows, :] = wo_part(head_hs, j)
            if LS <= g < NJ + LS:
                ps[g - LS] = scores(*qk.pop(g - LS))
            if g >= LP:
                pv(g - LP)
            for fn in fill.get(g, ()):
                fn()
        for j in range(5, KD):
            acc_v[j, 0:rows, :] = wo_part(head_hs, j)
        for j in range(KD):
            finish(j, acc_v[j, 0:rows, :] + wo_part(tail_hs, j))
        for fn in fill.get(NJ + LP, ()):
            fn()

    def attn_pair(i, fill_a, fill_b):
        xs = i % 2

        def finish_a(j, y):
            ya_v[j] = y[0:24]
            lhs_v[1, j, 8:16, :] = _pk(
                jnp.concatenate([hs_v[1, j], y[24:SEG]], axis=0))

        def finish_b(j, y):
            att = jnp.concatenate([ya_v[j], y[0:L]], axis=0)
            x = x_v[pl.ds(2 * i, 2), :, blk(j)].astype(F32).reshape(PAIR, LANE)
            x1_v[xs, :, blk(j)] = x + mod_blk(2, j) * att
            lhs_v[0, j, 8:16, :] = _pk(
                jnp.concatenate([hs_v[0, j], y[L:L + 8]], axis=0))

        segment(i, 0, fill_a, finish_a)
        segment(i, 1, fill_b, finish_b)

    x_copy.wait()
    late_mod.wait()
    mod_cols(2 * KD, 6 * KD)
    ln1(0)
    mem0 = mem0_ref[...].astype(F32)
    for k in range(KD):
        lhs_v[0, k, 8:16, :] = _pk(jnp.concatenate(
            [hs_v[0, k], mem0[:, blk(k)]], axis=0))
    wo_copy.wait()

    def head_body(i, carry):
        attn_pair(i, {}, {NJ: [lambda: ln1(i + 1)]})
        return carry

    lax.fori_loop(0, 2, head_body, 0)
    for cp in ffn_copies:
        cp.wait()

    def body(i, carry):
        slot = i % 2

        @pl.when(i >= 4)
        def _():
            out_copy(i - 4, slot).wait()

        ln2, ups, downs = ffn_pieces(slot, slot)
        fill_a, fill_b = {0: [ln2]}, {}
        for f in range(NF - 2):
            fill_a.setdefault(2 + f // 2, []).append(ups[f])
        fill_a[NJ + LP] = ups[NF - 2:]
        for j in range(KD):
            fill_b.setdefault(2 + 2 * j - (j == KD - 1), []).append(downs[j])
        nxt = jnp.minimum(i + 1, NP - 1)
        fill_b.setdefault(NJ, []).append(lambda: ln1(nxt))
        attn_pair(i, fill_a, fill_b)
        out_copy(i - 2, slot).start()
        return carry

    lax.fori_loop(2, NP, body, 0)

    def tail_body(i, carry):
        slot = i % 2
        out_copy(i - 4, slot).wait()
        ln2, ups, downs = ffn_pieces(slot, slot)
        ln2()
        for fn in ups:
            fn()
        for fn in downs:
            fn()
        out_copy(i - 2, slot).start()
        return carry

    lax.fori_loop(NP, NP + 2, tail_body, 0)
    out_copy(NP - 2, NP % 2).wait()
    out_copy(NP - 1, (NP + 1) % 2).wait()


@functools.partial(jax.jit, static_argnames=("A_seg_len",))
def pallas_adaLN_cond__memory_aug_recurrent_mem_tr__glu_gated_swiglu__prompt_kernel(
    A_x: jax.Array,
    A_mem0: jax.Array,
    A_Wq: jax.Array,
    A_Wk: jax.Array,
    A_Wv: jax.Array,
    A_Wo: jax.Array,
    A_seg_len,
    B_x: jax.Array,
    B_w1: jax.Array,
    B_w3: jax.Array,
    B_w2: jax.Array,
    c: jax.Array,
    w_mod: jax.Array,
):
    B, S, D = A_x.shape
    H, Dh = A_Wq.shape[1], A_Wq.shape[2]
    F = B_w1.shape[1]
    assert B == 1 and Dh == LANE and A_seg_len == SEG and A_mem0.shape[1] == MEM
    assert S % PAIR == 0 and S // PAIR >= 4 and D % LANE == 0 and F % LANE == 0
    KD, NF = D // LANE, F // LANE
    NSEG = S // SEG

    def split(w):
        return w.reshape(D // 2, 2, H // 2, 2, Dh)

    any_spec = pl.BlockSpec(memory_space=pl.ANY)
    vmem_spec = pl.BlockSpec(memory_space=pltpu.VMEM)
    out = pl.pallas_call(
        functools.partial(_kernel, S=S, D=D, H=H, F=F),
        out_shape=jax.ShapeDtypeStruct((S, D), A_x.dtype),
        in_specs=[any_spec, vmem_spec, any_spec, any_spec, any_spec, any_spec,
                  any_spec, any_spec, any_spec, vmem_spec, any_spec],
        out_specs=any_spec,
        scratch_shapes=[
            pltpu.VMEM((NSEG, SEG, D), BF16),
            pltpu.VMEM((NSEG, 8, D), BF16),
            pltpu.VMEM((KD, NSEG * 4, LANE), U32),
            pltpu.VMEM((3, H // 2, 2, NSEG * 4, LANE), U32),
            pltpu.VMEM((3, H // 2, 2, D // 2, LANE), U32),
            pltpu.VMEM((H * Dh // 2, D), U32),
            pltpu.VMEM((D // 2, F), U32),
            pltpu.VMEM((D // 2, F), U32),
            pltpu.VMEM((F // 2, D), U32),
            pltpu.VMEM((D // 2, 6 * D), U32),
            pltpu.VMEM((8, 6 * D), F32),
            pltpu.VMEM((2, KD, 8, LANE), F32),
            pltpu.VMEM((2, KD, 16, LANE), U32),
            pltpu.VMEM((H, 8, LANE), F32),
            pltpu.VMEM((H, 16, LANE), U32),
            pltpu.VMEM((H, 24, LANE), U32),
            pltpu.VMEM((KD, 48, LANE), F32),
            pltpu.VMEM((KD, 24, LANE), F32),
            pltpu.VMEM((2, PAIR, D), F32),
            pltpu.VMEM((KD, PAIR // 2, LANE), U32),
            pltpu.VMEM((NF, PAIR // 2, LANE), U32),
            pltpu.VMEM((2, PAIR, D), BF16),
            pltpu.SemaphoreType.DMA((2,)),
            pltpu.SemaphoreType.DMA((5,)),
            pltpu.SemaphoreType.DMA((H // 2,)),
            pltpu.SemaphoreType.DMA((4,)),
            pltpu.SemaphoreType.DMA((2,)),
        ],
        compiler_params=pltpu.CompilerParams(
            vmem_limit_bytes=110 * 1024 * 1024),
        name="rmt_block",
    )(A_x.reshape(NSEG, SEG, D), A_mem0.reshape(MEM, D), split(A_Wq), split(A_Wk),
      split(A_Wv), A_Wo.reshape(H * Dh, D), B_w1, B_w3, B_w2, c, w_mod)
    return out.reshape(B, S, D)
```

```python
import functools

import jax
import jax.numpy as jnp
from jax import lax
import jax.experimental.pallas as pl
import jax.experimental.pallas.tpu as pltpu

F32 = jnp.float32
BF16 = jnp.bfloat16
U32 = jnp.uint32

LANE = 128
SEG = 32
MEM = 8
PAIR = 2 * SEG
EPS = 1e-5


def _dot(a, b):
    return jnp.dot(a, b, preferred_element_type=F32)


def _cat_lanes(ref, n):
    return jnp.concatenate([ref[k] for k in range(n)], axis=1)


def _layernorm(x):
    m = jnp.mean(x, axis=-1, keepdims=True)
    xc = x - m
    v = jnp.mean(xc * xc, axis=-1, keepdims=True)
    return xc * lax.rsqrt(v + EPS)


def _pk(x):
    return pltpu.bitcast(x.astype(BF16), U32)


def _unpk(x):
    return pltpu.bitcast(x, BF16)


def _cat_pk(ref, ks):
    return jnp.concatenate([_unpk(ref[k]) for k in ks], axis=1)


def _kernel(x_hbm, mem0_hbm, wq_hbm, wk_hbm, wv_hbm, wo_hbm, w1_hbm, w3_hbm,
            w2_hbm, c_hbm, wmod_hbm, out_hbm,
            c_v, mem0_v, x_v, xpre_v, xn_v, hpre_v, pre_v, wq_v, wk_v, wv_v,
            wo_v, w1_v, w3_v, w2_v, wmod_v,
            mod_v, hs_v, lhs_v, so_v, oa_v, ob_v, acc_v, ya_v,
            x1_v, h2_v, act_v, stage_v,
            sem_x, sem_mod, sem_qkv, sem_w, sem_out,
            *, S, D, H, F):
    KD = D // LANE
    NF = F // LANE
    NP = S // PAIR
    NSEG = S // SEG
    NJ = H // 2
    L = SEG + MEM
    scale = float(LANE) ** -0.5
    w_hbm = (wq_hbm, wk_hbm, wv_hbm)
    w_v = (wq_v, wk_v, wv_v)

    def blk(j):
        return slice(j * LANE, (j + 1) * LANE)

    NCH = 4
    CK = KD // NCH

    def mod_copy(c0, n, sem):
        return pltpu.make_async_copy(
            wmod_hbm.bitcast(U32).at[:, pl.ds(c0, n)],
            wmod_v.at[:, pl.ds(c0, n)], sem)

    def early_mod(ch):
        return [mod_copy(t * D + ch * CK * LANE, CK * LANE, sem_mod.at[ch])
                for t in range(2)]

    late_mod = mod_copy(2 * D, 4 * D, sem_mod.at[NCH])

    def unit_copies(j, w):
        return [pltpu.make_async_copy(
            w_hbm[w].bitcast(U32).at[:, p, j, 0, :],
            w_v[w].at[j, p], sem_qkv.at[3 * j + w]) for p in range(2)]

    def start_unit(j, w):
        for cp in unit_copies(j, w):
            cp.start()

    def wait_unit(j, w):
        for cp in unit_copies(j, w):
            cp.wait()

    def w_copy(src, dst, k):
        return pltpu.make_async_copy(src.bitcast(U32), dst, sem_w.at[k])

    wo_copy = w_copy(wo_hbm, wo_v, 0)
    ffn_copies = [w_copy(w1_hbm, w1_v, 1), w_copy(w3_hbm, w3_v, 2),
                  w_copy(w2_hbm, w2_v, 3)]
    c_copy = pltpu.make_async_copy(c_hbm, c_v, sem_x.at[2])
    mem0_copy = pltpu.make_async_copy(mem0_hbm, mem0_v, sem_x.at[3])
    xpre_copy = pltpu.make_async_copy(
        x_hbm.at[:, pl.ds(0, 8), :], xpre_v, sem_x.at[0])
    x_copy = pltpu.make_async_copy(x_hbm, x_v, sem_x.at[1])

    def out_copy(i, slot):
        return pltpu.make_async_copy(
            stage_v.at[slot], out_hbm.at[pl.ds(i * PAIR, PAIR), :],
            sem_out.at[slot])

    NQ0 = 8
    xpre_copy.start()
    c_copy.start()
    for ch in range(NCH - 1):
        for cp in early_mod(ch):
            cp.start()
    start_unit(0, 0)
    for cp in early_mod(NCH - 1):
        cp.start()
    for j in range(NQ0):
        for w in range(3):
            if (j, w) != (0, 0):
                start_unit(j, w)
    mem0_copy.start()
    x1_v[1] = jnp.zeros((PAIR, D), F32)

    xpre_copy.wait()

    def ln_pre(b, carry):
        x = xpre_v[pl.ds(b * 8, 8)].astype(F32).reshape(64, D)
        xn_v[pl.ds(pl.multiple_of(b * 64, 64), 64), :] = _layernorm(x)
        return carry

    lax.fori_loop(0, NSEG // 8, ln_pre, 0)

    c_copy.wait()
    c = c_v[...].astype(F32)
    sc = (c * jax.nn.sigmoid(c)).astype(BF16)
    sc = jnp.broadcast_to(sc, (16, D))

    def mod_col(j):
        r = _dot(sc, _unpk(wmod_v[:, blk(j)]))[0:8]
        if j // KD in (1, 4):
            r = r + 1.0
        mod_v[:, blk(j)] = r

    def mod_row(k):
        return mod_v[0:1, k * D:(k + 1) * D]

    def mod_blk(k, j):
        return mod_v[0:1, k * D + j * LANE:k * D + (j + 1) * LANE]

    def relayout(j, w):
        for r in range(0, D // 2, 64):
            a = w_v[w][j, 0, r:r + 64, :]
            b = w_v[w][j, 1, r:r + 64, :]
            w_v[w][j, 0, r:r + 64, :] = (a & U32(0xFFFF)) | (b << 16)
            w_v[w][j, 1, r:r + 64, :] = (a >> 16) | (b & U32(0xFFFF0000))

    for ch in range(NCH):
        if ch == NCH - 1:
            wait_unit(0, 0)
            relayout(0, 0)
        for cp in early_mod(ch):
            cp.wait()
        for k in range(ch * CK, (ch + 1) * CK):
            mod_col(k)
            mod_col(KD + k)
        for k in range(ch * CK, (ch + 1) * CK):
            for r in range(0, NSEG * 8, 128):
                hpre_v[k, r // 2:r // 2 + 64, :] = _pk(
                    xn_v[r:r + 128, blk(k)] * mod_blk(1, k) + mod_blk(0, k))

    def pre_dot(j, w, p):
        hp = _cat_pk(hpre_v, range(KD))
        pre_v[w, j, p] = _pk(_dot(hp, _unpk(w_v[w][j, p])))

    wait_unit(0, 1)
    pre_dot(0, 0, 0)
    relayout(0, 1)
    pre_dot(0, 0, 1)

    def pre_body(j, carry):
        wait_unit(j, 2)
        wait_unit(j + 1, 0)
        wait_unit(j + 1, 1)

        @pl.when(j < (NJ - NQ0) // 2)
        def _():
            for t in range(2):
                for w in range(3):
                    start_unit(NQ0 + 2 * j + t, w)

        @pl.when(j == (NJ - NQ0) // 2)
        def _():
            wo_copy.start()
            x_copy.start()
            late_mod.start()
            for cp in ffn_copies:
                cp.start()

        for (dj, dw), (rj, rw) in (((j, 1), (j, 2)), ((j, 2), (j + 1, 0)),
                                   ((j + 1, 0), (j + 1, 1))):
            pre_dot(dj, dw, 0)
            relayout(rj, rw)
            pre_dot(dj, dw, 1)
        return carry

    lax.fori_loop(0, NJ - 1, pre_body, 0)

    def w_head(w, h):
        return _unpk(w_v[w][h // 2, h % 2])

    def ln1(i):
        for sg in range(2):
            x = x_v[2 * i + sg].astype(F32)[8:SEG]
            h = _layernorm(x) * mod_row(1) + mod_row(0)
            for k in range(KD):
                lhs_v[sg, k, 0:8, :] = _pk(h[0:16, blk(k)])
                hs_v[sg, k] = h[16:24, blk(k)]

    L2 = 2 * L
    rr = lax.broadcasted_iota(jnp.int32, (L2, L2), 0)
    cc = lax.broadcasted_iota(jnp.int32, (L2, L2), 1)
    same = (rr >= L) == (cc >= L)
    rr = jnp.where(rr >= L, rr - L, rr)
    cc = jnp.where(cc >= L, cc - L, cc)
    mask = same & ((rr >= SEG) | (cc >= SEG) | (cc <= rr))
    fill_val = jnp.where(same, -1000000000.0, -jnp.inf).astype(F32)

    def scores(q, k):
        s = lax.dot_general(q, k, (((1,), (1,)), ((), ())),
                            preferred_element_type=F32)
        s = jnp.where(mask, s * scale, fill_val)
        m = jnp.max(s, axis=-1, keepdims=True)
        e = jnp.exp(s - m)
        p = e / jnp.sum(e, axis=-1, keepdims=True)
        return p.astype(BF16)

    def ln2(xs):
        h = _layernorm(x1_v[xs]) * mod_row(4) + mod_row(3)
        for k in range(KD):
            h2_v[k] = _pk(h[:, blk(k)])

    def up(f):
        h2 = _cat_pk(h2_v, range(KD))
        g = _dot(h2, _unpk(w1_v[:, blk(f)]))
        u = _dot(h2, _unpk(w3_v[:, blk(f)]))
        act_v[f] = _pk(g * jax.nn.sigmoid(g) * u)

    def down(xs, j):
        a = _cat_pk(act_v, range(NF))
        y = _dot(a, _unpk(w2_v[:, blk(j)]))
        stage_v[xs, :, blk(j)] = (
            x1_v[xs, :, blk(j)] + mod_blk(5, j) * y).astype(BF16)

    LS, LP = 1, 2
    TAIL = 4

    def segment(i, sg, fill, finish):
        o_v = ob_v if sg else oa_v
        prow = pl.multiple_of(i * 8, 8)
        qk, vs, ps = {}, {}, {}

        def proj(g):
            r = []
            for w in range(3):
                parts = []
                for p in range(2):
                    lhs = _cat_pk(lhs_v.at[sg], range(KD))
                    pre = _unpk(pre_v[w, g, p, pl.ds(prow, 8), :]).astype(F32)
                    parts += [pre[8 * sg:8 * sg + 8],
                              _dot(lhs, w_head(w, 2 * g + p))]
                r.append(jnp.concatenate(parts, axis=0).astype(BF16))
            qk[g] = r[0:2]
            vs[g] = r[2]

        def pv(g):
            o2 = _dot(ps.pop(g), vs.pop(g))
            for p in range(2):
                h = 2 * g + p
                o = o2[p * L:(p + 1) * L]
                if sg == 0:
                    o_v[h] = _pk(jnp.concatenate([o[0:24], o[SEG:L]], axis=0))
                    so_v[h] = o[24:SEG]
                else:
                    o_v[h] = _pk(jnp.concatenate([so_v[h], o], axis=0))

        def wo_part(hs, j):
            lo, hi = hs[0] * (LANE // 2), (hs[-1] + 1) * (LANE // 2)
            return _dot(_cat_pk(o_v, hs), _unpk(wo_v[lo:hi, blk(j)]))

        rows = L + 8 if sg else SEG
        head_hs = list(range(H - TAIL))
        tail_hs = list(range(H - TAIL, H))
        wo_at = {NJ: range(0, 2), NJ + 1: range(2, 5)}
        for g in range(NJ + LP):
            if g < NJ:
                proj(g)
            for j in wo_at.get(g, ()):
                acc_v[j, 0:rows, :] = wo_part(head_hs, j)
            if LS <= g < NJ + LS:
                ps[g - LS] = scores(*qk.pop(g - LS))
            if g >= LP:
                pv(g - LP)
            for fn in fill.get(g, ()):
                fn()
        for j in range(5, KD):
            acc_v[j, 0:rows, :] = wo_part(head_hs, j)
        for j in range(KD):
            finish(j, acc_v[j, 0:rows, :] + wo_part(tail_hs, j))
        for fn in fill.get(NJ + LP, ()):
            fn()

    def attn_pair(i, fill_a, fill_b):
        xs = i % 2

        def finish_a(j, y):
            ya_v[j] = y[0:24]
            lhs_v[1, j, 8:16, :] = _pk(
                jnp.concatenate([hs_v[1, j], y[24:SEG]], axis=0))

        def finish_b(j, y):
            att = jnp.concatenate([ya_v[j], y[0:L]], axis=0)
            x = x_v[pl.ds(2 * i, 2), :, blk(j)].astype(F32).reshape(PAIR, LANE)
            x1_v[xs, :, blk(j)] = x + mod_blk(2, j) * att
            lhs_v[0, j, 8:16, :] = _pk(
                jnp.concatenate([hs_v[0, j], y[L:L + 8]], axis=0))

        segment(i, 0, fill_a, finish_a)
        segment(i, 1, fill_b, finish_b)

    P = functools.partial
    NU0 = 2

    wait_unit(NJ - 1, 2)
    x_copy.wait()
    late_mod.wait()
    mem0_copy.wait()
    wo_copy.wait()
    late = list(range(2 * KD, 6 * KD))
    for n, (w, p) in enumerate(((1, 0), (1, 1), (2, 0), (2, 1))):
        pre_dot(NJ - 1, w, p)
        if n == 0:
            relayout(NJ - 1, 2)
            ln1(0)
            mem0 = mem0_v[...].astype(F32)
            for k in range(KD):
                lhs_v[0, k, 8:16, :] = _pk(jnp.concatenate(
                    [hs_v[0, k], mem0[:, blk(k)]], axis=0))
        if n < 3:
            for j in late[n::3]:
                mod_col(j)

    def head_body(i, carry):
        attn_pair(i, {}, {2: [P(ln2, 1 - i)], NJ: [P(ln1, i + 1)]})
        return carry

    lax.fori_loop(0, 2, head_body, 0)
    for cp in ffn_copies:
        cp.wait()
    for f in range(NU0):
        up(f)

    def body(i, carry):
        slot = i % 2

        @pl.when(i >= 4)
        def _():
            out_copy(i - 4, slot).wait()

        fill_a, fill_b = {}, {}
        for f in range(NU0, NF):
            fill_a.setdefault((f - NU0) // 2, []).append(P(up, f))
        fill_a[NJ + LP] = [P(down, slot, 0)]
        for j in range(1, KD):
            fill_b.setdefault(2 * j - 1, []).append(P(down, slot, j))
        fill_b.setdefault(2, []).append(P(ln2, 1 - slot))
        fill_b.setdefault(NJ, []).append(P(ln1, jnp.minimum(i + 1, NP - 1)))
        fill_b[NJ + LP] = [P(up, f) for f in range(NU0)]
        attn_pair(i, fill_a, fill_b)
        out_copy(i - 2, slot).start()
        return carry

    lax.fori_loop(2, NP, body, 0)

    s0, s1 = NP % 2, (NP + 1) % 2
    out_copy(NP - 4, s0).wait()
    out_copy(NP - 3, s1).wait()
    for f in range(NU0, NF):
        up(f)
    ln2(s1)
    for j in range(KD):
        down(s0, j)
    for f in range(NF):
        up(f)
    for j in range(KD):
        down(s1, j)
    out_copy(NP - 2, s0).start()
    out_copy(NP - 1, s1).start()
    out_copy(NP - 2, s0).wait()
    out_copy(NP - 1, s1).wait()


@functools.partial(jax.jit, static_argnames=("A_seg_len",))
def pallas_adaLN_cond__memory_aug_recurrent_mem_tr__glu_gated_swiglu__prompt_kernel(
    A_x: jax.Array,
    A_mem0: jax.Array,
    A_Wq: jax.Array,
    A_Wk: jax.Array,
    A_Wv: jax.Array,
    A_Wo: jax.Array,
    A_seg_len,
    B_x: jax.Array,
    B_w1: jax.Array,
    B_w3: jax.Array,
    B_w2: jax.Array,
    c: jax.Array,
    w_mod: jax.Array,
):
    B, S, D = A_x.shape
    H, Dh = A_Wq.shape[1], A_Wq.shape[2]
    F = B_w1.shape[1]
    assert B == 1 and Dh == LANE and A_seg_len == SEG and A_mem0.shape[1] == MEM
    assert S % PAIR == 0 and S // PAIR >= 4 and D % LANE == 0 and F % LANE == 0
    KD, NF = D // LANE, F // LANE
    NSEG = S // SEG

    def split(w):
        return w.reshape(D // 2, 2, H // 2, 2, Dh)

    any_spec = pl.BlockSpec(memory_space=pl.ANY)
    out = pl.pallas_call(
        functools.partial(_kernel, S=S, D=D, H=H, F=F),
        out_shape=jax.ShapeDtypeStruct((S, D), A_x.dtype),
        in_specs=[any_spec] * 11,
        out_specs=any_spec,
        scratch_shapes=[
            pltpu.VMEM((1, D), BF16),
            pltpu.VMEM((MEM, D), BF16),
            pltpu.VMEM((NSEG, SEG, D), BF16),
            pltpu.VMEM((NSEG, 8, D), BF16),
            pltpu.VMEM((NSEG * 8, D), F32),
            pltpu.VMEM((KD, NSEG * 4, LANE), U32),
            pltpu.VMEM((3, H // 2, 2, NSEG * 4, LANE), U32),
            pltpu.VMEM((H // 2, 2, D // 2, LANE), U32),
            pltpu.VMEM((H // 2, 2, D // 2, LANE), U32),
            pltpu.VMEM((H // 2, 2, D // 2, LANE), U32),
            pltpu.VMEM((H * Dh // 2, D), U32),
            pltpu.VMEM((D // 2, F), U32),
            pltpu.VMEM((D // 2, F), U32),
            pltpu.VMEM((F // 2, D), U32),
            pltpu.VMEM((D // 2, 6 * D), U32),
            pltpu.VMEM((8, 6 * D), F32),
            pltpu.VMEM((2, KD, 8, LANE), F32),
            pltpu.VMEM((2, KD, 16, LANE), U32),
            pltpu.VMEM((H, 8, LANE), F32),
            pltpu.VMEM((H, 16, LANE), U32),
            pltpu.VMEM((H, 24, LANE), U32),
            pltpu.VMEM((KD, 48, LANE), F32),
            pltpu.VMEM((KD, 24, LANE), F32),
            pltpu.VMEM((2, PAIR, D), F32),
            pltpu.VMEM((KD, PAIR // 2, LANE), U32),
            pltpu.VMEM((NF, PAIR // 2, LANE), U32),
            pltpu.VMEM((2, PAIR, D), BF16),
            pltpu.SemaphoreType.DMA((4,)),
            pltpu.SemaphoreType.DMA((5,)),
            pltpu.SemaphoreType.DMA((3 * H // 2,)),
            pltpu.SemaphoreType.DMA((4,)),
            pltpu.SemaphoreType.DMA((2,)),
        ],
        compiler_params=pltpu.CompilerParams(
            vmem_limit_bytes=110 * 1024 * 1024,
            disable_bounds_checks=True,
            disable_semaphore_checks=True),
        name="rmt_block",
    )(A_x.reshape(NSEG, SEG, D), A_mem0.reshape(MEM, D), split(A_Wq), split(A_Wk),
      split(A_Wv), A_Wo.reshape(H * Dh, D), B_w1, B_w3, B_w2, c, w_mod)
    return out.reshape(B, S, D)
```

```python
import functools

import jax
import jax.numpy as jnp
from jax import lax
import jax.experimental.pallas as pl
import jax.experimental.pallas.tpu as pltpu

F32 = jnp.float32
BF16 = jnp.bfloat16
U32 = jnp.uint32

LANE = 128
SEG = 32
MEM = 8
PAIR = 2 * SEG
EPS = 1e-5

LS, LP = 1, 3
TAIL = 6
WO_AT = (1, 3, 5)


def _dot(a, b):
    return jnp.dot(a, b, preferred_element_type=F32)


def _cat_lanes(ref, n):
    return jnp.concatenate([ref[k] for k in range(n)], axis=1)


def _layernorm(x):
    m = jnp.mean(x, axis=-1, keepdims=True)
    xc = x - m
    v = jnp.mean(xc * xc, axis=-1, keepdims=True)
    return xc * lax.rsqrt(v + EPS)


def _silu(x):
    hx = 0.5 * x
    return hx + hx * jnp.tanh(hx)


def _recip(x):
    r = pl.reciprocal(x, approx=True)
    return r * (2.0 - x * r)


def _pk(x):
    return pltpu.bitcast(x.astype(BF16), U32)


def _unpk(x):
    return pltpu.bitcast(x, BF16)


def _cat_pk(ref, ks):
    return jnp.concatenate([_unpk(ref[k]) for k in ks], axis=1)


def _kernel(x_hbm, mem0_hbm, wq_hbm, wk_hbm, wv_hbm, wo_hbm, w1_hbm, w3_hbm,
            w2_hbm, c_hbm, wmod_hbm, out_hbm,
            c_v, mem0_v, x_v, xpre_v, xn_v, hpre_v, pre_v, wq_v, wk_v, wv_v,
            wo_v, w1_v, w3_v, w2_v, wmod_v,
            mod_v, hs_v, lhs_v, so_v, oa_v, ob_v, acc_v, ya_v,
            x1_v, h2_v, act_v, stage_v,
            sem_x, sem_mod, sem_qkv, sem_w, sem_out,
            *, S, D, H, F):
    KD = D // LANE
    NF = F // LANE
    NP = S // PAIR
    NSEG = S // SEG
    NJ = H // 2
    L = SEG + MEM
    scale = float(LANE) ** -0.5
    w_hbm = (wq_hbm, wk_hbm, wv_hbm)
    w_v = (wq_v, wk_v, wv_v)

    def blk(j):
        return slice(j * LANE, (j + 1) * LANE)

    NCH = 4
    CK = KD // NCH

    def mod_copy(c0, n, sem):
        return pltpu.make_async_copy(
            wmod_hbm.bitcast(U32).at[:, pl.ds(c0, n)],
            wmod_v.at[:, pl.ds(c0, n)], sem)

    def early_mod(ch):
        return [mod_copy(t * D + ch * CK * LANE, CK * LANE, sem_mod.at[ch])
                for t in range(2)]

    late_mod = mod_copy(2 * D, 4 * D, sem_mod.at[NCH])

    def unit_copies(j, w):
        return [pltpu.make_async_copy(
            w_hbm[w].bitcast(U32).at[:, p, j, 0, :],
            w_v[w].at[j, p], sem_qkv.at[3 * j + w]) for p in range(2)]

    def start_unit(j, w):
        for cp in unit_copies(j, w):
            cp.start()

    def wait_unit(j, w):
        for cp in unit_copies(j, w):
            cp.wait()

    def w_copy(src, dst, k):
        return pltpu.make_async_copy(
            src.bitcast(U32), dst.at[:, pl.ds(0, src.shape[1])], sem_w.at[k])

    wo_copy = w_copy(wo_hbm, wo_v, 0)
    ffn_copies = [w_copy(w1_hbm, w1_v, 1), w_copy(w3_hbm, w3_v, 2),
                  w_copy(w2_hbm, w2_v, 3)]
    c_copy = pltpu.make_async_copy(c_hbm, c_v, sem_x.at[2])
    mem0_copy = pltpu.make_async_copy(mem0_hbm, mem0_v, sem_x.at[3])
    xpre_copy = pltpu.make_async_copy(
        x_hbm.at[:, pl.ds(0, 8), :], xpre_v, sem_x.at[0])
    x_copy = pltpu.make_async_copy(x_hbm, x_v, sem_x.at[1])

    def out_copy(i, slot):
        return pltpu.make_async_copy(
            stage_v.at[slot], out_hbm.at[pl.ds(i * PAIR, PAIR), :],
            sem_out.at[slot])

    NQ0 = 8
    xpre_copy.start()
    c_copy.start()
    for ch in range(NCH - 1):
        for cp in early_mod(ch):
            cp.start()
    start_unit(0, 0)
    for cp in early_mod(NCH - 1):
        cp.start()
    for j in range(NQ0):
        for w in range(3):
            if (j, w) != (0, 0):
                start_unit(j, w)
    mem0_copy.start()
    x1_v[1] = jnp.zeros((PAIR, D), F32)

    xpre_copy.wait()

    def ln_pre(b, carry):
        x = xpre_v[pl.ds(b * 8, 8)].astype(F32).reshape(64, D)
        xn_v[pl.ds(pl.multiple_of(b * 64, 64), 64), :] = _layernorm(x)
        return carry

    lax.fori_loop(0, NSEG // 8, ln_pre, 0)

    c_copy.wait()
    c = c_v[...].astype(F32)
    sc = _silu(c).astype(BF16)
    sc = jnp.broadcast_to(sc, (16, D))

    def mod_col(j):
        r = _dot(sc, _unpk(wmod_v[:, blk(j)]))[0:8]
        if j // KD in (1, 4):
            r = r + 1.0
        mod_v[:, blk(j)] = r

    def mod_row(k):
        return mod_v[0:1, k * D:(k + 1) * D]

    def mod_blk(k, j):
        return mod_v[0:1, k * D + j * LANE:k * D + (j + 1) * LANE]

    def relayout(j, w):
        for r in range(0, D // 2, 64):
            a = w_v[w][j, 0, r:r + 64, :]
            b = w_v[w][j, 1, r:r + 64, :]
            w_v[w][j, 0, r:r + 64, :] = (a & U32(0xFFFF)) | (b << 16)
            w_v[w][j, 1, r:r + 64, :] = (a >> 16) | (b & U32(0xFFFF0000))

    for ch in range(NCH):
        if ch == NCH - 1:
            wait_unit(0, 0)
            relayout(0, 0)
        for cp in early_mod(ch):
            cp.wait()
        for k in range(ch * CK, (ch + 1) * CK):
            mod_col(k)
            mod_col(KD + k)
        for k in range(ch * CK, (ch + 1) * CK):
            for r in range(0, NSEG * 8, 128):
                hpre_v[k, r // 2:r // 2 + 64, :] = _pk(
                    xn_v[r:r + 128, blk(k)] * mod_blk(1, k) + mod_blk(0, k))

    def pre_dot(j, w, p):
        hp = _cat_pk(hpre_v, range(KD))
        pre_v[w, j, p] = _pk(_dot(hp, _unpk(w_v[w][j, p])))

    wait_unit(0, 1)
    pre_dot(0, 0, 0)
    relayout(0, 1)
    pre_dot(0, 0, 1)

    def pre_body(j, carry):
        wait_unit(j, 2)
        wait_unit(j + 1, 0)
        wait_unit(j + 1, 1)

        @pl.when(j < (NJ - NQ0) // 2)
        def _():
            for t in range(2):
                for w in range(3):
                    start_unit(NQ0 + 2 * j + t, w)

        @pl.when(j == (NJ - NQ0) // 2)
        def _():
            wo_copy.start()
            x_copy.start()
            late_mod.start()
            for cp in ffn_copies:
                cp.start()

        for (dj, dw), (rj, rw) in (((j, 1), (j, 2)), ((j, 2), (j + 1, 0)),
                                   ((j + 1, 0), (j + 1, 1))):
            pre_dot(dj, dw, 0)
            relayout(rj, rw)
            pre_dot(dj, dw, 1)
        return carry

    lax.fori_loop(0, NJ - 1, pre_body, 0)

    def w_head(w, h):
        return _unpk(w_v[w][h // 2, h % 2])

    def ln1(seg, sg):
        x = x_v[seg].astype(F32)[8:SEG]
        h = _layernorm(x) * mod_row(1) + mod_row(0)
        for k in range(KD):
            lhs_v[sg, k, 0:8, :] = _pk(h[0:16, blk(k)])
            hs_v[sg, k] = h[16:24, blk(k)]

    L2 = 2 * L
    rr = lax.broadcasted_iota(jnp.int32, (L2, L2), 0)
    cc = lax.broadcasted_iota(jnp.int32, (L2, L2), 1)
    same = (rr >= L) == (cc >= L)
    rr = jnp.where(rr >= L, rr - L, rr)
    cc = jnp.where(cc >= L, cc - L, cc)
    mask = same & ((rr >= SEG) | (cc >= SEG) | (cc <= rr))
    fill_val = jnp.where(same, -1000000000.0, -jnp.inf).astype(F32)

    def scores(q, k):
        s = lax.dot_general(q, k, (((1,), (1,)), ((), ())),
                            preferred_element_type=F32)
        s = jnp.where(mask, s * scale, fill_val)
        m = jnp.max(s, axis=-1, keepdims=True)
        e = jnp.exp(s - m)
        p = e * _recip(jnp.sum(e, axis=-1, keepdims=True))
        return p.astype(BF16)

    def ln2(xs):
        h = _layernorm(x1_v[xs]) * mod_row(4) + mod_row(3)
        for k in range(KD):
            h2_v[k] = _pk(h[:, blk(k)])

    def up(f):
        h2 = _cat_pk(h2_v, range(KD))
        g = _dot(h2, _unpk(w1_v[:, blk(f)]))
        u = _dot(h2, _unpk(w3_v[:, blk(f)]))
        act_v[f] = _pk(_silu(g) * u)

    def down(xs, j, slot=None):
        a = _cat_pk(act_v, range(NF))
        y = _dot(a, _unpk(w2_v[:, blk(j)]))
        stage_v[xs if slot is None else slot, :, blk(j)] = (
            x1_v[xs, :, blk(j)] + mod_blk(5, j) * y).astype(BF16)


    def segment(i, sg, fill, finish):
        o_v = ob_v if sg else oa_v
        prow = pl.multiple_of(i * 8, 8)
        qk, vs, ps = {}, {}, {}

        def proj(g):
            r = []
            for w in range(3):
                parts = []
                for p in range(2):
                    lhs = _cat_pk(lhs_v.at[sg], range(KD))
                    pre = _unpk(pre_v[w, g, p, pl.ds(prow, 8), :]).astype(F32)
                    parts += [pre[8 * sg:8 * sg + 8],
                              _dot(lhs, w_head(w, 2 * g + p))]
                r.append(jnp.concatenate(parts, axis=0).astype(BF16))
            qk[g] = r[0:2]
            vs[g] = r[2]

        def pv(g):
            o2 = _dot(ps.pop(g), vs.pop(g))
            for p in range(2):
                h = 2 * g + p
                o = o2[p * L:(p + 1) * L]
                if sg == 0:
                    o_v[h] = _pk(jnp.concatenate([o[0:24], o[SEG:L]], axis=0))
                    so_v[h] = o[24:SEG]
                else:
                    o_v[h] = _pk(jnp.concatenate([so_v[h], o], axis=0))

        def wo_part(hs, j):
            lo, hi = hs[0] * (LANE // 2), (hs[-1] + 1) * (LANE // 2)
            return _dot(_cat_pk(o_v, hs), _unpk(wo_v[lo:hi, blk(j)]))

        rows = L + 8 if sg else SEG
        head_hs = list(range(H - TAIL))
        tail_hs = list(range(H - TAIL, H))
        cuts = (0,) + WO_AT
        wo_at = {NJ + t: range(cuts[t], cuts[t + 1]) for t in range(LP)}
        for g in range(NJ + LP):
            if g < NJ:
                proj(g)
            for j in wo_at.get(g, ()):
                acc_v[j, 0:rows, :] = wo_part(head_hs, j)
            if LS <= g < NJ + LS:
                ps[g - LS] = scores(*qk.pop(g - LS))
            if g >= LP:
                pv(g - LP)
            for fn in fill.get(g, ()):
                fn()
        for j in range(WO_AT[-1], KD):
            acc_v[j, 0:rows, :] = wo_part(head_hs, j)
        for j in range(KD):
            finish(j, acc_v[j, 0:rows, :] + wo_part(tail_hs, j))
        for fn in fill.get(NJ + LP, ()):
            fn()

    def attn_pair(i, fill_a, fill_b):
        xs = i % 2

        def finish_a(j, y):
            ya_v[j] = y[0:24]
            lhs_v[1, j, 8:16, :] = _pk(
                jnp.concatenate([hs_v[1, j], y[24:SEG]], axis=0))

        def finish_b(j, y):
            att = jnp.concatenate([ya_v[j], y[0:L]], axis=0)
            x = x_v[pl.ds(2 * i, 2), :, blk(j)].astype(F32).reshape(PAIR, LANE)
            x1_v[xs, :, blk(j)] = x + mod_blk(2, j) * att
            lhs_v[0, j, 8:16, :] = _pk(
                jnp.concatenate([hs_v[0, j], y[L:L + 8]], axis=0))

        segment(i, 0, fill_a, finish_a)
        segment(i, 1, fill_b, finish_b)

    P = functools.partial
    NU0 = 2

    wait_unit(NJ - 1, 2)
    x_copy.wait()
    late_mod.wait()
    mem0_copy.wait()
    wo_copy.wait()
    late = list(range(2 * KD, 6 * KD))
    for n, (w, p) in enumerate(((1, 0), (1, 1), (2, 0), (2, 1))):
        pre_dot(NJ - 1, w, p)
        if n == 0:
            relayout(NJ - 1, 2)
            ln1(0, 0)
            mem0 = mem0_v[...].astype(F32)
            for k in range(KD):
                lhs_v[0, k, 8:16, :] = _pk(jnp.concatenate(
                    [hs_v[0, k], mem0[:, blk(k)]], axis=0))
        if n < 3:
            for j in late[n::3]:
                mod_col(j)

    def head_body(i, carry):
        attn_pair(i, {2: [P(ln1, 2 * i + 1, 1)]},
                  {2: [P(ln2, 1 - i)], 8: [P(ln1, 2 * i + 2, 0)]})
        return carry

    lax.fori_loop(0, 2, head_body, 0)
    for cp in ffn_copies:
        cp.wait()
    for f in range(NU0):
        up(f)

    def body(i, carry):
        slot = i % 2

        @pl.when(i >= 4)
        def _():
            out_copy(i - 4, slot).wait()

        fill_a, fill_b = {}, {}
        for f in range(NU0, NF):
            fill_a.setdefault((f - NU0) // 2, []).append(P(up, f))
        fill_a[NJ + LP] = [P(down, slot, 0)]
        for j in range(1, KD):
            fill_b.setdefault(2 * j - 1, []).append(P(down, slot, j))
        fill_b.setdefault(2, []).append(P(ln2, 1 - slot))
        fill_a.setdefault(2, []).append(P(ln1, 2 * i + 1, 1))
        fill_b.setdefault(8, []).append(
            P(ln1, jnp.minimum(2 * i + 2, NSEG - 1), 0))
        fill_b[NJ + LP] = [P(up, f) for f in range(NU0)]
        attn_pair(i, fill_a, fill_b)
        out_copy(i - 2, slot).start()
        return carry

    lax.fori_loop(2, NP, body, 0)

    s0, s1 = NP % 2, (NP + 1) % 2
    out_copy(NP - 4, s0).wait()
    for f in range(NU0, NF):
        up(f)
    ln2(s1)
    for j in range(KD):
        down(s0, j)
    for f in range(NF):
        up(f)
    for j in range(KD):
        down(s1, j, 2)
    out_copy(NP - 2, s0).start()
    out_copy(NP - 1, 2).start()
    out_copy(NP - 3, s1).wait()
    out_copy(NP - 2, s0).wait()
    out_copy(NP - 1, 2).wait()


@functools.partial(jax.jit, static_argnames=("A_seg_len",))
def pallas_adaLN_cond__memory_aug_recurrent_mem_tr__glu_gated_swiglu__prompt_kernel(
    A_x: jax.Array,
    A_mem0: jax.Array,
    A_Wq: jax.Array,
    A_Wk: jax.Array,
    A_Wv: jax.Array,
    A_Wo: jax.Array,
    A_seg_len,
    B_x: jax.Array,
    B_w1: jax.Array,
    B_w3: jax.Array,
    B_w2: jax.Array,
    c: jax.Array,
    w_mod: jax.Array,
):
    B, S, D = A_x.shape
    H, Dh = A_Wq.shape[1], A_Wq.shape[2]
    F = B_w1.shape[1]
    assert B == 1 and Dh == LANE and A_seg_len == SEG and A_mem0.shape[1] == MEM
    assert S % PAIR == 0 and S // PAIR >= 4 and D % LANE == 0 and F % LANE == 0
    KD, NF = D // LANE, F // LANE
    NSEG = S // SEG

    def split(w):
        return w.reshape(D // 2, 2, H // 2, 2, Dh)

    any_spec = pl.BlockSpec(memory_space=pl.ANY)
    out = pl.pallas_call(
        functools.partial(_kernel, S=S, D=D, H=H, F=F),
        out_shape=jax.ShapeDtypeStruct((S, D), A_x.dtype),
        in_specs=[any_spec] * 11,
        out_specs=any_spec,
        scratch_shapes=[
            pltpu.VMEM((1, D), BF16),
            pltpu.VMEM((MEM, D), BF16),
            pltpu.VMEM((NSEG, SEG, D), BF16),
            pltpu.VMEM((NSEG, 8, D), BF16),
            pltpu.VMEM((NSEG * 8, D), F32),
            pltpu.VMEM((KD, NSEG * 4, LANE), U32),
            pltpu.VMEM((3, H // 2, 2, NSEG * 4, LANE), U32),
            pltpu.VMEM((H // 2, 2, D // 2, LANE), U32),
            pltpu.VMEM((H // 2, 2, D // 2, LANE), U32),
            pltpu.VMEM((H // 2, 2, D // 2, LANE), U32),
            pltpu.VMEM((H * Dh // 2, D + LANE), U32),
            pltpu.VMEM((D // 2, F + LANE), U32),
            pltpu.VMEM((D // 2, F + LANE), U32),
            pltpu.VMEM((F // 2, D + LANE), U32),
            pltpu.VMEM((D // 2, 6 * D), U32),
            pltpu.VMEM((8, 6 * D), F32),
            pltpu.VMEM((2, KD, 8, LANE), F32),
            pltpu.VMEM((2, KD, 16, LANE), U32),
            pltpu.VMEM((H, 8, LANE), F32),
            pltpu.VMEM((H, 16, LANE), U32),
            pltpu.VMEM((H, 24, LANE), U32),
            pltpu.VMEM((KD, 48, LANE), F32),
            pltpu.VMEM((KD, 24, LANE), F32),
            pltpu.VMEM((2, PAIR, D), F32),
            pltpu.VMEM((KD, PAIR // 2, LANE), U32),
            pltpu.VMEM((NF, PAIR // 2, LANE), U32),
            pltpu.VMEM((3, PAIR, D), BF16),
            pltpu.SemaphoreType.DMA((4,)),
            pltpu.SemaphoreType.DMA((5,)),
            pltpu.SemaphoreType.DMA((3 * H // 2,)),
            pltpu.SemaphoreType.DMA((4,)),
            pltpu.SemaphoreType.DMA((3,)),
        ],
        compiler_params=pltpu.CompilerParams(
            vmem_limit_bytes=110 * 1024 * 1024,
            disable_bounds_checks=True,
            disable_semaphore_checks=True),
        name="rmt_block",
    )(A_x.reshape(NSEG, SEG, D), A_mem0.reshape(MEM, D), split(A_Wq), split(A_Wk),
      split(A_Wv), A_Wo.reshape(H * Dh, D), B_w1, B_w3, B_w2, c, w_mod)
    return out.reshape(B, S, D)
```

```python
import functools

import jax
import jax.numpy as jnp
from jax import lax
import jax.experimental.pallas as pl
import jax.experimental.pallas.tpu as pltpu

F32 = jnp.float32
BF16 = jnp.bfloat16
U32 = jnp.uint32

LANE = 128
SEG = 32
MEM = 8
PAIR = 2 * SEG
EPS = 1e-5

LS, LP = 1, 3
TAIL = 8
WO_AT = (2, 4, 6)


def _dot(a, b):
    return jnp.dot(a, b, preferred_element_type=F32)


def _cat_lanes(ref, n):
    return jnp.concatenate([ref[k] for k in range(n)], axis=1)


def _layernorm(x):
    m = jnp.mean(x, axis=-1, keepdims=True)
    xc = x - m
    v = jnp.mean(xc * xc, axis=-1, keepdims=True)
    return xc * lax.rsqrt(v + EPS)


def _silu(x):
    hx = 0.5 * x
    return hx + hx * jnp.tanh(hx)


def _recip(x):
    r = pl.reciprocal(x, approx=True)
    return r * (2.0 - x * r)


def _pk(x):
    return pltpu.bitcast(x.astype(BF16), U32)


def _unpk(x):
    return pltpu.bitcast(x, BF16)


def _cat_pk(ref, ks):
    return jnp.concatenate([_unpk(ref[k]) for k in ks], axis=1)


def _kernel(x_hbm, mem0_hbm, wq_hbm, wk_hbm, wv_hbm, wo_hbm, w1_hbm, w3_hbm,
            w2_hbm, c_hbm, wmod_hbm, out_hbm,
            c_v, mem0_v, x_v, xpre_v, xn_v, hpre_v, pre_v, wq_v, wk_v, wv_v,
            wo_v, w1_v, w3_v, w2_v, wmod_v,
            mod_v, hs_v, lhs_v, so_v, oa_v, ob_v, acc_v, ya_v,
            x1_v, h2_v, act_v, stage_v,
            sem_x, sem_mod, sem_qkv, sem_w, sem_out,
            *, S, D, H, F):
    KD = D // LANE
    NF = F // LANE
    NP = S // PAIR
    NSEG = S // SEG
    NJ = H // 2
    L = SEG + MEM
    scale = float(LANE) ** -0.5
    w_hbm = (wq_hbm, wk_hbm, wv_hbm)
    w_v = (wq_v, wk_v, wv_v)

    def blk(j):
        return slice(j * LANE, (j + 1) * LANE)

    NCH = 4
    CK = KD // NCH

    def mod_copy(c0, n, sem):
        return pltpu.make_async_copy(
            wmod_hbm.bitcast(U32).at[:, pl.ds(c0, n)],
            wmod_v.at[:, pl.ds(c0, n)], sem)

    def early_mod(ch):
        return [mod_copy(t * D + ch * CK * LANE, CK * LANE, sem_mod.at[ch])
                for t in range(2)]

    late_mod = mod_copy(2 * D, 4 * D, sem_mod.at[NCH])

    def unit_copy(j, w):
        return pltpu.make_async_copy(
            w_hbm[w].bitcast(U32).at[:, :, j, 0, :],
            w_v[w].at[j], sem_qkv.at[3 * j + w])

    def start_unit(j, w):
        unit_copy(j, w).start()

    def wait_unit(j, w):
        unit_copy(j, w).wait()

    def w_copy(src, dst, k):
        return pltpu.make_async_copy(
            src.bitcast(U32), dst.at[:, pl.ds(0, src.shape[1])], sem_w.at[k])

    wo_copy = w_copy(wo_hbm, wo_v, 0)
    ffn_copies = [w_copy(w1_hbm, w1_v, 1), w_copy(w3_hbm, w3_v, 2),
                  w_copy(w2_hbm, w2_v, 3)]
    c_copy = pltpu.make_async_copy(c_hbm, c_v, sem_x.at[2])
    mem0_copy = pltpu.make_async_copy(mem0_hbm, mem0_v, sem_x.at[3])
    xpre_copy = pltpu.make_async_copy(
        x_hbm.at[:, pl.ds(0, 8), :], xpre_v, sem_x.at[0])
    x_copy = pltpu.make_async_copy(x_hbm, x_v, sem_x.at[1])

    def out_copy(i, slot):
        return pltpu.make_async_copy(
            stage_v.at[slot], out_hbm.at[pl.ds(i * PAIR, PAIR), :],
            sem_out.at[slot])

    xpre_copy.start()
    c_copy.start()
    for ch in range(NCH - 1):
        for cp in early_mod(ch):
            cp.start()
    start_unit(0, 0)
    for cp in early_mod(NCH - 1):
        cp.start()
    for j in range(NJ):
        for w in range(3):
            if (j, w) != (0, 0):
                start_unit(j, w)
    mem0_copy.start()
    x1_v[1] = jnp.zeros((PAIR, D), F32)

    xpre_copy.wait()

    def ln_pre(b, carry):
        x = xpre_v[pl.ds(b * 8, 8)].astype(F32).reshape(64, D)
        xn_v[pl.ds(pl.multiple_of(b * 64, 64), 64), :] = _layernorm(x)
        return carry

    lax.fori_loop(0, NSEG // 8, ln_pre, 0)

    c_copy.wait()
    c = c_v[...].astype(F32)
    sc = _silu(c).astype(BF16)
    sc = jnp.broadcast_to(sc, (16, D))

    def mod_col(j):
        r = _dot(sc, _unpk(wmod_v[:, blk(j)]))[0:8]
        if j // KD in (1, 4):
            r = r + 1.0
        mod_v[:, blk(j)] = r

    def mod_row(k):
        return mod_v[0:1, k * D:(k + 1) * D]

    def mod_blk(k, j):
        return mod_v[0:1, k * D + j * LANE:k * D + (j + 1) * LANE]

    def relayout(j, w):
        for r in range(0, D // 16, 8):
            a = w_v[w][j, r:r + 8, pl.ds(0, 8, stride=2), :]
            b = w_v[w][j, r:r + 8, pl.ds(1, 8, stride=2), :]
            w_v[w][j, r:r + 8, 0:8, :] = (a & U32(0xFFFF)) | (b << 16)
            w_v[w][j, r:r + 8, 8:16, :] = (a >> 16) | (b & U32(0xFFFF0000))

    def w_head(w, j, p):
        return _unpk(w_v[w][j, :, 8 * p:8 * p + 8, :].reshape(D // 2, LANE))

    for ch in range(NCH):
        if ch == NCH - 1:
            wait_unit(0, 0)
            relayout(0, 0)
        for cp in early_mod(ch):
            cp.wait()
        for k in range(ch * CK, (ch + 1) * CK):
            mod_col(k)
            mod_col(KD + k)
        for k in range(ch * CK, (ch + 1) * CK):
            for r in range(0, NSEG * 8, 128):
                hpre_v[k, r // 2:r // 2 + 64, :] = _pk(
                    xn_v[r:r + 128, blk(k)] * mod_blk(1, k) + mod_blk(0, k))

    def pre_dot(j, w, p):
        hp = _cat_pk(hpre_v, range(KD))
        pre_v[w, j, p] = _pk(_dot(hp, w_head(w, j, p)))

    wait_unit(0, 1)
    wo_copy.start()
    x_copy.start()
    late_mod.start()
    for cp in ffn_copies:
        cp.start()
    pre_dot(0, 0, 0)
    relayout(0, 1)
    pre_dot(0, 0, 1)

    def pre_body(j, carry):
        wait_unit(j, 2)
        wait_unit(j + 1, 0)
        wait_unit(j + 1, 1)

        for (dj, dw), (rj, rw) in (((j, 1), (j, 2)), ((j, 2), (j + 1, 0)),
                                   ((j + 1, 0), (j + 1, 1))):
            pre_dot(dj, dw, 0)
            relayout(rj, rw)
            pre_dot(dj, dw, 1)
        return carry

    lax.fori_loop(0, NJ - 1, pre_body, 0)

    def ln1(seg, sg):
        x = x_v[seg].astype(F32)[8:SEG]
        h = _layernorm(x) * mod_row(1) + mod_row(0)
        for k in range(KD):
            lhs_v[sg, k, 0:8, :] = _pk(h[0:16, blk(k)])
            hs_v[sg, k] = h[16:24, blk(k)]

    L2 = 2 * L
    rr = lax.broadcasted_iota(jnp.int32, (L2, L2), 0)
    cc = lax.broadcasted_iota(jnp.int32, (L2, L2), 1)
    same = (rr >= L) == (cc >= L)
    rr = jnp.where(rr >= L, rr - L, rr)
    cc = jnp.where(cc >= L, cc - L, cc)
    mask = same & ((rr >= SEG) | (cc >= SEG) | (cc <= rr))
    fill_val = jnp.where(same, -1000000000.0, -jnp.inf).astype(F32)

    def scores(q, k):
        s = lax.dot_general(q, k, (((1,), (1,)), ((), ())),
                            preferred_element_type=F32)
        s = jnp.where(mask, s * scale, fill_val)
        m = jnp.max(s, axis=-1, keepdims=True)
        e = jnp.exp(s - m)
        p = e * _recip(jnp.sum(e, axis=-1, keepdims=True))
        return p.astype(BF16)

    def ln2(xs):
        h = _layernorm(x1_v[xs]) * mod_row(4) + mod_row(3)
        for k in range(KD):
            h2_v[k] = _pk(h[:, blk(k)])

    def up(f):
        h2 = _cat_pk(h2_v, range(KD))
        g = _dot(h2, _unpk(w1_v[:, blk(f)]))
        u = _dot(h2, _unpk(w3_v[:, blk(f)]))
        act_v[f] = _pk(_silu(g) * u)

    def down(xs, j, slot=None):
        a = _cat_pk(act_v, range(NF))
        y = _dot(a, _unpk(w2_v[:, blk(j)]))
        stage_v[xs if slot is None else slot, :, blk(j)] = (
            x1_v[xs, :, blk(j)] + mod_blk(5, j) * y).astype(BF16)


    def segment(i, sg, fill, finish):
        o_v = ob_v if sg else oa_v
        prow = pl.multiple_of(i * 8, 8)
        qk, vs, ps = {}, {}, {}

        def proj(g):
            r = []
            for w in range(3):
                parts = []
                for p in range(2):
                    lhs = _cat_pk(lhs_v.at[sg], range(KD))
                    pre = _unpk(pre_v[w, g, p, pl.ds(prow, 8), :]).astype(F32)
                    parts += [pre[8 * sg:8 * sg + 8],
                              _dot(lhs, w_head(w, g, p))]
                r.append(jnp.concatenate(parts, axis=0).astype(BF16))
            qk[g] = r[0:2]
            vs[g] = r[2]

        def pv(g):
            o2 = _dot(ps.pop(g), vs.pop(g))
            for p in range(2):
                h = 2 * g + p
                o = o2[p * L:(p + 1) * L]
                if sg == 0:
                    o_v[h] = _pk(jnp.concatenate([o[0:24], o[SEG:L]], axis=0))
                    so_v[h] = o[24:SEG]
                else:
                    o_v[h] = _pk(jnp.concatenate([so_v[h], o], axis=0))

        def wo_part(hs, j):
            lo, hi = hs[0] * (LANE // 2), (hs[-1] + 1) * (LANE // 2)
            return _dot(_cat_pk(o_v, hs), _unpk(wo_v[lo:hi, blk(j)]))

        rows = L + 8 if sg else SEG
        head_hs = list(range(H - TAIL))
        tail_hs = list(range(H - TAIL, H))
        cuts = (0,) + WO_AT
        wo_at = {NJ + t: range(cuts[t], cuts[t + 1]) for t in range(LP)}
        for g in range(NJ + LP):
            if g < NJ:
                proj(g)
            for j in wo_at.get(g, ()):
                acc_v[j, 0:rows, :] = wo_part(head_hs, j)
            if LS <= g < NJ + LS:
                ps[g - LS] = scores(*qk.pop(g - LS))
            if g >= LP:
                pv(g - LP)
            for fn in fill.get(g, ()):
                fn()
        for j in range(WO_AT[-1], KD):
            acc_v[j, 0:rows, :] = wo_part(head_hs, j)
        for j in range(KD):
            finish(j, acc_v[j, 0:rows, :] + wo_part(tail_hs, j))
        for fn in fill.get(NJ + LP, ()):
            fn()

    def attn_pair(i, fill_a, fill_b):
        xs = i % 2

        def finish_a(j, y):
            ya_v[j] = y[0:24]
            lhs_v[1, j, 8:16, :] = _pk(
                jnp.concatenate([hs_v[1, j], y[24:SEG]], axis=0))

        def finish_b(j, y):
            att = jnp.concatenate([ya_v[j], y[0:L]], axis=0)
            x = x_v[pl.ds(2 * i, 2), :, blk(j)].astype(F32).reshape(PAIR, LANE)
            x1_v[xs, :, blk(j)] = x + mod_blk(2, j) * att
            lhs_v[0, j, 8:16, :] = _pk(
                jnp.concatenate([hs_v[0, j], y[L:L + 8]], axis=0))

        segment(i, 0, fill_a, finish_a)
        segment(i, 1, fill_b, finish_b)

    P = functools.partial
    NU0 = 2

    wait_unit(NJ - 1, 2)
    x_copy.wait()
    late_mod.wait()
    mem0_copy.wait()
    wo_copy.wait()
    late = list(range(2 * KD, 6 * KD))
    for n, (w, p) in enumerate(((1, 0), (1, 1), (2, 0), (2, 1))):
        pre_dot(NJ - 1, w, p)
        if n == 0:
            relayout(NJ - 1, 2)
            ln1(0, 0)
            mem0 = mem0_v[...].astype(F32)
            for k in range(KD):
                lhs_v[0, k, 8:16, :] = _pk(jnp.concatenate(
                    [hs_v[0, k], mem0[:, blk(k)]], axis=0))
        if n < 3:
            for j in late[n::3]:
                mod_col(j)

    def head_body(i, carry):
        attn_pair(i, {2: [P(ln1, 2 * i + 1, 1)]},
                  {2: [P(ln2, 1 - i)], 8: [P(ln1, 2 * i + 2, 0)]})
        return carry

    lax.fori_loop(0, 2, head_body, 0)
    for cp in ffn_copies:
        cp.wait()
    for f in range(NU0):
        up(f)

    def body(i, carry):
        slot = i % 2

        @pl.when(i >= 4)
        def _():
            out_copy(i - 4, slot).wait()

        fill_a, fill_b = {}, {}
        for f in range(NU0, NF):
            fill_a.setdefault((f - NU0) * 16 // (NF - NU0), []).append(P(up, f))
        fill_a[NJ + LP] = [P(down, slot, 0)]
        for j in range(1, KD):
            fill_b.setdefault(2 * j - 1, []).append(P(down, slot, j))
        fill_b.setdefault(2, []).append(P(ln2, 1 - slot))
        fill_a.setdefault(2, []).append(P(ln1, 2 * i + 1, 1))
        fill_b.setdefault(8, []).append(
            P(ln1, jnp.minimum(2 * i + 2, NSEG - 1), 0))
        fill_b[NJ + LP] = [P(up, f) for f in range(NU0)]
        attn_pair(i, fill_a, fill_b)
        out_copy(i - 2, slot).start()
        return carry

    lax.fori_loop(2, NP, body, 0)

    s0, s1 = NP % 2, (NP + 1) % 2
    out_copy(NP - 4, s0).wait()
    for f in range(NU0, NF):
        up(f)
    ln2(s1)
    for j in range(KD):
        down(s0, j)
    for f in range(NF):
        up(f)
    for j in range(KD):
        down(s1, j, 2)
    out_copy(NP - 2, s0).start()
    out_copy(NP - 1, 2).start()
    out_copy(NP - 3, s1).wait()
    out_copy(NP - 2, s0).wait()
    out_copy(NP - 1, 2).wait()


@functools.partial(jax.jit, static_argnames=("A_seg_len",))
def pallas_adaLN_cond__memory_aug_recurrent_mem_tr__glu_gated_swiglu__prompt_kernel(
    A_x: jax.Array,
    A_mem0: jax.Array,
    A_Wq: jax.Array,
    A_Wk: jax.Array,
    A_Wv: jax.Array,
    A_Wo: jax.Array,
    A_seg_len,
    B_x: jax.Array,
    B_w1: jax.Array,
    B_w3: jax.Array,
    B_w2: jax.Array,
    c: jax.Array,
    w_mod: jax.Array,
):
    B, S, D = A_x.shape
    H, Dh = A_Wq.shape[1], A_Wq.shape[2]
    F = B_w1.shape[1]
    assert B == 1 and Dh == LANE and A_seg_len == SEG and A_mem0.shape[1] == MEM
    assert S % PAIR == 0 and S // PAIR >= 4 and D % LANE == 0 and F % LANE == 0
    KD, NF = D // LANE, F // LANE
    NSEG = S // SEG

    def split(w):
        return w.reshape(D // 16, 16, H // 2, 2, Dh)

    any_spec = pl.BlockSpec(memory_space=pl.ANY)
    out = pl.pallas_call(
        functools.partial(_kernel, S=S, D=D, H=H, F=F),
        out_shape=jax.ShapeDtypeStruct((S, D), A_x.dtype),
        in_specs=[any_spec] * 11,
        out_specs=any_spec,
        scratch_shapes=[
            pltpu.VMEM((1, D), BF16),
            pltpu.VMEM((MEM, D), BF16),
            pltpu.VMEM((NSEG, SEG, D), BF16),
            pltpu.VMEM((NSEG, 8, D), BF16),
            pltpu.VMEM((NSEG * 8, D), F32),
            pltpu.VMEM((KD, NSEG * 4, LANE), U32),
            pltpu.VMEM((3, H // 2, 2, NSEG * 4, LANE), U32),
            pltpu.VMEM((H // 2, D // 16, 16, LANE), U32),
            pltpu.VMEM((H // 2, D // 16, 16, LANE), U32),
            pltpu.VMEM((H // 2, D // 16, 16, LANE), U32),
            pltpu.VMEM((H * Dh // 2, D + LANE), U32),
            pltpu.VMEM((D // 2, F + LANE), U32),
            pltpu.VMEM((D // 2, F + LANE), U32),
            pltpu.VMEM((F // 2, D + LANE), U32),
            pltpu.VMEM((D // 2, 6 * D), U32),
            pltpu.VMEM((8, 6 * D), F32),
            pltpu.VMEM((2, KD, 8, LANE), F32),
            pltpu.VMEM((2, KD, 16, LANE), U32),
            pltpu.VMEM((H, 8, LANE), F32),
            pltpu.VMEM((H, 16, LANE), U32),
            pltpu.VMEM((H, 24, LANE), U32),
            pltpu.VMEM((KD, 48, LANE), F32),
            pltpu.VMEM((KD, 24, LANE), F32),
            pltpu.VMEM((2, PAIR, D), F32),
            pltpu.VMEM((KD, PAIR // 2, LANE), U32),
            pltpu.VMEM((NF, PAIR // 2, LANE), U32),
            pltpu.VMEM((3, PAIR, D), BF16),
            pltpu.SemaphoreType.DMA((4,)),
            pltpu.SemaphoreType.DMA((5,)),
            pltpu.SemaphoreType.DMA((3 * H // 2,)),
            pltpu.SemaphoreType.DMA((4,)),
            pltpu.SemaphoreType.DMA((3,)),
        ],
        compiler_params=pltpu.CompilerParams(
            vmem_limit_bytes=110 * 1024 * 1024,
            disable_bounds_checks=True,
            disable_semaphore_checks=True),
        name="rmt_block",
    )(A_x.reshape(NSEG, SEG, D), A_mem0.reshape(MEM, D), split(A_Wq), split(A_Wk),
      split(A_Wv), A_Wo.reshape(H * Dh, D), B_w1, B_w3, B_w2, c, w_mod)
    return out.reshape(B, S, D)
```

```python
import functools

import jax
import jax.numpy as jnp
from jax import lax
import jax.experimental.pallas as pl
import jax.experimental.pallas.tpu as pltpu

F32 = jnp.float32
BF16 = jnp.bfloat16
U32 = jnp.uint32

LANE = 128
SEG = 32
MEM = 8
PAIR = 2 * SEG
EPS = 1e-5

LS, LP = 1, 3
TAIL = 8
WO_AT = (2, 4, 6)


def _dot(a, b):
    return jnp.dot(a, b, preferred_element_type=F32)


def _cat_lanes(ref, n):
    return jnp.concatenate([ref[k] for k in range(n)], axis=1)


def _layernorm(x):
    m = jnp.mean(x, axis=-1, keepdims=True)
    xc = x - m
    v = jnp.mean(xc * xc, axis=-1, keepdims=True)
    return xc * lax.rsqrt(v + EPS)


def _silu(x):
    hx = 0.5 * x
    return hx + hx * jnp.tanh(hx)


def _recip(x):
    r = pl.reciprocal(x, approx=True)
    return r * (2.0 - x * r)


def _pk(x):
    return pltpu.bitcast(x.astype(BF16), U32)


def _unpk(x):
    return pltpu.bitcast(x, BF16)


def _cat_pk(ref, ks):
    return jnp.concatenate([_unpk(ref[k]) for k in ks], axis=1)


def _kernel(x_hbm, mem0_hbm, wq_hbm, wk_hbm, wv_hbm, wo_hbm, w1_hbm, w3_hbm,
            w2_hbm, c_hbm, wmod_hbm, out_hbm,
            c_v, mem0_v, x_v, xpre_v, xn_v, hpre_v, acc0_v, pre_v,
            wq_v, wk_v, wv_v, wo_v, w1_v, w3_v, w2_v, wme_v, wml_v,
            mod_v, hs_v, lhs_v, so_v, oa_v, ob_v, acc_v, ya_v,
            x1_v, h2_v, act_v, stage_v,
            sem_x, sem_mod, sem_qkv, sem_w, sem_out,
            *, S, D, H, F):
    KD = D // LANE
    NF = F // LANE
    NP = S // PAIR
    NSEG = S // SEG
    NJ = H // 2
    L = SEG + MEM
    scale = float(LANE) ** -0.5
    w_hbm = (wq_hbm, wk_hbm, wv_hbm)
    w_v = (wq_v, wk_v, wv_v)

    def blk(j):
        return slice(j * LANE, (j + 1) * LANE)

    NCH = 4
    CK = KD // NCH

    def early_mod(ch):
        return [pltpu.make_async_copy(
            wmod_hbm.bitcast(U32).at[:, pl.ds(
                pl.multiple_of(t * D + ch * (CK * LANE), LANE), CK * LANE)],
            wme_v.at[ch, t], sem_mod.at[ch]) for t in range(2)]

    late_mod = pltpu.make_async_copy(
        wmod_hbm.bitcast(U32).at[:, pl.ds(2 * D, 4 * D)], wml_v,
        sem_mod.at[NCH])

    def unit_copy(j, w):
        return pltpu.make_async_copy(
            w_hbm[w].bitcast(U32).at[:, :, j, 0, :],
            w_v[w].at[j], sem_qkv.at[3 * j + w])

    def start_unit(j, w):
        unit_copy(j, w).start()

    def wait_unit(j, w):
        unit_copy(j, w).wait()

    def w_copy(src, dst, k):
        return pltpu.make_async_copy(
            src.bitcast(U32), dst.at[:, pl.ds(0, src.shape[1])], sem_w.at[k])

    wo_copy = w_copy(wo_hbm, wo_v, 0)
    ffn_copies = [w_copy(w1_hbm, w1_v, 1), w_copy(w3_hbm, w3_v, 2),
                  w_copy(w2_hbm, w2_v, 3)]
    c_copy = pltpu.make_async_copy(c_hbm, c_v, sem_x.at[2])
    mem0_copy = pltpu.make_async_copy(mem0_hbm, mem0_v, sem_x.at[3])
    xpre_copy = pltpu.make_async_copy(
        x_hbm.at[:, pl.ds(0, 8), :], xpre_v, sem_x.at[0])
    x_copy = pltpu.make_async_copy(x_hbm, x_v, sem_x.at[1])

    def out_copy(i, slot):
        return pltpu.make_async_copy(
            stage_v.at[slot], out_hbm.at[pl.ds(i * PAIR, PAIR), :],
            sem_out.at[slot])

    first_units = ((0, 0), (0, 1), (0, 2), (1, 0))
    xpre_copy.start()
    c_copy.start()
    for j, w in first_units:
        start_unit(j, w)
    for ch in range(NCH):
        for cp in early_mod(ch):
            cp.start()
    for j in range(NJ):
        for w in range(3):
            if (j, w) not in first_units:
                start_unit(j, w)
    mem0_copy.start()
    x1_v[1] = jnp.zeros((PAIR, D), F32)

    xpre_copy.wait()

    def ln_pre(b, carry):
        x = xpre_v[pl.ds(b * 8, 8)].astype(F32).reshape(64, D)
        xn = _layernorm(x)
        r0 = pl.multiple_of(b * 64, 64)
        for k in range(KD):
            xn_v[k, pl.ds(r0, 64), :] = xn[:, blk(k)]
        for u in range(len(first_units)):
            acc0_v[u, pl.ds(r0, 64), :] = jnp.zeros((64, 2 * LANE), F32)
        return carry

    lax.fori_loop(0, NSEG // 8, ln_pre, 0)

    def relayout(j, w):
        for r in range(0, D // 16, 8):
            a = w_v[w][j, r:r + 8, pl.ds(0, 8, stride=2), :]
            b = w_v[w][j, r:r + 8, pl.ds(1, 8, stride=2), :]
            w_v[w][j, r:r + 8, 0:8, :] = (a & U32(0xFFFF)) | (b << 16)
            w_v[w][j, r:r + 8, 8:16, :] = (a >> 16) | (b & U32(0xFFFF0000))

    def w_head(w, j, p, k0=0, nk=KD):
        t = w_v[w][j, pl.ds(k0 * 8, nk * 8), 8 * p:8 * p + 8, :]
        return _unpk(t.reshape(nk * LANE // 2, LANE))

    c_copy.wait()
    for j, w in first_units:
        wait_unit(j, w)
    wo_copy.start()
    x_copy.start()
    late_mod.start()
    for cp in ffn_copies:
        cp.start()
    for j, w in first_units:
        relayout(j, w)

    c = c_v[...].astype(F32)
    sc = _silu(c).astype(BF16)
    sc = jnp.broadcast_to(sc, (16, D))

    def mod_row(k):
        return jnp.concatenate([mod_blk(k, j) for j in range(KD)], axis=1)

    def mod_blk(k, j):
        return mod_v[k * KD + j, 0:1, :]

    def late_mod_col(j):
        r = _dot(sc, _unpk(wml_v[:, blk(j - 2 * KD)]))[0:8]
        if j // KD == 4:
            r = r + 1.0
        mod_v[j] = r

    def chunk_body(ch, carry):
        for cp in early_mod(ch):
            cp.wait()
        k0 = ch * CK
        for kk in range(CK):
            sa = _dot(sc, _unpk(wme_v[ch, 0, :, blk(kk)]))[0:8]
            ca = _dot(sc, _unpk(wme_v[ch, 1, :, blk(kk)]))[0:8] + 1.0
            mod_v[k0 + kk] = sa
            mod_v[KD + k0 + kk] = ca
            for r in range(0, NSEG * 8, 128):
                hpre_v[k0 + kk, r // 2:r // 2 + 64, :] = _pk(
                    xn_v[k0 + kk, r:r + 128, :] * ca[0:1] + sa[0:1])
        for u, (j, w) in enumerate(first_units):
            hp = jnp.concatenate(
                [_unpk(hpre_v[k0 + kk]) for kk in range(CK)], axis=1)
            wt = jnp.concatenate(
                [w_head(w, j, p, k0, CK) for p in range(2)], axis=1)
            acc = acc0_v[u] + _dot(hp, wt)
            acc0_v[u] = acc
            for p in range(2):
                pre_v[w, j, p] = _pk(acc[:, blk(p)])
        return carry

    lax.fori_loop(0, NCH, chunk_body, 0)

    def pre_dot(j, w, p):
        hp = _cat_pk(hpre_v, range(KD))
        pre_v[w, j, p] = _pk(_dot(hp, w_head(w, j, p)))

    wait_unit(1, 1)
    relayout(1, 1)

    def pre_body(j, carry):
        wait_unit(j, 2)
        wait_unit(j + 1, 0)
        wait_unit(j + 1, 1)

        for (dj, dw), (rj, rw) in (((j, 1), (j, 2)), ((j, 2), (j + 1, 0)),
                                   ((j + 1, 0), (j + 1, 1))):
            pre_dot(dj, dw, 0)
            relayout(rj, rw)
            pre_dot(dj, dw, 1)
        return carry

    lax.fori_loop(1, NJ - 1, pre_body, 0)

    def ln1(seg, sg):
        x = x_v[seg].astype(F32)[8:SEG]
        h = _layernorm(x) * mod_row(1) + mod_row(0)
        for k in range(KD):
            lhs_v[sg, k, 0:8, :] = _pk(h[0:16, blk(k)])
            hs_v[sg, k] = h[16:24, blk(k)]

    L2 = 2 * L
    rr = lax.broadcasted_iota(jnp.int32, (L2, L2), 0)
    cc = lax.broadcasted_iota(jnp.int32, (L2, L2), 1)
    same = (rr >= L) == (cc >= L)
    rr = jnp.where(rr >= L, rr - L, rr)
    cc = jnp.where(cc >= L, cc - L, cc)
    mask = same & ((rr >= SEG) | (cc >= SEG) | (cc <= rr))
    fill_val = jnp.where(same, -1000000000.0, -jnp.inf).astype(F32)

    def scores(q, k):
        s = lax.dot_general(q, k, (((1,), (1,)), ((), ())),
                            preferred_element_type=F32)
        s = jnp.where(mask, s * scale, fill_val)
        m = jnp.max(s, axis=-1, keepdims=True)
        e = jnp.exp(s - m)
        p = e * _recip(jnp.sum(e, axis=-1, keepdims=True))
        return p.astype(BF16)

    def ln2(xs):
        h = _layernorm(x1_v[xs]) * mod_row(4) + mod_row(3)
        for k in range(KD):
            h2_v[k] = _pk(h[:, blk(k)])

    def up(f):
        h2 = _cat_pk(h2_v, range(KD))
        g = _dot(h2, _unpk(w1_v[:, blk(f)]))
        u = _dot(h2, _unpk(w3_v[:, blk(f)]))
        act_v[f] = _pk(_silu(g) * u)

    def down(xs, j, slot=None):
        a = _cat_pk(act_v, range(NF))
        y = _dot(a, _unpk(w2_v[:, blk(j)]))
        stage_v[xs if slot is None else slot, :, blk(j)] = (
            x1_v[xs, :, blk(j)] + mod_blk(5, j) * y).astype(BF16)


    def segment(i, sg, fill, finish):
        o_v = ob_v if sg else oa_v
        prow = pl.multiple_of(i * 8, 8)
        qk, vs, ps = {}, {}, {}

        def proj(g):
            r = []
            for w in range(3):
                parts = []
                for p in range(2):
                    lhs = _cat_pk(lhs_v.at[sg], range(KD))
                    pre = _unpk(pre_v[w, g, p, pl.ds(prow, 8), :]).astype(F32)
                    parts += [pre[8 * sg:8 * sg + 8],
                              _dot(lhs, w_head(w, g, p))]
                r.append(jnp.concatenate(parts, axis=0).astype(BF16))
            qk[g] = r[0:2]
            vs[g] = r[2]

        def pv(g):
            o2 = _dot(ps.pop(g), vs.pop(g))
            for p in range(2):
                h = 2 * g + p
                o = o2[p * L:(p + 1) * L]
                if sg == 0:
                    o_v[h] = _pk(jnp.concatenate([o[0:24], o[SEG:L]], axis=0))
                    so_v[h] = o[24:SEG]
                else:
                    o_v[h] = _pk(jnp.concatenate([so_v[h], o], axis=0))

        def wo_part(hs, j):
            lo, hi = hs[0] * (LANE // 2), (hs[-1] + 1) * (LANE // 2)
            return _dot(_cat_pk(o_v, hs), _unpk(wo_v[lo:hi, blk(j)]))

        rows = L + 8 if sg else SEG
        head_hs = list(range(H - TAIL))
        tail_hs = list(range(H - TAIL, H))
        cuts = (0,) + WO_AT
        wo_at = {NJ + t: range(cuts[t], cuts[t + 1]) for t in range(LP)}
        for g in range(NJ + LP):
            if g < NJ:
                proj(g)
            for j in wo_at.get(g, ()):
                acc_v[j, 0:rows, :] = wo_part(head_hs, j)
            if LS <= g < NJ + LS:
                ps[g - LS] = scores(*qk.pop(g - LS))
            if g >= LP:
                pv(g - LP)
            for fn in fill.get(g, ()):
                fn()
        for j in range(WO_AT[-1], KD):
            acc_v[j, 0:rows, :] = wo_part(head_hs, j)
        for j in range(KD):
            finish(j, acc_v[j, 0:rows, :] + wo_part(tail_hs, j))
        for fn in fill.get(NJ + LP, ()):
            fn()

    def attn_pair(i, fill_a, fill_b):
        xs = i % 2

        def finish_a(j, y):
            ya_v[j] = y[0:24]
            lhs_v[1, j, 8:16, :] = _pk(
                jnp.concatenate([hs_v[1, j], y[24:SEG]], axis=0))

        def finish_b(j, y):
            att = jnp.concatenate([ya_v[j], y[0:L]], axis=0)
            x = x_v[pl.ds(2 * i, 2), :, blk(j)].astype(F32).reshape(PAIR, LANE)
            x1_v[xs, :, blk(j)] = x + mod_blk(2, j) * att
            lhs_v[0, j, 8:16, :] = _pk(
                jnp.concatenate([hs_v[0, j], y[L:L + 8]], axis=0))

        segment(i, 0, fill_a, finish_a)
        segment(i, 1, fill_b, finish_b)

    P = functools.partial
    NU0 = 2

    wait_unit(NJ - 1, 2)
    x_copy.wait()
    late_mod.wait()
    mem0_copy.wait()
    wo_copy.wait()
    late = list(range(2 * KD, 6 * KD))
    for n, (w, p) in enumerate(((1, 0), (1, 1), (2, 0), (2, 1))):
        pre_dot(NJ - 1, w, p)
        if n == 0:
            relayout(NJ - 1, 2)
            ln1(0, 0)
            mem0 = mem0_v[...].astype(F32)
            for k in range(KD):
                lhs_v[0, k, 8:16, :] = _pk(jnp.concatenate(
                    [hs_v[0, k], mem0[:, blk(k)]], axis=0))
        if n < 3:
            for j in late[n::3]:
                late_mod_col(j)

    def head_body(i, carry):
        attn_pair(i, {2: [P(ln1, 2 * i + 1, 1)]},
                  {2: [P(ln2, 1 - i)], 8: [P(ln1, 2 * i + 2, 0)]})
        return carry

    lax.fori_loop(0, 2, head_body, 0)
    for cp in ffn_copies:
        cp.wait()
    for f in range(NU0):
        up(f)

    def body(i, carry):
        slot = i % 2

        @pl.when(i >= 4)
        def _():
            out_copy(i - 4, slot).wait()

        fill_a, fill_b = {}, {}
        for f in range(NU0, NF):
            fill_a.setdefault((f - NU0) * 16 // (NF - NU0), []).append(P(up, f))
        fill_a[NJ + LP] = [P(down, slot, 0)]
        for j in range(1, KD):
            fill_b.setdefault(2 * j - 1, []).append(P(down, slot, j))
        fill_b.setdefault(2, []).append(P(ln2, 1 - slot))
        fill_a.setdefault(2, []).append(P(ln1, 2 * i + 1, 1))
        fill_b.setdefault(8, []).append(
            P(ln1, jnp.minimum(2 * i + 2, NSEG - 1), 0))
        fill_b[NJ + LP] = [P(up, f) for f in range(NU0)]
        attn_pair(i, fill_a, fill_b)
        out_copy(i - 2, slot).start()
        return carry

    lax.fori_loop(2, NP, body, 0)

    s0, s1 = NP % 2, (NP + 1) % 2
    out_copy(NP - 4, s0).wait()
    for f in range(NU0, NF):
        up(f)
    ln2(s1)
    for j in range(KD):
        down(s0, j)
    for f in range(NF):
        up(f)
    for j in range(KD):
        down(s1, j, 2)
    out_copy(NP - 2, s0).start()
    out_copy(NP - 1, 2).start()
    out_copy(NP - 3, s1).wait()
    out_copy(NP - 2, s0).wait()
    out_copy(NP - 1, 2).wait()


@functools.partial(jax.jit, static_argnames=("A_seg_len",))
def pallas_adaLN_cond__memory_aug_recurrent_mem_tr__glu_gated_swiglu__prompt_kernel(
    A_x: jax.Array,
    A_mem0: jax.Array,
    A_Wq: jax.Array,
    A_Wk: jax.Array,
    A_Wv: jax.Array,
    A_Wo: jax.Array,
    A_seg_len,
    B_x: jax.Array,
    B_w1: jax.Array,
    B_w3: jax.Array,
    B_w2: jax.Array,
    c: jax.Array,
    w_mod: jax.Array,
):
    B, S, D = A_x.shape
    H, Dh = A_Wq.shape[1], A_Wq.shape[2]
    F = B_w1.shape[1]
    assert B == 1 and Dh == LANE and A_seg_len == SEG and A_mem0.shape[1] == MEM
    assert S % PAIR == 0 and S // PAIR >= 4 and D % LANE == 0 and F % LANE == 0
    KD, NF = D // LANE, F // LANE
    NSEG = S // SEG

    def split(w):
        return w.reshape(D // 16, 16, H // 2, 2, Dh)

    any_spec = pl.BlockSpec(memory_space=pl.ANY)
    out = pl.pallas_call(
        functools.partial(_kernel, S=S, D=D, H=H, F=F),
        out_shape=jax.ShapeDtypeStruct((S, D), A_x.dtype),
        in_specs=[any_spec] * 11,
        out_specs=any_spec,
        scratch_shapes=[
            pltpu.VMEM((1, D), BF16),
            pltpu.VMEM((MEM, D), BF16),
            pltpu.VMEM((NSEG, SEG, D), BF16),
            pltpu.VMEM((NSEG, 8, D), BF16),
            pltpu.VMEM((KD, NSEG * 8, LANE), F32),
            pltpu.VMEM((KD, NSEG * 4, LANE), U32),
            pltpu.VMEM((4, NSEG * 8, 2 * LANE), F32),
            pltpu.VMEM((3, H // 2, 2, NSEG * 4, LANE), U32),
            pltpu.VMEM((H // 2, D // 16, 16, LANE), U32),
            pltpu.VMEM((H // 2, D // 16, 16, LANE), U32),
            pltpu.VMEM((H // 2, D // 16, 16, LANE), U32),
            pltpu.VMEM((H * Dh // 2, D + LANE), U32),
            pltpu.VMEM((D // 2, F + LANE), U32),
            pltpu.VMEM((D // 2, F + LANE), U32),
            pltpu.VMEM((F // 2, D + LANE), U32),
            pltpu.VMEM((4, 2, D // 2, D // 4), U32),
            pltpu.VMEM((D // 2, 4 * D), U32),
            pltpu.VMEM((6 * KD, 8, LANE), F32),
            pltpu.VMEM((2, KD, 8, LANE), F32),
            pltpu.VMEM((2, KD, 16, LANE), U32),
            pltpu.VMEM((H, 8, LANE), F32),
            pltpu.VMEM((H, 16, LANE), U32),
            pltpu.VMEM((H, 24, LANE), U32),
            pltpu.VMEM((KD, 48, LANE), F32),
            pltpu.VMEM((KD, 24, LANE), F32),
            pltpu.VMEM((2, PAIR, D), F32),
            pltpu.VMEM((KD, PAIR // 2, LANE), U32),
            pltpu.VMEM((NF, PAIR // 2, LANE), U32),
            pltpu.VMEM((3, PAIR, D), BF16),
            pltpu.SemaphoreType.DMA((4,)),
            pltpu.SemaphoreType.DMA((5,)),
            pltpu.SemaphoreType.DMA((3 * H // 2,)),
            pltpu.SemaphoreType.DMA((4,)),
            pltpu.SemaphoreType.DMA((3,)),
        ],
        compiler_params=pltpu.CompilerParams(
            vmem_limit_bytes=110 * 1024 * 1024,
            disable_bounds_checks=True,
            disable_semaphore_checks=True),
        name="rmt_block",
    )(A_x.reshape(NSEG, SEG, D), A_mem0.reshape(MEM, D), split(A_Wq), split(A_Wk),
      split(A_Wv), A_Wo.reshape(H * Dh, D), B_w1, B_w3, B_w2, c, w_mod)
    return out.reshape(B, S, D)
```

```python
import functools

import jax
import jax.numpy as jnp
from jax import lax
import jax.experimental.pallas as pl
import jax.experimental.pallas.tpu as pltpu

F32 = jnp.float32
BF16 = jnp.bfloat16
U32 = jnp.uint32

LANE = 128
SEG = 32
MEM = 8
PAIR = 2 * SEG
EPS = 1e-5

LS, LP = 1, 3
TAIL = 8
WO_AT = (2, 4, 6)


def _dot(a, b):
    return jnp.dot(a, b, preferred_element_type=F32)


def _cat_lanes(ref, n):
    return jnp.concatenate([ref[k] for k in range(n)], axis=1)


def _layernorm(x):
    m = jnp.mean(x, axis=-1, keepdims=True)
    xc = x - m
    v = jnp.mean(xc * xc, axis=-1, keepdims=True)
    return xc * lax.rsqrt(v + EPS)


def _silu(x):
    hx = 0.5 * x
    return hx + hx * jnp.tanh(hx)


def _recip(x):
    r = pl.reciprocal(x, approx=True)
    return r * (2.0 - x * r)


def _pk(x):
    return pltpu.bitcast(x.astype(BF16), U32)


def _unpk(x):
    return pltpu.bitcast(x, BF16)


def _cat_pk(ref, ks):
    return jnp.concatenate([_unpk(ref[k]) for k in ks], axis=1)


def _kernel(x_hbm, mem0_hbm, wq_hbm, wk_hbm, wv_hbm, wo_hbm, w1_hbm, w3_hbm,
            w2_hbm, c_hbm, wmod_hbm, out_hbm,
            c_v, mem0_v, x_v, xpre_v, xn_v, hpre_v, acc0_v, pre_v,
            wq_v, wk_v, wv_v, wo_v, w1_v, w3_v, w2_v, wme_v, wml_v,
            mod_v, hs_v, lhs_v, so_v, oa_v, ob_v, acc_v, ya_v,
            x1_v, h2_v, act_v, stage_v,
            sem_x, sem_mod, sem_qkv, sem_w, sem_out,
            *, S, D, H, F):
    KD = D // LANE
    NF = F // LANE
    NP = S // PAIR
    NSEG = S // SEG
    NJ = H // 2
    L = SEG + MEM
    scale = float(LANE) ** -0.5
    w_hbm = (wq_hbm, wk_hbm, wv_hbm)
    w_v = (wq_v, wk_v, wv_v)

    def blk(j):
        return slice(j * LANE, (j + 1) * LANE)

    NCH = 4
    CK = KD // NCH

    def early_mod(ch):
        return [pltpu.make_async_copy(
            wmod_hbm.bitcast(U32).at[:, pl.ds(
                pl.multiple_of(t * D + ch * (CK * LANE), LANE), CK * LANE)],
            wme_v.at[ch, t], sem_mod.at[ch]) for t in range(2)]

    late_mod = pltpu.make_async_copy(
        wmod_hbm.bitcast(U32).at[:, pl.ds(2 * D, 4 * D)], wml_v,
        sem_mod.at[NCH])

    def unit_copy(j, w):
        return pltpu.make_async_copy(
            w_hbm[w].bitcast(U32).at[:, :, j, 0, :],
            w_v[w].at[j], sem_qkv.at[3 * j + w])

    def start_unit(j, w):
        unit_copy(j, w).start()

    def wait_unit(j, w):
        unit_copy(j, w).wait()

    def w_copy(src, dst, k):
        return pltpu.make_async_copy(
            src.bitcast(U32), dst.at[:, pl.ds(0, src.shape[1])], sem_w.at[k])

    wo_copy = w_copy(wo_hbm, wo_v, 0)
    ffn_copies = [w_copy(w1_hbm, w1_v, 1), w_copy(w3_hbm, w3_v, 2),
                  w_copy(w2_hbm, w2_v, 3)]
    c_copy = pltpu.make_async_copy(c_hbm, c_v, sem_x.at[2])
    mem0_copy = pltpu.make_async_copy(mem0_hbm, mem0_v, sem_x.at[3])
    xpre_copy = pltpu.make_async_copy(
        x_hbm.at[:, pl.ds(0, 8), :], xpre_v, sem_x.at[0])
    x_copy = pltpu.make_async_copy(x_hbm, x_v, sem_x.at[1])

    def out_copy(i, slot):
        return pltpu.make_async_copy(
            stage_v.at[slot], out_hbm.at[pl.ds(i * PAIR, PAIR), :],
            sem_out.at[slot])

    first_units = ((0, 0), (0, 1), (0, 2), (1, 0))
    xpre_copy.start()
    c_copy.start()
    for j, w in first_units:
        start_unit(j, w)
    for ch in range(NCH):
        for cp in early_mod(ch):
            cp.start()
    for j in range(NJ):
        for w in range(3):
            if (j, w) not in first_units:
                start_unit(j, w)
    mem0_copy.start()
    x1_v[1] = jnp.zeros((PAIR, D), F32)

    xpre_copy.wait()

    def ln_pre(b, carry):
        x = xpre_v[pl.ds(b * 8, 8)].astype(F32).reshape(64, D)
        xn = _layernorm(x)
        r0 = pl.multiple_of(b * 64, 64)
        for k in range(KD):
            xn_v[k, pl.ds(r0, 64), :] = xn[:, blk(k)]
        for u in range(len(first_units)):
            acc0_v[u, pl.ds(r0, 64), :] = jnp.zeros((64, 2 * LANE), F32)
        return carry

    lax.fori_loop(0, NSEG // 8, ln_pre, 0)

    def relayout(j, w):
        for r in range(0, D // 16, 8):
            a = w_v[w][j, r:r + 8, pl.ds(0, 8, stride=2), :]
            b = w_v[w][j, r:r + 8, pl.ds(1, 8, stride=2), :]
            w_v[w][j, r:r + 8, 0:8, :] = (a & U32(0xFFFF)) | (b << 16)
            w_v[w][j, r:r + 8, 8:16, :] = (a >> 16) | (b & U32(0xFFFF0000))

    def w_head(w, j, p, k0=0, nk=KD):
        t = w_v[w][j, pl.ds(k0 * 8, nk * 8), 8 * p:8 * p + 8, :]
        return _unpk(t.reshape(nk * LANE // 2, LANE))

    c_copy.wait()
    for j, w in first_units:
        wait_unit(j, w)
    wo_copy.start()
    x_copy.start()
    late_mod.start()
    for cp in ffn_copies:
        cp.start()
    for j, w in first_units:
        relayout(j, w)

    c = c_v[...].astype(F32)
    sc = _silu(c).astype(BF16)
    sc = jnp.broadcast_to(sc, (16, D))

    def mod_row(k):
        return jnp.concatenate([mod_blk(k, j) for j in range(KD)], axis=1)

    def mod_blk(k, j):
        return mod_v[k * KD + j, 0:1, :]

    def late_mod_col(j):
        r = _dot(sc, _unpk(wml_v[:, blk(j - 2 * KD)]))[0:8]
        if j // KD == 4:
            r = r + 1.0
        mod_v[j] = r

    def chunk_body(ch, carry):
        for cp in early_mod(ch):
            cp.wait()
        k0 = ch * CK
        for kk in range(CK):
            sa = _dot(sc, _unpk(wme_v[ch, 0, :, blk(kk)]))[0:8]
            ca = _dot(sc, _unpk(wme_v[ch, 1, :, blk(kk)]))[0:8] + 1.0
            mod_v[k0 + kk] = sa
            mod_v[KD + k0 + kk] = ca
            for r in range(0, NSEG * 8, 128):
                hpre_v[k0 + kk, r // 2:r // 2 + 64, :] = _pk(
                    xn_v[k0 + kk, r:r + 128, :] * ca[0:1] + sa[0:1])
        for u, (j, w) in enumerate(first_units):
            hp = jnp.concatenate(
                [_unpk(hpre_v[k0 + kk]) for kk in range(CK)], axis=1)
            wt = jnp.concatenate(
                [w_head(w, j, p, k0, CK) for p in range(2)], axis=1)
            acc = acc0_v[u] + _dot(hp, wt)
            acc0_v[u] = acc
            for p in range(2):
                pre_v[w, j, p] = _pk(acc[:, blk(p)])
        return carry

    lax.fori_loop(0, NCH, chunk_body, 0)

    def pre_dot(j, w, p):
        hp = _cat_pk(hpre_v, range(KD))
        pre_v[w, j, p] = _pk(_dot(hp, w_head(w, j, p)))

    wait_unit(1, 1)
    relayout(1, 1)

    def pre_body(j, carry):
        wait_unit(j, 2)
        wait_unit(j + 1, 0)
        wait_unit(j + 1, 1)

        for (dj, dw), (rj, rw) in (((j, 1), (j, 2)), ((j, 2), (j + 1, 0)),
                                   ((j + 1, 0), (j + 1, 1))):
            pre_dot(dj, dw, 0)
            relayout(rj, rw)
            pre_dot(dj, dw, 1)
        return carry

    lax.fori_loop(1, NJ - 1, pre_body, 0)

    def ln1(seg, sg):
        x = x_v[seg].astype(F32)[8:SEG]
        h = _layernorm(x) * mod_row(1) + mod_row(0)
        for k in range(KD):
            lhs_v[sg, k, 0:8, :] = _pk(h[0:16, blk(k)])
            hs_v[sg, k] = h[16:24, blk(k)]

    L2 = 2 * L
    rr = lax.broadcasted_iota(jnp.int32, (L2, L2), 0)
    cc = lax.broadcasted_iota(jnp.int32, (L2, L2), 1)
    same = (rr >= L) == (cc >= L)
    rr = jnp.where(rr >= L, rr - L, rr)
    cc = jnp.where(cc >= L, cc - L, cc)
    mask = same & ((rr >= SEG) | (cc >= SEG) | (cc <= rr))
    fill_val = jnp.where(same, -1000000000.0, -jnp.inf).astype(F32)

    def scores(q, k):
        s = lax.dot_general(q, k, (((1,), (1,)), ((), ())),
                            preferred_element_type=F32)
        s = jnp.where(mask, s * scale, fill_val)
        m = jnp.max(s, axis=-1, keepdims=True)
        e = jnp.exp(s - m)
        p = e * _recip(jnp.sum(e, axis=-1, keepdims=True))
        return p.astype(BF16)

    def ln2(xs):
        h = _layernorm(x1_v[xs]) * mod_row(4) + mod_row(3)
        for k in range(KD):
            h2_v[k] = _pk(h[:, blk(k)])

    def up(f):
        h2 = _cat_pk(h2_v, range(KD))
        g = _dot(h2, _unpk(w1_v[:, blk(f)]))
        u = _dot(h2, _unpk(w3_v[:, blk(f)]))
        act_v[f] = _pk(_silu(g) * u)

    def down(xs, j, slot=None):
        a = _cat_pk(act_v, range(NF))
        y = _dot(a, _unpk(w2_v[:, blk(j)]))
        stage_v[xs if slot is None else slot, :, blk(j)] = (
            x1_v[xs, :, blk(j)] + mod_blk(5, j) * y).astype(BF16)


    def segment(i, sg, fill, finish):
        o_v = ob_v if sg else oa_v
        prow = pl.multiple_of(i * 8, 8)
        qk, vs, ps = {}, {}, {}

        def proj(g):
            r = []
            for w in range(3):
                parts = []
                for p in range(2):
                    lhs = _cat_pk(lhs_v.at[sg], range(KD))
                    pre = _unpk(pre_v[w, g, p, pl.ds(prow, 8), :]).astype(F32)
                    parts += [pre[8 * sg:8 * sg + 8],
                              _dot(lhs, w_head(w, g, p))]
                r.append(jnp.concatenate(parts, axis=0).astype(BF16))
            qk[g] = r[0:2]
            vs[g] = r[2]

        def pv(g):
            o2 = _dot(ps.pop(g), vs.pop(g))
            for p in range(2):
                h = 2 * g + p
                o = o2[p * L:(p + 1) * L]
                if sg == 0:
                    o_v[h] = _pk(jnp.concatenate([o[0:24], o[SEG:L]], axis=0))
                    so_v[h] = o[24:SEG]
                else:
                    o_v[h] = _pk(jnp.concatenate([so_v[h], o], axis=0))

        def wo_part(hs, j):
            lo, hi = hs[0] * (LANE // 2), (hs[-1] + 1) * (LANE // 2)
            return _dot(_cat_pk(o_v, hs), _unpk(wo_v[lo:hi, blk(j)]))

        rows = L + 8 if sg else SEG
        head_hs = list(range(H - TAIL))
        tail_hs = list(range(H - TAIL, H))
        cuts = (0,) + WO_AT
        wo_at = {NJ + t: range(cuts[t], cuts[t + 1]) for t in range(LP)}
        for g in range(NJ + LP):
            if g < NJ:
                proj(g)
            for j in wo_at.get(g, ()):
                acc_v[j, 0:rows, :] = wo_part(head_hs, j)
            if LS <= g < NJ + LS:
                ps[g - LS] = scores(*qk.pop(g - LS))
            if g >= LP:
                pv(g - LP)
            for fn in fill.get(g, ()):
                fn()
        for j in range(WO_AT[-1], KD):
            acc_v[j, 0:rows, :] = wo_part(head_hs, j)
        for j in range(KD):
            finish(j, acc_v[j, 0:rows, :] + wo_part(tail_hs, j))
        for fn in fill.get(NJ + LP, ()):
            fn()

    def attn_pair(i, fill_a, fill_b):
        xs = i % 2

        def finish_a(j, y):
            ya_v[j] = y[0:24]
            lhs_v[1, j, 8:16, :] = _pk(
                jnp.concatenate([hs_v[1, j], y[24:SEG]], axis=0))

        def finish_b(j, y):
            att = jnp.concatenate([ya_v[j], y[0:L]], axis=0)
            x = x_v[pl.ds(2 * i, 2), :, blk(j)].astype(F32).reshape(PAIR, LANE)
            x1_v[xs, :, blk(j)] = x + mod_blk(2, j) * att
            lhs_v[0, j, 8:16, :] = _pk(
                jnp.concatenate([hs_v[0, j], y[L:L + 8]], axis=0))

        segment(i, 0, fill_a, finish_a)
        segment(i, 1, fill_b, finish_b)

    P = functools.partial
    NU0 = 2

    wait_unit(NJ - 1, 2)
    x_copy.wait()
    late_mod.wait()
    mem0_copy.wait()
    wo_copy.wait()
    late = iter(range(2 * KD, 6 * KD))
    for n, (w, p) in enumerate(((1, 0), (1, 1), (2, 0), (2, 1))):
        for m in range(0, NSEG * 4, 32):
            hp = jnp.concatenate(
                [_unpk(hpre_v[k, m:m + 32, :]) for k in range(KD)], axis=1)
            pre_v[w, NJ - 1, p, m:m + 32, :] = _pk(
                _dot(hp, w_head(w, NJ - 1, p)))
            late_mod_col(next(late))
        if n == 0:
            relayout(NJ - 1, 2)
            ln1(0, 0)
            mem0 = mem0_v[...].astype(F32)
            for k in range(KD):
                lhs_v[0, k, 8:16, :] = _pk(jnp.concatenate(
                    [hs_v[0, k], mem0[:, blk(k)]], axis=0))

    def head_body(i, carry):
        attn_pair(i, {2: [P(ln1, 2 * i + 1, 1)]},
                  {2: [P(ln2, 1 - i)], 8: [P(ln1, 2 * i + 2, 0)]})
        return carry

    lax.fori_loop(0, 2, head_body, 0)
    for cp in ffn_copies:
        cp.wait()
    for f in range(NU0):
        up(f)

    def body(i, carry):
        slot = i % 2

        @pl.when(i >= 4)
        def _():
            out_copy(i - 4, slot).wait()

        fill_a, fill_b = {}, {}
        for f in range(NU0, NF):
            fill_a.setdefault((f - NU0) * 16 // (NF - NU0), []).append(P(up, f))
        fill_a[NJ + LP] = [P(down, slot, 0)]
        for j in range(1, KD):
            fill_b.setdefault(2 * j - 1, []).append(P(down, slot, j))
        fill_b.setdefault(2, []).append(P(ln2, 1 - slot))
        fill_a.setdefault(2, []).append(P(ln1, 2 * i + 1, 1))
        fill_b.setdefault(8, []).append(
            P(ln1, jnp.minimum(2 * i + 2, NSEG - 1), 0))
        fill_b[NJ + LP] = [P(up, f) for f in range(NU0)]
        attn_pair(i, fill_a, fill_b)
        out_copy(i - 2, slot).start()
        return carry

    lax.fori_loop(2, NP, body, 0)

    s0, s1 = NP % 2, (NP + 1) % 2
    out_copy(NP - 4, s0).wait()
    for f in range(NU0, NF):
        up(f)
    ln2(s1)
    for j in range(KD):
        down(s0, j)
    for f in range(NF):
        up(f)
    for j in range(KD):
        down(s1, j, 2)
    out_copy(NP - 2, s0).start()
    out_copy(NP - 1, 2).start()
    out_copy(NP - 3, s1).wait()
    out_copy(NP - 2, s0).wait()
    out_copy(NP - 1, 2).wait()


@functools.partial(jax.jit, static_argnames=("A_seg_len",))
def pallas_adaLN_cond__memory_aug_recurrent_mem_tr__glu_gated_swiglu__prompt_kernel(
    A_x: jax.Array,
    A_mem0: jax.Array,
    A_Wq: jax.Array,
    A_Wk: jax.Array,
    A_Wv: jax.Array,
    A_Wo: jax.Array,
    A_seg_len,
    B_x: jax.Array,
    B_w1: jax.Array,
    B_w3: jax.Array,
    B_w2: jax.Array,
    c: jax.Array,
    w_mod: jax.Array,
):
    B, S, D = A_x.shape
    H, Dh = A_Wq.shape[1], A_Wq.shape[2]
    F = B_w1.shape[1]
    assert B == 1 and Dh == LANE and A_seg_len == SEG and A_mem0.shape[1] == MEM
    assert S % PAIR == 0 and S // PAIR >= 4 and D % LANE == 0 and F % LANE == 0
    KD, NF = D // LANE, F // LANE
    NSEG = S // SEG

    def split(w):
        return w.reshape(D // 16, 16, H // 2, 2, Dh)

    any_spec = pl.BlockSpec(memory_space=pl.ANY)
    out = pl.pallas_call(
        functools.partial(_kernel, S=S, D=D, H=H, F=F),
        out_shape=jax.ShapeDtypeStruct((S, D), A_x.dtype),
        in_specs=[any_spec] * 11,
        out_specs=any_spec,
        scratch_shapes=[
            pltpu.VMEM((1, D), BF16),
            pltpu.VMEM((MEM, D), BF16),
            pltpu.VMEM((NSEG, SEG, D), BF16),
            pltpu.VMEM((NSEG, 8, D), BF16),
            pltpu.VMEM((KD, NSEG * 8, LANE), F32),
            pltpu.VMEM((KD, NSEG * 4, LANE), U32),
            pltpu.VMEM((4, NSEG * 8, 2 * LANE), F32),
            pltpu.VMEM((3, H // 2, 2, NSEG * 4, LANE), U32),
            pltpu.VMEM((H // 2, D // 16, 16, LANE), U32),
            pltpu.VMEM((H // 2, D // 16, 16, LANE), U32),
            pltpu.VMEM((H // 2, D // 16, 16, LANE), U32),
            pltpu.VMEM((H * Dh // 2, D + LANE), U32),
            pltpu.VMEM((D // 2, F + LANE), U32),
            pltpu.VMEM((D // 2, F + LANE), U32),
            pltpu.VMEM((F // 2, D + LANE), U32),
            pltpu.VMEM((4, 2, D // 2, D // 4), U32),
            pltpu.VMEM((D // 2, 4 * D), U32),
            pltpu.VMEM((6 * KD, 8, LANE), F32),
            pltpu.VMEM((2, KD, 8, LANE), F32),
            pltpu.VMEM((2, KD, 16, LANE), U32),
            pltpu.VMEM((H, 8, LANE), F32),
            pltpu.VMEM((H, 16, LANE), U32),
            pltpu.VMEM((H, 24, LANE), U32),
            pltpu.VMEM((KD, 48, LANE), F32),
            pltpu.VMEM((KD, 24, LANE), F32),
            pltpu.VMEM((2, PAIR, D), F32),
            pltpu.VMEM((KD, PAIR // 2, LANE), U32),
            pltpu.VMEM((NF, PAIR // 2, LANE), U32),
            pltpu.VMEM((3, PAIR, D), BF16),
            pltpu.SemaphoreType.DMA((4,)),
            pltpu.SemaphoreType.DMA((5,)),
            pltpu.SemaphoreType.DMA((3 * H // 2,)),
            pltpu.SemaphoreType.DMA((4,)),
            pltpu.SemaphoreType.DMA((3,)),
        ],
        compiler_params=pltpu.CompilerParams(
            vmem_limit_bytes=110 * 1024 * 1024,
            disable_bounds_checks=True,
            disable_semaphore_checks=True),
        name="rmt_block",
    )(A_x.reshape(NSEG, SEG, D), A_mem0.reshape(MEM, D), split(A_Wq), split(A_Wk),
      split(A_Wv), A_Wo.reshape(H * Dh, D), B_w1, B_w3, B_w2, c, w_mod)
    return out.reshape(B, S, D)
```

```python
import functools

import jax
import jax.numpy as jnp
from jax import lax
import jax.experimental.pallas as pl
import jax.experimental.pallas.tpu as pltpu

F32 = jnp.float32
BF16 = jnp.bfloat16
U32 = jnp.uint32

LANE = 128
SEG = 32
MEM = 8
PAIR = 2 * SEG
EPS = 1e-5

LS, LP = 1, 3
TAIL = 8
WO_AT = (2, 4, 6)


def _dot(a, b):
    return jnp.dot(a, b, preferred_element_type=F32)


def _cat_lanes(ref, n):
    return jnp.concatenate([ref[k] for k in range(n)], axis=1)


def _layernorm(x):
    m = jnp.mean(x, axis=-1, keepdims=True)
    xc = x - m
    v = jnp.mean(xc * xc, axis=-1, keepdims=True)
    return xc * lax.rsqrt(v + EPS)


def _silu(x):
    hx = 0.5 * x
    return hx + hx * jnp.tanh(hx)


def _recip(x):
    r = pl.reciprocal(x, approx=True)
    return r * (2.0 - x * r)


def _pk(x):
    return pltpu.bitcast(x.astype(BF16), U32)


def _unpk(x):
    return pltpu.bitcast(x, BF16)


def _cat_pk(ref, ks):
    return jnp.concatenate([_unpk(ref[k]) for k in ks], axis=1)


def _kernel(x_hbm, mem0_hbm, wq_hbm, wk_hbm, wv_hbm, wo_hbm, w1_hbm, w3_hbm,
            w2_hbm, c_hbm, wmod_hbm, out_hbm,
            c_v, mem0_v, x_v, xpre_v, xn_v, hpre_v, acc0_v, pre_v,
            wq_v, wk_v, wv_v, wo_v, w1_v, w3_v, w2_v, wme_v, wml_v,
            mod_v, hs_v, lhs_v, so_v, oa_v, ob_v, acc_v, ya_v,
            x1_v, h2_v, act_v, yh_v, stage_v,
            sem_x, sem_mod, sem_qkv, sem_w, sem_out,
            *, S, D, H, F):
    KD = D // LANE
    NF = F // LANE
    NP = S // PAIR
    NSEG = S // SEG
    NJ = H // 2
    L = SEG + MEM
    scale = float(LANE) ** -0.5
    w_hbm = (wq_hbm, wk_hbm, wv_hbm)
    w_v = (wq_v, wk_v, wv_v)

    def blk(j):
        return slice(j * LANE, (j + 1) * LANE)

    NCH = 4
    CK = KD // NCH

    def early_mod(ch):
        return [pltpu.make_async_copy(
            wmod_hbm.bitcast(U32).at[:, pl.ds(
                pl.multiple_of(t * D + ch * (CK * LANE), LANE), CK * LANE)],
            wme_v.at[ch, t], sem_mod.at[ch]) for t in range(2)]

    late_mod = [pltpu.make_async_copy(
        wmod_hbm.bitcast(U32).at[:, pl.ds((2 + 2 * t) * D, 2 * D)],
        wml_v.at[t], sem_mod.at[NCH]) for t in range(2)]

    def unit_copy(j, w):
        return pltpu.make_async_copy(
            w_hbm[w].bitcast(U32).at[:, :, j, 0, :],
            w_v[w].at[j], sem_qkv.at[3 * j + w])

    def start_unit(j, w):
        unit_copy(j, w).start()

    def wait_unit(j, w):
        unit_copy(j, w).wait()

    def w_copy(src, dst, k):
        return pltpu.make_async_copy(
            src.bitcast(U32), dst.at[:, pl.ds(0, src.shape[1])], sem_w.at[k])

    wo_copy = w_copy(wo_hbm, wo_v, 0)
    FH = F // 2
    NH = NF // 2
    ffn_copies = []
    for hf in range(2):
        for n, (src, dst) in enumerate(((w1_hbm, w1_v), (w3_hbm, w3_v))):
            ffn_copies.append(pltpu.make_async_copy(
                src.bitcast(U32).at[:, pl.ds(hf * FH, FH)],
                dst.at[hf, :, pl.ds(0, FH)], sem_w.at[1]))
    for hf in range(2):
        ffn_copies.append(pltpu.make_async_copy(
            w2_hbm.bitcast(U32).at[pl.ds(hf * FH // 2, FH // 2), :],
            w2_v.at[hf, :, pl.ds(0, D)], sem_w.at[1]))
    c_copy = pltpu.make_async_copy(c_hbm, c_v, sem_x.at[2])
    mem0_copy = pltpu.make_async_copy(mem0_hbm, mem0_v, sem_x.at[3])
    xpre_copy = pltpu.make_async_copy(
        x_hbm.at[:, pl.ds(0, 8), :], xpre_v, sem_x.at[0])
    x_copy = pltpu.make_async_copy(x_hbm, x_v, sem_x.at[1])

    def out_copy(i, slot):
        return pltpu.make_async_copy(
            stage_v.at[slot], out_hbm.at[pl.ds(i * PAIR, PAIR), :],
            sem_out.at[slot])

    first_units = ((0, 0), (0, 1), (0, 2), (1, 0))
    xpre_copy.start()
    c_copy.start()
    for j, w in first_units:
        start_unit(j, w)
    for ch in range(NCH):
        for cp in early_mod(ch):
            cp.start()
    for j in range(NJ):
        for w in range(3):
            if (j, w) not in first_units:
                start_unit(j, w)
    mem0_copy.start()
    x1_v[1] = jnp.zeros((PAIR, D), F32)

    xpre_copy.wait()

    def ln_pre(b, carry):
        x = xpre_v[pl.ds(b * 8, 8)].astype(F32).reshape(64, D)
        xn = _layernorm(x)
        r0 = pl.multiple_of(b * 64, 64)
        for k in range(KD):
            xn_v[k, pl.ds(r0, 64), :] = xn[:, blk(k)]
        for u in range(len(first_units)):
            acc0_v[u, pl.ds(r0, 64), :] = jnp.zeros((64, 2 * LANE), F32)
        return carry

    lax.fori_loop(0, NSEG // 8, ln_pre, 0)

    def relayout_rows(j, w, r):
        rows = pl.ds(r, 8)
        a = w_v[w][j, rows, pl.ds(0, 8, stride=2), :]
        b = w_v[w][j, rows, pl.ds(1, 8, stride=2), :]
        w_v[w][j, rows, 0:8, :] = (a & U32(0xFFFF)) | (b << 16)
        w_v[w][j, rows, 8:16, :] = (a >> 16) | (b & U32(0xFFFF0000))

    def relayout(j, w):
        for k in range(KD):
            relayout_rows(j, w, k * 8)

    def relayout_loop(units):
        def step(k, carry):
            for j, w in units:
                relayout_rows(j, w, k * 8)
            return carry

        lax.fori_loop(0, KD, step, 0)

    def w_head(w, j, p, k0=0, nk=KD):
        p8 = 8 * p if isinstance(p, int) else pl.multiple_of(8 * p, 8)
        t = w_v[w][j, pl.ds(k0 * 8, nk * 8), pl.ds(p8, 8), :]
        return _unpk(t.reshape(nk * LANE // 2, LANE))

    c_copy.wait()
    for j, w in first_units:
        wait_unit(j, w)
    wo_copy.start()
    x_copy.start()
    for cp in late_mod:
        cp.start()
    for cp in ffn_copies:
        cp.start()
    relayout_loop(first_units)

    c = c_v[...].astype(F32)
    sc = _silu(c).astype(BF16)
    sc = jnp.broadcast_to(sc, (16, D))

    def mod_row(k):
        return jnp.concatenate([mod_blk(k, j) for j in range(KD)], axis=1)

    def mod_blk(k, j):
        return mod_v[k * KD + j, 0:1, :]

    def chunk_body(ch, carry):
        for cp in early_mod(ch):
            cp.wait()
        k0 = ch * CK
        for kk in range(CK):
            sa = _dot(sc, _unpk(wme_v[ch, 0, :, blk(kk)]))[0:8]
            ca = _dot(sc, _unpk(wme_v[ch, 1, :, blk(kk)]))[0:8] + 1.0
            mod_v[k0 + kk] = sa
            mod_v[KD + k0 + kk] = ca
            for r in range(0, NSEG * 8, 128):
                hpre_v[k0 + kk, r // 2:r // 2 + 64, :] = _pk(
                    xn_v[k0 + kk, r:r + 128, :] * ca[0:1] + sa[0:1])
        for u, (j, w) in enumerate(first_units):
            hp = jnp.concatenate(
                [_unpk(hpre_v[k0 + kk]) for kk in range(CK)], axis=1)
            wt = jnp.concatenate(
                [w_head(w, j, p, k0, CK) for p in range(2)], axis=1)
            acc = acc0_v[u] + _dot(hp, wt)
            acc0_v[u] = acc
            for p in range(2):
                pre_v[w, j, p] = _pk(acc[:, blk(p)])
        return carry

    lax.fori_loop(0, NCH, chunk_body, 0)

    def pre_dot(j, w, p):
        hp = _cat_pk(hpre_v, range(KD))
        pre_v[w, j, p] = _pk(_dot(hp, w_head(w, j, p)))

    wait_unit(1, 1)
    relayout(1, 1)

    def pre_body(j, carry):
        wait_unit(j, 2)
        wait_unit(j + 1, 0)
        wait_unit(j + 1, 1)

        for (dj, dw), (rj, rw) in (((j, 1), (j, 2)), ((j, 2), (j + 1, 0)),
                                   ((j + 1, 0), (j + 1, 1))):
            pre_dot(dj, dw, 0)
            relayout(rj, rw)
            pre_dot(dj, dw, 1)
        return carry

    lax.fori_loop(1, NJ - 1, pre_body, 0)

    def ln1(seg, sg):
        x = x_v[seg].astype(F32)[8:SEG]
        h = _layernorm(x) * mod_row(1) + mod_row(0)
        for k in range(KD):
            lhs_v[sg, k, 0:8, :] = _pk(h[0:16, blk(k)])
            hs_v[sg, k] = h[16:24, blk(k)]

    L2 = 2 * L
    rr = lax.broadcasted_iota(jnp.int32, (L2, L2), 0)
    cc = lax.broadcasted_iota(jnp.int32, (L2, L2), 1)
    same = (rr >= L) == (cc >= L)
    rr = jnp.where(rr >= L, rr - L, rr)
    cc = jnp.where(cc >= L, cc - L, cc)
    mask = same & ((rr >= SEG) | (cc >= SEG) | (cc <= rr))
    fill_val = jnp.where(same, -1000000000.0, -jnp.inf).astype(F32)

    def scores(q, k):
        s = lax.dot_general(q, k, (((1,), (1,)), ((), ())),
                            preferred_element_type=F32)
        s = jnp.where(mask, s * scale, fill_val)
        m = jnp.max(s, axis=-1, keepdims=True)
        e = jnp.exp(s - m)
        p = e * _recip(jnp.sum(e, axis=-1, keepdims=True))
        return p.astype(BF16)

    def ln2(xs, hs=0):
        h = _layernorm(x1_v[xs]) * mod_row(4) + mod_row(3)
        for k in range(KD):
            h2_v[hs, k] = _pk(h[:, blk(k)])

    def up_half(hf, f, hs, dst):
        h2 = _cat_pk(h2_v.at[hs], range(KD))
        g = _dot(h2, _unpk(w1_v[hf, :, blk(f)]))
        u = _dot(h2, _unpk(w3_v[hf, :, blk(f)]))
        act_v[dst] = _pk(_silu(g) * u)

    def up(f):
        up_half(f // NH, f % NH, 0, f)

    def down(xs, j):
        a = _cat_pk(act_v, range(NF))
        w2 = jnp.concatenate(
            [_unpk(w2_v[hf, :, blk(j)]) for hf in range(2)], axis=0)
        stage_v[xs, :, blk(j)] = (
            x1_v[xs, :, blk(j)] + mod_blk(5, j) * _dot(a, w2)).astype(BF16)

    def segment(i, sg, fill, finish):
        o_v = ob_v if sg else oa_v
        prow = pl.multiple_of(i * 8, 8)
        qk, vs, ps = {}, {}, {}

        def proj(g):
            r = []
            for w in range(3):
                parts = []
                for p in range(2):
                    lhs = _cat_pk(lhs_v.at[sg], range(KD))
                    pre = _unpk(pre_v[w, g, p, pl.ds(prow, 8), :]).astype(F32)
                    parts += [pre[8 * sg:8 * sg + 8],
                              _dot(lhs, w_head(w, g, p))]
                r.append(jnp.concatenate(parts, axis=0).astype(BF16))
            qk[g] = r[0:2]
            vs[g] = r[2]

        def pv(g):
            o2 = _dot(ps.pop(g), vs.pop(g))
            for p in range(2):
                h = 2 * g + p
                o = o2[p * L:(p + 1) * L]
                if sg == 0:
                    o_v[h] = _pk(jnp.concatenate([o[0:24], o[SEG:L]], axis=0))
                    so_v[h] = o[24:SEG]
                else:
                    o_v[h] = _pk(jnp.concatenate([so_v[h], o], axis=0))

        def wo_part(hs, j):
            lo, hi = hs[0] * (LANE // 2), (hs[-1] + 1) * (LANE // 2)
            return _dot(_cat_pk(o_v, hs), _unpk(wo_v[lo:hi, blk(j)]))

        rows = L + 8 if sg else SEG
        head_hs = list(range(H - TAIL))
        tail_hs = list(range(H - TAIL, H))
        cuts = (0,) + WO_AT
        wo_at = {NJ + t: range(cuts[t], cuts[t + 1]) for t in range(LP)}
        for g in range(NJ + LP):
            if g < NJ:
                proj(g)
            for j in wo_at.get(g, ()):
                acc_v[j, 0:rows, :] = wo_part(head_hs, j)
            if LS <= g < NJ + LS:
                ps[g - LS] = scores(*qk.pop(g - LS))
            if g >= LP:
                pv(g - LP)
            for fn in fill.get(g, ()):
                fn()
        for j in range(WO_AT[-1], KD):
            acc_v[j, 0:rows, :] = wo_part(head_hs, j)
        for j in range(KD):
            finish(j, acc_v[j, 0:rows, :] + wo_part(tail_hs, j))
        for fn in fill.get(NJ + LP, ()):
            fn()

    def attn_pair(i, fill_a, fill_b):
        xs = i % 2

        def finish_a(j, y):
            ya_v[j] = y[0:24]
            lhs_v[1, j, 8:16, :] = _pk(
                jnp.concatenate([hs_v[1, j], y[24:SEG]], axis=0))

        def finish_b(j, y):
            att = jnp.concatenate([ya_v[j], y[0:L]], axis=0)
            x = x_v[pl.ds(2 * i, 2), :, blk(j)].astype(F32).reshape(PAIR, LANE)
            x1_v[xs, :, blk(j)] = x + mod_blk(2, j) * att
            lhs_v[0, j, 8:16, :] = _pk(
                jnp.concatenate([hs_v[0, j], y[L:L + 8]], axis=0))

        segment(i, 0, fill_a, finish_a)
        segment(i, 1, fill_b, finish_b)

    P = functools.partial
    NU0 = 2

    wait_unit(NJ - 1, 2)
    x_copy.wait()
    for cp in late_mod:
        cp.wait()
    mem0_copy.wait()
    wo_copy.wait()
    relayout(NJ - 1, 2)

    def last_body(p, carry):
        one = p.astype(F32)
        for n, w in enumerate((1, 2)):
            for m in range(KD):
                rows = slice(m * 32, (m + 1) * 32)
                hp = jnp.concatenate(
                    [_unpk(hpre_v[k, rows, :]) for k in range(KD)], axis=1)
                pre_v[w, NJ - 1, p, rows, :] = _pk(
                    _dot(hp, w_head(w, NJ - 1, p)))
                r = _dot(sc, _unpk(wml_v[p, :, blk(n * KD + m)]))[0:8]
                mod_v[(2 + n) * KD + m + 2 * KD * p] = r + one if n == 0 else r
            if n == 0:
                ln1(0, 0)
                mem0 = mem0_v[...].astype(F32)
                for k in range(KD):
                    lhs_v[0, k, 8:16, :] = _pk(jnp.concatenate(
                        [hs_v[0, k], mem0[:, blk(k)]], axis=0))
        return carry

    lax.fori_loop(0, 2, last_body, 0)

    def head_body(i, carry):
        attn_pair(i, {2: [P(ln1, 2 * i + 1, 1)]},
                  {2: [P(ln2, 1 - i)], 8: [P(ln1, 2 * i + 2, 0)]})
        return carry

    lax.fori_loop(0, 2, head_body, 0)
    for cp in ffn_copies:
        cp.wait()
    for f in range(NU0):
        up(f)

    def body(i, carry):
        slot = i % 2

        @pl.when(i >= 4)
        def _():
            out_copy(i - 4, slot).wait()

        fill_a, fill_b = {}, {}
        for f in range(NU0, NF):
            fill_a.setdefault((f - NU0) * 16 // (NF - NU0), []).append(P(up, f))
        fill_a[NJ + LP] = [P(down, slot, 0)]
        for j in range(1, KD):
            fill_b.setdefault(2 * j - 1, []).append(P(down, slot, j))
        fill_b.setdefault(2, []).append(P(ln2, 1 - slot))
        fill_a.setdefault(2, []).append(P(ln1, 2 * i + 1, 1))
        fill_b.setdefault(8, []).append(
            P(ln1, jnp.minimum(2 * i + 2, NSEG - 1), 0))
        fill_b[NJ + LP] = [P(up, f) for f in range(NU0)]
        attn_pair(i, fill_a, fill_b)
        out_copy(i - 2, slot).start()
        return carry

    lax.fori_loop(2, NP, body, 0)

    out_copy(NP - 4, NP % 2).wait()

    def tail_body(q, carry):
        t, hf = q // 2, q % 2
        xs = (NP + t) % 2

        @pl.when(q == 2)
        def _():
            out_copy(NP - 3, xs).wait()

        for f in range(NH):
            up_half(hf, f, t, f)
        ln2((NP + 1) % 2, 1)
        for j in range(KD):
            y = _dot(_cat_pk(act_v, range(NH)), _unpk(w2_v[hf, :, blk(j)]))
            y = y + jnp.where(hf == 1, yh_v[:, blk(j)], 0.0)
            yh_v[:, blk(j)] = y
            stage_v[xs, :, blk(j)] = (
                x1_v[xs, :, blk(j)] + mod_blk(5, j) * y).astype(BF16)

        @pl.when(hf == 1)
        def _():
            out_copy(NP - 2 + t, xs).start()

        return carry

    lax.fori_loop(0, 4, tail_body, 0)
    out_copy(NP - 2, NP % 2).wait()
    out_copy(NP - 1, (NP + 1) % 2).wait()


@functools.partial(jax.jit, static_argnames=("A_seg_len",))
def pallas_adaLN_cond__memory_aug_recurrent_mem_tr__glu_gated_swiglu__prompt_kernel(
    A_x: jax.Array,
    A_mem0: jax.Array,
    A_Wq: jax.Array,
    A_Wk: jax.Array,
    A_Wv: jax.Array,
    A_Wo: jax.Array,
    A_seg_len,
    B_x: jax.Array,
    B_w1: jax.Array,
    B_w3: jax.Array,
    B_w2: jax.Array,
    c: jax.Array,
    w_mod: jax.Array,
):
    B, S, D = A_x.shape
    H, Dh = A_Wq.shape[1], A_Wq.shape[2]
    F = B_w1.shape[1]
    assert B == 1 and Dh == LANE and A_seg_len == SEG and A_mem0.shape[1] == MEM
    assert S % PAIR == 0 and S // PAIR >= 4 and D % LANE == 0 and F % LANE == 0
    KD, NF = D // LANE, F // LANE
    NSEG = S // SEG

    def split(w):
        return w.reshape(D // 16, 16, H // 2, 2, Dh)

    any_spec = pl.BlockSpec(memory_space=pl.ANY)
    out = pl.pallas_call(
        functools.partial(_kernel, S=S, D=D, H=H, F=F),
        out_shape=jax.ShapeDtypeStruct((S, D), A_x.dtype),
        in_specs=[any_spec] * 11,
        out_specs=any_spec,
        scratch_shapes=[
            pltpu.VMEM((1, D), BF16),
            pltpu.VMEM((MEM, D), BF16),
            pltpu.VMEM((NSEG, SEG, D), BF16),
            pltpu.VMEM((NSEG, 8, D), BF16),
            pltpu.VMEM((KD, NSEG * 8, LANE), F32),
            pltpu.VMEM((KD, NSEG * 4, LANE), U32),
            pltpu.VMEM((4, NSEG * 8, 2 * LANE), F32),
            pltpu.VMEM((3, H // 2, 2, NSEG * 4, LANE), U32),
            pltpu.VMEM((H // 2, D // 16, 16, LANE), U32),
            pltpu.VMEM((H // 2, D // 16, 16, LANE), U32),
            pltpu.VMEM((H // 2, D // 16, 16, LANE), U32),
            pltpu.VMEM((H * Dh // 2, D + LANE), U32),
            pltpu.VMEM((2, D // 2, F // 2 + LANE), U32),
            pltpu.VMEM((2, D // 2, F // 2 + LANE), U32),
            pltpu.VMEM((2, F // 4, D + LANE), U32),
            pltpu.VMEM((4, 2, D // 2, D // 4), U32),
            pltpu.VMEM((2, D // 2, 2 * D), U32),
            pltpu.VMEM((6 * KD, 8, LANE), F32),
            pltpu.VMEM((2, KD, 8, LANE), F32),
            pltpu.VMEM((2, KD, 16, LANE), U32),
            pltpu.VMEM((H, 8, LANE), F32),
            pltpu.VMEM((H, 16, LANE), U32),
            pltpu.VMEM((H, 24, LANE), U32),
            pltpu.VMEM((KD, 48, LANE), F32),
            pltpu.VMEM((KD, 24, LANE), F32),
            pltpu.VMEM((2, PAIR, D), F32),
            pltpu.VMEM((2, KD, PAIR // 2, LANE), U32),
            pltpu.VMEM((NF, PAIR // 2, LANE), U32),
            pltpu.VMEM((PAIR, D), F32),
            pltpu.VMEM((2, PAIR, D), BF16),
            pltpu.SemaphoreType.DMA((4,)),
            pltpu.SemaphoreType.DMA((5,)),
            pltpu.SemaphoreType.DMA((3 * H // 2,)),
            pltpu.SemaphoreType.DMA((2,)),
            pltpu.SemaphoreType.DMA((2,)),
        ],
        compiler_params=pltpu.CompilerParams(
            vmem_limit_bytes=110 * 1024 * 1024,
            disable_bounds_checks=True,
            disable_semaphore_checks=True),
        name="rmt_block",
    )(A_x.reshape(NSEG, SEG, D), A_mem0.reshape(MEM, D), split(A_Wq), split(A_Wk),
      split(A_Wv), A_Wo.reshape(H * Dh, D), B_w1, B_w3, B_w2, c, w_mod)
    return out.reshape(B, S, D)
```

```python
import functools

import jax
import jax.numpy as jnp
from jax import lax
import jax.experimental.pallas as pl
import jax.experimental.pallas.tpu as pltpu

F32 = jnp.float32
BF16 = jnp.bfloat16
U32 = jnp.uint32

LANE = 128
SEG = 32
MEM = 8
PAIR = 2 * SEG
EPS = 1e-5

LS, LP = 1, 3
TAIL = 8
WO_AT = (2, 4, 6)
NU0 = 3


def _dot(a, b):
    return jnp.dot(a, b, preferred_element_type=F32)


def _layernorm(x):
    m = jnp.mean(x, axis=-1, keepdims=True)
    xc = x - m
    v = jnp.mean(xc * xc, axis=-1, keepdims=True)
    return xc * lax.rsqrt(v + EPS)


def _silu(x):
    hx = 0.5 * x
    return hx + hx * jnp.tanh(hx)


def _recip(x):
    r = pl.reciprocal(x, approx=True)
    return r * (2.0 - x * r)


def _pk(x):
    return pltpu.bitcast(x.astype(BF16), U32)


def _unpk(x):
    return pltpu.bitcast(x, BF16)


def _cat_pk(ref, ks):
    return jnp.concatenate([_unpk(ref[k]) for k in ks], axis=1)


def _kernel(x_hbm, mem0_hbm, wq_hbm, wk_hbm, wv_hbm, wo_hbm, w1_hbm, w3_hbm,
            w2_hbm, c_hbm, wmod_hbm, out_hbm,
            c_v, mem0_v, x_v, xpre_v, xn_v, hpre_v, acc0_v, pre_v,
            wq_v, wk_v, wv_v, wo_v, w1_v, w3_v, w2_v, wme_v, wml_v,
            mod_v, hs_v, lhs_v, so_v, oa_v, ob_v, acc_v, ya_v,
            x1_v, h2_v, act_v, yh_v, stage_v,
            sem_x, sem_mod, sem_qkv, sem_w, sem_out,
            *, S, D, H, F):
    KD = D // LANE
    NF = F // LANE
    NP = S // PAIR
    NSEG = S // SEG
    NJ = H // 2
    L = SEG + MEM
    scale = float(LANE) ** -0.5
    w_hbm = (wq_hbm, wk_hbm, wv_hbm)
    w_v = (wq_v, wk_v, wv_v)

    def blk(j):
        return slice(j * LANE, (j + 1) * LANE)

    NCH = 4
    CK = KD // NCH

    def early_mod(ch):
        return [pltpu.make_async_copy(
            wmod_hbm.bitcast(U32).at[:, pl.ds(
                pl.multiple_of(t * D + ch * (CK * LANE), LANE), CK * LANE)],
            wme_v.at[ch, t], sem_mod.at[ch]) for t in range(2)]

    late_mod = [pltpu.make_async_copy(
        wmod_hbm.bitcast(U32).at[:, pl.ds((2 + 2 * t) * D, 2 * D)],
        wml_v.at[t], sem_mod.at[NCH]) for t in range(2)]

    def unit_copy(j, w):
        return pltpu.make_async_copy(
            w_hbm[w].bitcast(U32).at[:, :, j, 0, :],
            w_v[w].at[j], sem_qkv.at[3 * j + w])

    def start_unit(j, w):
        unit_copy(j, w).start()

    def wait_unit(j, w):
        unit_copy(j, w).wait()

    wo_copy = pltpu.make_async_copy(
        wo_hbm.bitcast(U32), wo_v.at[:, pl.ds(0, D)], sem_w.at[0])
    FH = F // 2
    NH = NF // 2
    ffn_copies = []
    for hf in range(2):
        for src, dst in ((w1_hbm, w1_v), (w3_hbm, w3_v)):
            ffn_copies.append(pltpu.make_async_copy(
                src.bitcast(U32).at[:, pl.ds(hf * FH, FH)],
                dst.at[hf, :, pl.ds(0, FH)], sem_w.at[1]))
    for hf in range(2):
        ffn_copies.append(pltpu.make_async_copy(
            w2_hbm.bitcast(U32).at[pl.ds(hf * FH // 2, FH // 2), :],
            w2_v.at[hf, :, pl.ds(0, D)], sem_w.at[1]))
    c_copy = pltpu.make_async_copy(c_hbm, c_v, sem_x.at[2])
    mem0_copy = pltpu.make_async_copy(mem0_hbm, mem0_v, sem_x.at[3])
    xpre_copy = pltpu.make_async_copy(
        x_hbm.at[:, pl.ds(0, 8), :], xpre_v, sem_x.at[0])
    x_copy = pltpu.make_async_copy(x_hbm, x_v, sem_x.at[1])

    def out_copy(i, slot):
        return pltpu.make_async_copy(
            stage_v.at[slot], out_hbm.at[pl.ds(i * PAIR, PAIR), :],
            sem_out.at[slot])

    first_units = ((0, 0), (0, 1), (0, 2), (1, 0))
    xpre_copy.start()
    c_copy.start()
    for j, w in first_units:
        start_unit(j, w)
    for ch in range(NCH):
        for cp in early_mod(ch):
            cp.start()
    for j in range(NJ):
        for w in range(3):
            if (j, w) not in first_units:
                start_unit(j, w)
    mem0_copy.start()
    x1_v[1] = jnp.zeros((PAIR, D), F32)

    xpre_copy.wait()

    def ln_pre(b, carry):
        x = xpre_v[pl.ds(b * 8, 8)].astype(F32).reshape(64, D)
        xn = _layernorm(x)
        r0 = pl.multiple_of(b * 64, 64)
        for k in range(KD):
            xn_v[k, pl.ds(r0, 64), :] = xn[:, blk(k)]
        for u in range(len(first_units)):
            acc0_v[u, pl.ds(r0, 64), :] = jnp.zeros((64, 2 * LANE), F32)
        return carry

    lax.fori_loop(0, NSEG // 8, ln_pre, 0)

    def relayout_rows(j, w, r):
        rows = pl.ds(r, 8)
        a = w_v[w][j, rows, pl.ds(0, 8, stride=2), :]
        b = w_v[w][j, rows, pl.ds(1, 8, stride=2), :]
        w_v[w][j, rows, 0:8, :] = (a & U32(0xFFFF)) | (b << 16)
        w_v[w][j, rows, 8:16, :] = (a >> 16) | (b & U32(0xFFFF0000))

    def relayout(j, w):
        for k in range(KD):
            relayout_rows(j, w, k * 8)

    def relayout_loop(units):
        def step(k, carry):
            for j, w in units:
                relayout_rows(j, w, k * 8)
            return carry

        lax.fori_loop(0, KD, step, 0)

    def w_head(w, j, p, k0=0, nk=KD):
        p8 = 8 * p if isinstance(p, int) else pl.multiple_of(8 * p, 8)
        t = w_v[w][j, pl.ds(k0 * 8, nk * 8), pl.ds(p8, 8), :]
        return _unpk(t.reshape(nk * LANE // 2, LANE))

    c_copy.wait()
    for j, w in first_units:
        wait_unit(j, w)
    wo_copy.start()
    x_copy.start()
    for cp in late_mod:
        cp.start()
    for cp in ffn_copies:
        cp.start()
    relayout_loop(first_units)

    c = c_v[...].astype(F32)
    sc = _silu(c).astype(BF16)
    sc = jnp.broadcast_to(sc, (16, D))

    def mod_row(k):
        return jnp.concatenate([mod_blk(k, j) for j in range(KD)], axis=1)

    def mod_blk(k, j):
        return mod_v[k * KD + j, 0:1, :]

    def chunk_body(ch, carry):
        for cp in early_mod(ch):
            cp.wait()
        k0 = ch * CK
        for kk in range(CK):
            sa = _dot(sc, _unpk(wme_v[ch, 0, :, blk(kk)]))[0:8]
            ca = _dot(sc, _unpk(wme_v[ch, 1, :, blk(kk)]))[0:8] + 1.0
            mod_v[k0 + kk] = sa
            mod_v[KD + k0 + kk] = ca
            for r in range(0, NSEG * 8, 128):
                hpre_v[k0 + kk, r // 2:r // 2 + 64, :] = _pk(
                    xn_v[k0 + kk, r:r + 128, :] * ca[0:1] + sa[0:1])
        for u, (j, w) in enumerate(first_units):
            hp = jnp.concatenate(
                [_unpk(hpre_v[k0 + kk]) for kk in range(CK)], axis=1)
            wt = jnp.concatenate(
                [w_head(w, j, p, k0, CK) for p in range(2)], axis=1)
            acc = acc0_v[u] + _dot(hp, wt)
            acc0_v[u] = acc
            for p in range(2):
                pre_v[w, j, p] = _pk(acc[:, blk(p)])
        return carry

    lax.fori_loop(0, NCH, chunk_body, 0)

    def pre_dot(j, w, p):
        hp = _cat_pk(hpre_v, range(KD))
        pre_v[w, j, p] = _pk(_dot(hp, w_head(w, j, p)))

    wait_unit(1, 1)
    relayout(1, 1)

    def pre_body(j, carry):
        wait_unit(j, 2)
        wait_unit(j + 1, 0)
        wait_unit(j + 1, 1)

        for (dj, dw), (rj, rw) in (((j, 1), (j, 2)), ((j, 2), (j + 1, 0)),
                                   ((j + 1, 0), (j + 1, 1))):
            pre_dot(dj, dw, 0)
            relayout(rj, rw)
            pre_dot(dj, dw, 1)
        return carry

    lax.fori_loop(1, NJ - 1, pre_body, 0)

    def ln1(seg, sg):
        x = x_v[seg].astype(F32)[8:SEG]
        h = _layernorm(x) * mod_row(1) + mod_row(0)
        for k in range(KD):
            lhs_v[sg, k, 0:8, :] = _pk(h[0:16, blk(k)])
            hs_v[sg, k] = h[16:24, blk(k)]

    L2 = 2 * L
    rr = lax.broadcasted_iota(jnp.int32, (L2, L2), 0)
    cc = lax.broadcasted_iota(jnp.int32, (L2, L2), 1)
    same = (rr >= L) == (cc >= L)
    rr = jnp.where(rr >= L, rr - L, rr)
    cc = jnp.where(cc >= L, cc - L, cc)
    mask = same & ((rr >= SEG) | (cc >= SEG) | (cc <= rr))
    fill_val = jnp.where(same, -1000000000.0, -jnp.inf).astype(F32)

    def scores(q, k):
        s = lax.dot_general(q, k, (((1,), (1,)), ((), ())),
                            preferred_element_type=F32)
        s = jnp.where(mask, s * scale, fill_val)
        m = jnp.max(s, axis=-1, keepdims=True)
        e = jnp.exp(s - m)
        p = e * _recip(jnp.sum(e, axis=-1, keepdims=True))
        return p.astype(BF16)

    def ln2(xs, hs=0):
        h = _layernorm(x1_v[xs]) * mod_row(4) + mod_row(3)
        for k in range(KD):
            h2_v[hs, k] = _pk(h[:, blk(k)])

    def up_half(hf, f, hs, dst):
        h2 = _cat_pk(h2_v.at[hs], range(KD))
        g = _dot(h2, _unpk(w1_v[hf, :, blk(f)]))
        u = _dot(h2, _unpk(w3_v[hf, :, blk(f)]))
        act_v[dst] = _pk(_silu(g) * u)

    def up(f):
        up_half(f // NH, f % NH, 0, f)

    def down(xs, j, hf):
        a = _cat_pk(act_v, range(hf * NH, (hf + 1) * NH))
        y = _dot(a, _unpk(w2_v[hf, :, blk(j)]))
        if hf == 0:
            yh_v[:, blk(j)] = y
        else:
            y = y + yh_v[:, blk(j)]
            stage_v[xs, :, blk(j)] = (
                x1_v[xs, :, blk(j)] + mod_blk(5, j) * y).astype(BF16)

    def segment(i, sg, fill, finish):
        o_v = ob_v if sg else oa_v
        prow = pl.multiple_of(i * 8, 8)
        qk, vs, ps = {}, {}, {}

        def proj(g):
            r = []
            for w in range(3):
                parts = []
                for p in range(2):
                    lhs = _cat_pk(lhs_v.at[sg], range(KD))
                    pre = _unpk(pre_v[w, g, p, pl.ds(prow, 8), :]).astype(F32)
                    parts += [pre[8 * sg:8 * sg + 8],
                              _dot(lhs, w_head(w, g, p))]
                r.append(jnp.concatenate(parts, axis=0).astype(BF16))
            qk[g] = r[0:2]
            vs[g] = r[2]

        def pv(g):
            o2 = _dot(ps.pop(g), vs.pop(g))
            for p in range(2):
                h = 2 * g + p
                o = o2[p * L:(p + 1) * L]
                if sg == 0:
                    o_v[h] = _pk(jnp.concatenate([o[0:24], o[SEG:L]], axis=0))
                    so_v[h] = o[24:SEG]
                else:
                    o_v[h] = _pk(jnp.concatenate([so_v[h], o], axis=0))

        def wo_part(hs, j):
            lo, hi = hs[0] * (LANE // 2), (hs[-1] + 1) * (LANE // 2)
            return _dot(_cat_pk(o_v, hs), _unpk(wo_v[lo:hi, blk(j)]))

        rows = L + 8 if sg else SEG
        head_hs = list(range(H - TAIL))
        tail_hs = list(range(H - TAIL, H))
        cuts = (0,) + WO_AT
        wo_at = {NJ + t: range(cuts[t], cuts[t + 1]) for t in range(LP)}
        for g in range(NJ + LP):
            if g < NJ:
                proj(g)
            for j in wo_at.get(g, ()):
                acc_v[j, 0:rows, :] = wo_part(head_hs, j)
            if LS <= g < NJ + LS:
                ps[g - LS] = scores(*qk.pop(g - LS))
            if g >= LP:
                pv(g - LP)
            for fn in fill.get(g, ()):
                fn()
        for j in range(WO_AT[-1], KD):
            acc_v[j, 0:rows, :] = wo_part(head_hs, j)
        for j in range(KD):
            finish(j, acc_v[j, 0:rows, :] + wo_part(tail_hs, j))
        for fn in fill.get(NJ + LP, ()):
            fn()

    def attn_pair(i, fill_a, fill_b):
        xs = i % 2

        def finish_a(j, y):
            ya_v[j] = y[0:24]
            lhs_v[1, j, 8:16, :] = _pk(
                jnp.concatenate([hs_v[1, j], y[24:SEG]], axis=0))

        def finish_b(j, y):
            att = jnp.concatenate([ya_v[j], y[0:L]], axis=0)
            x = x_v[pl.ds(2 * i, 2), :, blk(j)].astype(F32).reshape(PAIR, LANE)
            x1_v[xs, :, blk(j)] = x + mod_blk(2, j) * att
            lhs_v[0, j, 8:16, :] = _pk(
                jnp.concatenate([hs_v[0, j], y[L:L + 8]], axis=0))

        segment(i, 0, fill_a, finish_a)
        segment(i, 1, fill_b, finish_b)

    P = functools.partial

    wait_unit(NJ - 1, 2)
    x_copy.wait()
    for cp in late_mod:
        cp.wait()
    mem0_copy.wait()
    wo_copy.wait()
    relayout(NJ - 1, 2)

    def last_body(p, carry):
        one = p.astype(F32)
        for n, w in enumerate((1, 2)):
            for m in range(KD):
                rows = slice(m * 32, (m + 1) * 32)
                hp = jnp.concatenate(
                    [_unpk(hpre_v[k, rows, :]) for k in range(KD)], axis=1)
                pre_v[w, NJ - 1, p, rows, :] = _pk(
                    _dot(hp, w_head(w, NJ - 1, p)))
                r = _dot(sc, _unpk(wml_v[p, :, blk(n * KD + m)]))[0:8]
                mod_v[(2 + n) * KD + m + 2 * KD * p] = r + one if n == 0 else r
            if n == 0:
                ln1(0, 0)
                mem0 = mem0_v[...].astype(F32)
                for k in range(KD):
                    lhs_v[0, k, 8:16, :] = _pk(jnp.concatenate(
                        [hs_v[0, k], mem0[:, blk(k)]], axis=0))
        return carry

    lax.fori_loop(0, 2, last_body, 0)

    def head_body(i, carry):
        attn_pair(i, {2: [P(ln1, 2 * i + 1, 1)]},
                  {2: [P(ln2, 1 - i)], 8: [P(ln1, 2 * i + 2, 0)]})
        return carry

    lax.fori_loop(0, 2, head_body, 0)
    for cp in ffn_copies:
        cp.wait()
    for f in range(NU0):
        up(f)

    def body(i, carry):
        slot = i % 2

        @pl.when(i >= 4)
        def _():
            out_copy(i - 4, slot).wait()

        fill_a, fill_b = {}, {}
        for f in range(NU0, NF):
            fill_a.setdefault((f - NU0) * NJ // (NF - NU0), []).append(P(up, f))
        downs = [P(down, slot, j, hf) for j in range(KD) for hf in range(2)]
        fill_a[NJ + LP] = downs[0:1]
        for n, fn in enumerate(downs[1:]):
            fill_b.setdefault(n, []).append(fn)
        fill_b.setdefault(2, []).append(P(ln2, 1 - slot))
        fill_a.setdefault(2, []).append(P(ln1, 2 * i + 1, 1))
        fill_b.setdefault(8, []).append(
            P(ln1, jnp.minimum(2 * i + 2, NSEG - 1), 0))
        fill_b.setdefault(NJ + LP - 1, []).append(P(up, 0))
        fill_b[NJ + LP] = [P(up, f) for f in range(1, NU0)]
        attn_pair(i, fill_a, fill_b)
        out_copy(i - 2, slot).start()
        return carry

    lax.fori_loop(2, NP, body, 0)

    out_copy(NP - 4, NP % 2).wait()

    def tail_body(q, carry):
        t, hf = q // 2, q % 2
        xs = (NP + t) % 2

        @pl.when(q == 2)
        def _():
            out_copy(NP - 3, xs).wait()

        for f in range(NH):
            up_half(hf, f, t, f)
        ln2((NP + 1) % 2, 1)
        for j in range(KD):
            y = _dot(_cat_pk(act_v, range(NH)), _unpk(w2_v[hf, :, blk(j)]))
            y = y + jnp.where(hf == 1, yh_v[:, blk(j)], 0.0)
            yh_v[:, blk(j)] = y
            stage_v[xs, :, blk(j)] = (
                x1_v[xs, :, blk(j)] + mod_blk(5, j) * y).astype(BF16)

        @pl.when(hf == 1)
        def _():
            out_copy(NP - 2 + t, xs).start()

        return carry

    lax.fori_loop(0, 4, tail_body, 0)
    out_copy(NP - 2, NP % 2).wait()
    out_copy(NP - 1, (NP + 1) % 2).wait()


@functools.partial(jax.jit, static_argnames=("A_seg_len",))
def pallas_adaLN_cond__memory_aug_recurrent_mem_tr__glu_gated_swiglu__prompt_kernel(
    A_x: jax.Array,
    A_mem0: jax.Array,
    A_Wq: jax.Array,
    A_Wk: jax.Array,
    A_Wv: jax.Array,
    A_Wo: jax.Array,
    A_seg_len,
    B_x: jax.Array,
    B_w1: jax.Array,
    B_w3: jax.Array,
    B_w2: jax.Array,
    c: jax.Array,
    w_mod: jax.Array,
):
    B, S, D = A_x.shape
    H, Dh = A_Wq.shape[1], A_Wq.shape[2]
    F = B_w1.shape[1]
    assert B == 1 and Dh == LANE and A_seg_len == SEG and A_mem0.shape[1] == MEM
    assert (S, D, H) == (2048, 1024, 32) and F % (2 * LANE) == 0
    KD, NF = D // LANE, F // LANE
    NSEG = S // SEG

    def split(w):
        return w.reshape(D // 16, 16, H // 2, 2, Dh)

    any_spec = pl.BlockSpec(memory_space=pl.ANY)
    out = pl.pallas_call(
        functools.partial(_kernel, S=S, D=D, H=H, F=F),
        out_shape=jax.ShapeDtypeStruct((S, D), A_x.dtype),
        in_specs=[any_spec] * 11,
        out_specs=any_spec,
        scratch_shapes=[
            pltpu.VMEM((1, D), BF16),
            pltpu.VMEM((MEM, D), BF16),
            pltpu.VMEM((NSEG, SEG, D), BF16),
            pltpu.VMEM((NSEG, 8, D), BF16),
            pltpu.VMEM((KD, NSEG * 8, LANE), F32),
            pltpu.VMEM((KD, NSEG * 4, LANE), U32),
            pltpu.VMEM((4, NSEG * 8, 2 * LANE), F32),
            pltpu.VMEM((3, H // 2, 2, NSEG * 4, LANE), U32),
            pltpu.VMEM((H // 2, D // 16, 16, LANE), U32),
            pltpu.VMEM((H // 2, D // 16, 16, LANE), U32),
            pltpu.VMEM((H // 2, D // 16, 16, LANE), U32),
            pltpu.VMEM((H * Dh // 2, D + LANE), U32),
            pltpu.VMEM((2, D // 2, F // 2 + LANE), U32),
            pltpu.VMEM((2, D // 2, F // 2 + LANE), U32),
            pltpu.VMEM((2, F // 4, D + LANE), U32),
            pltpu.VMEM((4, 2, D // 2, D // 4), U32),
            pltpu.VMEM((2, D // 2, 2 * D), U32),
            pltpu.VMEM((6 * KD, 8, LANE), F32),
            pltpu.VMEM((2, KD, 8, LANE), F32),
            pltpu.VMEM((2, KD, 16, LANE), U32),
            pltpu.VMEM((H, 8, LANE), F32),
            pltpu.VMEM((H, 16, LANE), U32),
            pltpu.VMEM((H, 24, LANE), U32),
            pltpu.VMEM((KD, 48, LANE), F32),
            pltpu.VMEM((KD, 24, LANE), F32),
            pltpu.VMEM((2, PAIR, D), F32),
            pltpu.VMEM((2, KD, PAIR // 2, LANE), U32),
            pltpu.VMEM((NF, PAIR // 2, LANE), U32),
            pltpu.VMEM((PAIR, D), F32),
            pltpu.VMEM((2, PAIR, D), BF16),
            pltpu.SemaphoreType.DMA((4,)),
            pltpu.SemaphoreType.DMA((5,)),
            pltpu.SemaphoreType.DMA((3 * H // 2,)),
            pltpu.SemaphoreType.DMA((2,)),
            pltpu.SemaphoreType.DMA((2,)),
        ],
        compiler_params=pltpu.CompilerParams(
            vmem_limit_bytes=110 * 1024 * 1024,
            disable_bounds_checks=True,
            disable_semaphore_checks=True),
        name="rmt_block",
    )(A_x.reshape(NSEG, SEG, D), A_mem0.reshape(MEM, D), split(A_Wq),
      split(A_Wk), split(A_Wv), A_Wo.reshape(H * Dh, D), B_w1, B_w3, B_w2, c,
      w_mod)
    return out.reshape(B, S, D)
```

```python
import functools

import jax
import jax.numpy as jnp
from jax import lax
import jax.experimental.pallas as pl
import jax.experimental.pallas.tpu as pltpu

F32 = jnp.float32
BF16 = jnp.bfloat16
U32 = jnp.uint32

LANE = 128
SEG = 32
MEM = 8
PAIR = 2 * SEG
EPS = 1e-5

LS, LP = 1, 3
TAIL = 8
WO_AT = (2, 4, 6)
NU_FIRST = 7
NU0 = 3


def _dot(a, b):
    return jnp.dot(a, b, preferred_element_type=F32)


def _layernorm(x):
    m = jnp.mean(x, axis=-1, keepdims=True)
    xc = x - m
    v = jnp.mean(xc * xc, axis=-1, keepdims=True)
    return xc * lax.rsqrt(v + EPS)


def _silu(x):
    hx = 0.5 * x
    return hx + hx * jnp.tanh(hx)


def _recip(x):
    r = pl.reciprocal(x, approx=True)
    return r * (2.0 - x * r)


def _pk(x):
    return pltpu.bitcast(x.astype(BF16), U32)


def _unpk(x):
    return pltpu.bitcast(x, BF16)


def _cat_pk(ref, ks, rows):
    return jnp.concatenate(
        [_unpk(ref[k, 0:rows // 2, :]) for k in ks], axis=1)


def _kernel(x_hbm, mem0_hbm, wq_hbm, wk_hbm, wv_hbm, wo_hbm, w1_hbm, w3_hbm,
            w2_hbm, c_hbm, wmod_hbm, out_hbm,
            c_v, mem0_v, x_v, xpre_v, xn_v, hpre_v, acc0_v, pre_v,
            wq_v, wk_v, wv_v, wo_v, w1_v, w3_v, w2_v, wme_v, wml_v,
            mod_v, hs_v, lhs_v, so_v, oa_v, ob_v, acc_v, ya_v,
            x1_v, h2_v, act_v, yh_v, stage_v,
            sem_x, sem_xp, sem_mod, sem_qkv, sem_w, sem_out,
            *, S, D, H, F):
    KD = D // LANE
    NF = F // LANE
    NP = S // PAIR
    NSEG = S // SEG
    NJ = H // 2
    NPRE = NSEG * 8
    L = SEG + MEM
    scale = float(LANE) ** -0.5
    w_hbm = (wq_hbm, wk_hbm, wv_hbm)
    w_v = (wq_v, wk_v, wv_v)

    def blk(j):
        return slice(j * LANE, (j + 1) * LANE)

    NCH = 4
    CK = KD // NCH

    def early_mod(ch):
        return [pltpu.make_async_copy(
            wmod_hbm.bitcast(U32).at[:, pl.ds(
                pl.multiple_of(t * D + ch * (CK * LANE), LANE), CK * LANE)],
            wme_v.at[ch, t], sem_mod.at[ch]) for t in range(2)]

    late_mod = [pltpu.make_async_copy(
        wmod_hbm.bitcast(U32).at[:, pl.ds((2 + 2 * t) * D, 2 * D)],
        wml_v.at[t], sem_mod.at[NCH]) for t in range(2)]

    def unit_copy(j, w):
        return pltpu.make_async_copy(
            w_hbm[w].bitcast(U32).at[:, :, j, 0, :],
            w_v[w].at[j], sem_qkv.at[3 * j + w])

    def start_unit(j, w):
        unit_copy(j, w).start()

    def wait_unit(j, w):
        unit_copy(j, w).wait()

    first_units = [(u // 3, u % 3) for u in range(NU_FIRST)]

    def slice_copies(ch):
        rows = pl.ds(ch * (CK * 8), CK * 8)
        return [pltpu.make_async_copy(
            w_hbm[w].bitcast(U32).at[rows, :, j, 0, :], w_v[w].at[j, rows],
            sem_mod.at[ch]) for j, w in first_units]

    wo_copy = pltpu.make_async_copy(
        wo_hbm.bitcast(U32), wo_v.at[:, pl.ds(0, D)], sem_w.at[0])
    FH = F // 2
    NH = NF // 2
    ffn_copies = []
    for hf in range(2):
        for src, dst in ((w1_hbm, w1_v), (w3_hbm, w3_v)):
            ffn_copies.append(pltpu.make_async_copy(
                src.bitcast(U32).at[:, pl.ds(hf * FH, FH)],
                dst.at[hf, :, pl.ds(0, FH)], sem_w.at[1]))
    for hf in range(2):
        ffn_copies.append(pltpu.make_async_copy(
            w2_hbm.bitcast(U32).at[pl.ds(hf * FH // 2, FH // 2), :],
            w2_v.at[hf, :, pl.ds(0, D)], sem_w.at[1]))
    c_copy = pltpu.make_async_copy(c_hbm, c_v, sem_x.at[2])
    mem0_copy = pltpu.make_async_copy(mem0_hbm, mem0_v, sem_x.at[3])
    x_copy = pltpu.make_async_copy(x_hbm, x_v, sem_x.at[1])
    NXP = 4
    XS = NSEG // NXP

    def xpre_copy(b):
        return pltpu.make_async_copy(
            x_hbm.at[pl.ds(b * XS, XS), pl.ds(0, 8), :],
            xpre_v.at[pl.ds(b * XS, XS)], sem_xp.at[b])

    def out_copy(i, slot):
        return pltpu.make_async_copy(
            stage_v.at[slot], out_hbm.at[pl.ds(i * PAIR, PAIR), :],
            sem_out.at[slot])

    def start_units(j0, j1):
        def step(j, carry):
            for w in range(3):
                start_unit(j, w)
            return carry

        lax.fori_loop(j0, j1, step, 0)

    j1 = NU_FIRST // 3
    for b in range(NXP):
        xpre_copy(b).start()
    c_copy.start()
    for ch in range(NCH):
        for cp in early_mod(ch) + slice_copies(ch):
            cp.start()
    start_unit(j1, 1)
    start_unit(j1, 2)
    start_units(j1 + 1, j1 + 7)
    x1_v[1] = jnp.zeros((PAIR, D), F32)

    def ln_pre(b, carry):
        xpre_copy(b).wait()
        for t in range(0, XS, 8):
            x = xpre_v[pl.ds(b * XS + t, 8)].astype(F32).reshape(64, D)
            xn = _layernorm(x)
            r0 = pl.multiple_of((b * XS + t) * 8, 64)
            for k in range(KD):
                xn_v[k, pl.ds(r0, 64), :] = xn[:, blk(k)]
        return carry

    lax.fori_loop(0, NXP, ln_pre, 0)

    def relayout_rows(j, w, r):
        rows = pl.ds(r, 8)
        a = w_v[w][j, rows, pl.ds(0, 8, stride=2), :]
        b = w_v[w][j, rows, pl.ds(1, 8, stride=2), :]
        w_v[w][j, rows, 0:8, :] = (a & U32(0xFFFF)) | (b << 16)
        w_v[w][j, rows, 8:16, :] = (a >> 16) | (b & U32(0xFFFF0000))

    def relayout(j, w):
        for k in range(KD):
            relayout_rows(j, w, k * 8)

    def w_head(w, j, p, k0=0, nk=KD):
        p8 = 8 * p if isinstance(p, int) else pl.multiple_of(8 * p, 8)
        t = w_v[w][j, pl.ds(k0 * 8, nk * 8), pl.ds(p8, 8), :]
        return _unpk(t.reshape(nk * LANE // 2, LANE))

    c_copy.wait()
    start_units(j1 + 7, NJ)
    mem0_copy.start()

    c = c_v[...].astype(F32)
    sc = _silu(c).astype(BF16)
    sc = jnp.broadcast_to(sc, (16, D))

    def mod_row(k):
        return jnp.concatenate([mod_blk(k, j) for j in range(KD)], axis=1)

    def mod_blk(k, j):
        return mod_v[k * KD + j, 0:1, :]

    def chunk_body(ch, carry):
        for cp in early_mod(ch) + slice_copies(ch):
            cp.wait()
        k0 = ch * CK
        for kk in range(CK):
            sa = _dot(sc, _unpk(wme_v[ch, 0, :, blk(kk)]))[0:8]
            ca = _dot(sc, _unpk(wme_v[ch, 1, :, blk(kk)]))[0:8] + 1.0
            mod_v[k0 + kk] = sa
            mod_v[KD + k0 + kk] = ca
            for r in range(0, NSEG * 8, 128):
                hpre_v[k0 + kk, r // 2:r // 2 + 64, :] = _pk(
                    xn_v[k0 + kk, r:r + 128, :] * ca[0:1] + sa[0:1])
        for u, (j, w) in enumerate(first_units):
            for kk in range(CK):
                relayout_rows(j, w, (k0 + kk) * 8)
            hp = _cat_pk(hpre_v, [k0 + kk for kk in range(CK)], NPRE)
            wt = jnp.concatenate(
                [w_head(w, j, p, k0, CK) for p in range(2)], axis=1)
            acc = jnp.where(ch > 0, acc0_v[u], 0.0) + _dot(hp, wt)
            acc0_v[u] = acc
            for p in range(2):
                pre_v[w, j, p] = _pk(acc[:, blk(p)])
        return carry

    lax.fori_loop(0, NCH, chunk_body, 0)

    def pre_dot(j, w, p):
        hp = _cat_pk(hpre_v, range(KD), NPRE)
        pre_v[w, j, p] = _pk(_dot(hp, w_head(w, j, p)))

    wait_unit(j1, 1)
    wo_copy.start()
    x_copy.start()
    for cp in late_mod + ffn_copies:
        cp.start()
    relayout(j1, 1)

    def pre_body(j, carry):
        wait_unit(j, 2)
        wait_unit(j + 1, 0)
        wait_unit(j + 1, 1)

        for (dj, dw), (rj, rw) in (((j, 1), (j, 2)), ((j, 2), (j + 1, 0)),
                                   ((j + 1, 0), (j + 1, 1))):
            pre_dot(dj, dw, 0)
            relayout(rj, rw)
            pre_dot(dj, dw, 1)
        return carry

    lax.fori_loop(j1, NJ - 1, pre_body, 0)

    def ln1(seg, sg):
        x = x_v[seg].astype(F32)[8:SEG]
        h = _layernorm(x) * mod_row(1) + mod_row(0)
        for k in range(KD):
            lhs_v[sg, k, 0:8, :] = _pk(h[0:16, blk(k)])
            hs_v[sg, k] = h[16:24, blk(k)]

    L2 = 2 * L
    rr = lax.broadcasted_iota(jnp.int32, (L2, L2), 0)
    cc = lax.broadcasted_iota(jnp.int32, (L2, L2), 1)
    same = (rr >= L) == (cc >= L)
    rr = jnp.where(rr >= L, rr - L, rr)
    cc = jnp.where(cc >= L, cc - L, cc)
    mask = same & ((rr >= SEG) | (cc >= SEG) | (cc <= rr))
    fill_val = jnp.where(same, -1000000000.0, -jnp.inf).astype(F32)

    def scores(q, k):
        s = lax.dot_general(q, k, (((1,), (1,)), ((), ())),
                            preferred_element_type=F32)
        s = jnp.where(mask, s * scale, fill_val)
        m = jnp.max(s, axis=-1, keepdims=True)
        e = jnp.exp(s - m)
        p = e * _recip(jnp.sum(e, axis=-1, keepdims=True))
        return p.astype(BF16)

    def ln2(xs, hs=0):
        h = _layernorm(x1_v[xs]) * mod_row(4) + mod_row(3)
        for k in range(KD):
            h2_v[hs, k, 0:PAIR // 2, :] = _pk(h[:, blk(k)])

    def up_half(hf, f, hs, dst):
        h2 = _cat_pk(h2_v.at[hs], range(KD), PAIR)
        g = _dot(h2, _unpk(w1_v[hf, :, blk(f)]))
        u = _dot(h2, _unpk(w3_v[hf, :, blk(f)]))
        act_v[dst, 0:PAIR // 2, :] = _pk(_silu(g) * u)

    def up(f):
        up_half(f // NH, f % NH, 0, f)

    def down(xs, j, hf):
        a = _cat_pk(act_v, range(hf * NH, (hf + 1) * NH), PAIR)
        y = _dot(a, _unpk(w2_v[hf, :, blk(j)]))
        if hf == 0:
            yh_v[:, blk(j)] = y
        else:
            y = y + yh_v[:, blk(j)]
            stage_v[xs, :, blk(j)] = (
                x1_v[xs, :, blk(j)] + mod_blk(5, j) * y).astype(BF16)

    def segment(i, sg, fill, finish):
        o_v = ob_v if sg else oa_v
        rows = L + 8 if sg else SEG
        prow = pl.multiple_of(i * 8, 8)
        qk, vs, ps = {}, {}, {}

        def proj(g):
            r = []
            for w in range(3):
                parts = []
                for p in range(2):
                    lhs = _cat_pk(lhs_v.at[sg], range(KD), SEG)
                    pre = _unpk(pre_v[w, g, p, pl.ds(prow, 8), :]).astype(F32)
                    parts += [pre[8 * sg:8 * sg + 8],
                              _dot(lhs, w_head(w, g, p))]
                r.append(jnp.concatenate(parts, axis=0).astype(BF16))
            qk[g] = r[0:2]
            vs[g] = r[2]

        def pv(g):
            o2 = _dot(ps.pop(g), vs.pop(g))
            for p in range(2):
                h = 2 * g + p
                o = o2[p * L:(p + 1) * L]
                if sg == 0:
                    o_v[h, 0:16, :] = _pk(
                        jnp.concatenate([o[0:24], o[SEG:L]], axis=0))
                    so_v[h] = o[24:SEG]
                else:
                    o_v[h] = _pk(jnp.concatenate([so_v[h], o], axis=0))

        def wo_part(hs, j):
            lo, hi = hs[0] * (LANE // 2), (hs[-1] + 1) * (LANE // 2)
            return _dot(_cat_pk(o_v, hs, rows), _unpk(wo_v[lo:hi, blk(j)]))

        head_hs = list(range(H - TAIL))
        tail_hs = list(range(H - TAIL, H))
        cuts = (0,) + WO_AT
        wo_at = {NJ + t: range(cuts[t], cuts[t + 1]) for t in range(LP)}
        for g in range(NJ + LP):
            if g < NJ:
                proj(g)
            for j in wo_at.get(g, ()):
                acc_v[j, 0:rows, :] = wo_part(head_hs, j)
            if LS <= g < NJ + LS:
                ps[g - LS] = scores(*qk.pop(g - LS))
            if g >= LP:
                pv(g - LP)
            for fn in fill.get(g, ()):
                fn()
        for j in range(WO_AT[-1], KD):
            acc_v[j, 0:rows, :] = wo_part(head_hs, j)
        for j in range(KD):
            finish(j, acc_v[j, 0:rows, :] + wo_part(tail_hs, j))
        for fn in fill.get(NJ + LP, ()):
            fn()

    def attn_pair(i, fill_a, fill_b):
        xs = i % 2

        def finish_a(j, y):
            ya_v[j] = y[0:24]
            lhs_v[1, j, 8:16, :] = _pk(
                jnp.concatenate([hs_v[1, j], y[24:SEG]], axis=0))

        def finish_b(j, y):
            att = jnp.concatenate([ya_v[j], y[0:L]], axis=0)
            x = x_v[pl.ds(2 * i, 2), :, blk(j)].astype(F32).reshape(PAIR, LANE)
            x1_v[xs, :, blk(j)] = x + mod_blk(2, j) * att
            lhs_v[0, j, 8:16, :] = _pk(
                jnp.concatenate([hs_v[0, j], y[L:L + 8]], axis=0))

        segment(i, 0, fill_a, finish_a)
        segment(i, 1, fill_b, finish_b)

    P = functools.partial

    wait_unit(NJ - 1, 2)
    x_copy.wait()
    for cp in late_mod:
        cp.wait()
    mem0_copy.wait()
    wo_copy.wait()
    relayout(NJ - 1, 2)

    def last_body(p, carry):
        one = p.astype(F32)
        for n, w in enumerate((1, 2)):
            for m in range(KD):
                rows = slice(m * 32, (m + 1) * 32)
                hp = jnp.concatenate(
                    [_unpk(hpre_v[k, rows, :]) for k in range(KD)], axis=1)
                pre_v[w, NJ - 1, p, rows, :] = _pk(
                    _dot(hp, w_head(w, NJ - 1, p)))
                r = _dot(sc, _unpk(wml_v[p, :, blk(n * KD + m)]))[0:8]
                mod_v[(2 + n) * KD + m + 2 * KD * p] = r + one if n == 0 else r
            if n == 0:
                ln1(0, 0)
                mem0 = mem0_v[...].astype(F32)
                for k in range(KD):
                    lhs_v[0, k, 8:16, :] = _pk(jnp.concatenate(
                        [hs_v[0, k], mem0[:, blk(k)]], axis=0))
        return carry

    lax.fori_loop(0, 2, last_body, 0)

    def head_body(i, carry):
        attn_pair(i, {2: [P(ln1, 2 * i + 1, 1)]},
                  {2: [P(ln2, 1 - i)], 8: [P(ln1, 2 * i + 2, 0)]})
        return carry

    lax.fori_loop(0, 2, head_body, 0)
    for cp in ffn_copies:
        cp.wait()
    for f in range(NU0):
        up(f)

    def body(i, carry):
        slot = i % 2

        @pl.when(i >= 4)
        def _():
            out_copy(i - 4, slot).wait()

        fill_a, fill_b = {}, {}
        for f in range(NU0, NF):
            fill_a.setdefault((f - NU0) * NJ // (NF - NU0), []).append(P(up, f))
        downs = [P(down, slot, j, hf) for j in range(KD) for hf in range(2)]
        fill_a[NJ + LP] = downs[0:1]
        for n, fn in enumerate(downs[1:]):
            fill_b.setdefault(n, []).append(fn)
        fill_b.setdefault(2, []).append(P(ln2, 1 - slot))
        fill_a.setdefault(2, []).append(P(ln1, 2 * i + 1, 1))
        fill_b.setdefault(8, []).append(
            P(ln1, jnp.minimum(2 * i + 2, NSEG - 1), 0))
        fill_b.setdefault(NJ + LP - 1, []).append(P(up, 0))
        fill_b[NJ + LP] = [P(up, f) for f in range(1, NU0)]
        attn_pair(i, fill_a, fill_b)
        out_copy(i - 2, slot).start()
        return carry

    lax.fori_loop(2, NP, body, 0)

    out_copy(NP - 4, NP % 2).wait()

    def tail_body(q, carry):
        t, hf = q // 2, q % 2
        xs = (NP + t) % 2

        @pl.when(q == 2)
        def _():
            out_copy(NP - 3, xs).wait()

        for f in range(NH):
            up_half(hf, f, t, f)
        ln2((NP + 1) % 2, 1)
        for j in range(KD):
            y = _dot(_cat_pk(act_v, range(NH), PAIR),
                     _unpk(w2_v[hf, :, blk(j)]))
            y = y + jnp.where(hf == 1, yh_v[:, blk(j)], 0.0)
            yh_v[:, blk(j)] = y
            stage_v[xs, :, blk(j)] = (
                x1_v[xs, :, blk(j)] + mod_blk(5, j) * y).astype(BF16)

        @pl.when(hf == 1)
        def _():
            out_copy(NP - 2 + t, xs).start()

        return carry

    lax.fori_loop(0, 4, tail_body, 0)
    out_copy(NP - 2, NP % 2).wait()
    out_copy(NP - 1, (NP + 1) % 2).wait()


@functools.partial(jax.jit, static_argnames=("A_seg_len",))
def pallas_adaLN_cond__memory_aug_recurrent_mem_tr__glu_gated_swiglu__prompt_kernel(
    A_x: jax.Array,
    A_mem0: jax.Array,
    A_Wq: jax.Array,
    A_Wk: jax.Array,
    A_Wv: jax.Array,
    A_Wo: jax.Array,
    A_seg_len,
    B_x: jax.Array,
    B_w1: jax.Array,
    B_w3: jax.Array,
    B_w2: jax.Array,
    c: jax.Array,
    w_mod: jax.Array,
):
    B, S, D = A_x.shape
    H, Dh = A_Wq.shape[1], A_Wq.shape[2]
    F = B_w1.shape[1]
    assert B == 1 and Dh == LANE and A_seg_len == SEG and A_mem0.shape[1] == MEM
    assert (S, D, H) == (2048, 1024, 32) and F % (2 * LANE) == 0
    KD, NF = D // LANE, F // LANE
    NSEG = S // SEG

    def split(w):
        return w.reshape(D // 16, 16, H // 2, 2, Dh)

    any_spec = pl.BlockSpec(memory_space=pl.ANY)
    out = pl.pallas_call(
        functools.partial(_kernel, S=S, D=D, H=H, F=F),
        out_shape=jax.ShapeDtypeStruct((S, D), A_x.dtype),
        in_specs=[any_spec] * 11,
        out_specs=any_spec,
        scratch_shapes=[
            pltpu.VMEM((1, D), BF16),
            pltpu.VMEM((MEM, D), BF16),
            pltpu.VMEM((NSEG, SEG, D), BF16),
            pltpu.VMEM((NSEG, 8, D), BF16),
            pltpu.VMEM((KD, NSEG * 8, LANE), F32),
            pltpu.VMEM((KD, NSEG * 4 + 8, LANE), U32),
            pltpu.VMEM((NU_FIRST, NSEG * 8, 2 * LANE), F32),
            pltpu.VMEM((3, H // 2, 2, NSEG * 4, LANE), U32),
            pltpu.VMEM((H // 2, D // 16, 16, LANE), U32),
            pltpu.VMEM((H // 2, D // 16, 16, LANE), U32),
            pltpu.VMEM((H // 2, D // 16, 16, LANE), U32),
            pltpu.VMEM((H * Dh // 2, D + LANE), U32),
            pltpu.VMEM((2, D // 2, F // 2 + LANE), U32),
            pltpu.VMEM((2, D // 2, F // 2 + LANE), U32),
            pltpu.VMEM((2, F // 4, D + LANE), U32),
            pltpu.VMEM((4, 2, D // 2, D // 4), U32),
            pltpu.VMEM((2, D // 2, 2 * D), U32),
            pltpu.VMEM((6 * KD, 8, LANE), F32),
            pltpu.VMEM((2, KD, 8, LANE), F32),
            pltpu.VMEM((2, KD, 24, LANE), U32),
            pltpu.VMEM((H, 8, LANE), F32),
            pltpu.VMEM((H, 24, LANE), U32),
            pltpu.VMEM((H, 24, LANE), U32),
            pltpu.VMEM((KD, 48, LANE), F32),
            pltpu.VMEM((KD, 24, LANE), F32),
            pltpu.VMEM((2, PAIR, D), F32),
            pltpu.VMEM((2, KD, PAIR // 2 + 8, LANE), U32),
            pltpu.VMEM((NF, PAIR // 2 + 8, LANE), U32),
            pltpu.VMEM((PAIR, D), F32),
            pltpu.VMEM((2, PAIR, D), BF16),
            pltpu.SemaphoreType.DMA((4,)),
            pltpu.SemaphoreType.DMA((4,)),
            pltpu.SemaphoreType.DMA((5,)),
            pltpu.SemaphoreType.DMA((3 * H // 2,)),
            pltpu.SemaphoreType.DMA((2,)),
            pltpu.SemaphoreType.DMA((2,)),
        ],
        compiler_params=pltpu.CompilerParams(
            vmem_limit_bytes=110 * 1024 * 1024,
            disable_bounds_checks=True,
            disable_semaphore_checks=True),
        name="rmt_block",
    )(A_x.reshape(NSEG, SEG, D), A_mem0.reshape(MEM, D), split(A_Wq),
      split(A_Wk), split(A_Wv), A_Wo.reshape(H * Dh, D), B_w1, B_w3, B_w2, c,
      w_mod)
    return out.reshape(B, S, D)
```

```python
import functools

import jax
import jax.numpy as jnp
from jax import lax
import jax.experimental.pallas as pl
import jax.experimental.pallas.tpu as pltpu

F32 = jnp.float32
BF16 = jnp.bfloat16
U32 = jnp.uint32

LANE = 128
SEG = 32
MEM = 8
PAIR = 2 * SEG
EPS = 1e-5

LS, LP = 1, 3
TAIL = 8
WO_AT = (2, 4, 6)
NU_FIRST = 7
NU0 = 3


def _dot(a, b):
    return jnp.dot(a, b, preferred_element_type=F32)


def _layernorm(x):
    m = jnp.mean(x, axis=-1, keepdims=True)
    xc = x - m
    v = jnp.mean(xc * xc, axis=-1, keepdims=True)
    return xc * lax.rsqrt(v + EPS)


def _silu(x):
    hx = 0.5 * x
    return hx + hx * jnp.tanh(hx)


def _recip(x):
    r = pl.reciprocal(x, approx=True)
    return r * (2.0 - x * r)


def _pk(x):
    return pltpu.bitcast(x.astype(BF16), U32)


def _unpk(x):
    return pltpu.bitcast(x, BF16)


def _cat_pk(ref, ks, rows):
    return jnp.concatenate(
        [_unpk(ref[k, 0:rows // 2, :]) for k in ks], axis=1)


def _kernel(x_hbm, mem0_hbm, wq_hbm, wk_hbm, wv_hbm, wo_hbm, w1_hbm, w3_hbm,
            w2_hbm, c_hbm, wmod_hbm, out_hbm,
            c_v, mem0_v, x_v, xpre_v, xn_v, hpre_v, acc0_v, pre_v,
            wq_v, wk_v, wv_v, wo_v, w1_v, w3_v, w2_v, wme_v, wml_v,
            mod_v, hs_v, lhs_v, so_v, oa_v, ob_v, acc_v, ya_v,
            x1_v, h2_v, act_v, yh_v, stage_v,
            sem_x, sem_xp, sem_mod, sem_qkv, sem_w, sem_out,
            *, S, D, H, F):
    KD = D // LANE
    NF = F // LANE
    NP = S // PAIR
    NSEG = S // SEG
    NJ = H // 2
    NPRE = NSEG * 8
    L = SEG + MEM
    scale = float(LANE) ** -0.5
    w_hbm = (wq_hbm, wk_hbm, wv_hbm)
    w_v = (wq_v, wk_v, wv_v)

    def blk(j):
        return slice(j * LANE, (j + 1) * LANE)

    NCH = 4
    CK = KD // NCH

    def early_mod(ch):
        return [pltpu.make_async_copy(
            wmod_hbm.bitcast(U32).at[:, pl.ds(
                pl.multiple_of(t * D + ch * (CK * LANE), LANE), CK * LANE)],
            wme_v.at[ch, t], sem_mod.at[ch]) for t in range(2)]

    late_mod = [pltpu.make_async_copy(
        wmod_hbm.bitcast(U32).at[:, pl.ds((2 + 2 * t) * D, 2 * D)],
        wml_v.at[t], sem_mod.at[NCH]) for t in range(2)]

    def unit_copy(j, w):
        return pltpu.make_async_copy(
            w_hbm[w].bitcast(U32).at[:, :, j, 0, :],
            w_v[w].at[j], sem_qkv.at[3 * j + w])

    def start_unit(j, w):
        unit_copy(j, w).start()

    def wait_unit(j, w):
        unit_copy(j, w).wait()

    first_units = [(u // 3, u % 3) for u in range(NU_FIRST)]

    def slice_copies(ch):
        rows = pl.ds(ch * (CK * 8), CK * 8)
        return [pltpu.make_async_copy(
            w_hbm[w].bitcast(U32).at[rows, :, j, 0, :], w_v[w].at[j, rows],
            sem_mod.at[ch]) for j, w in first_units]

    wo_copy = pltpu.make_async_copy(
        wo_hbm.bitcast(U32), wo_v.at[:, pl.ds(0, D)], sem_w.at[0])
    FH = F // 2
    NH = NF // 2
    ffn_copies = []
    for hf in range(2):
        for src, dst in ((w1_hbm, w1_v), (w3_hbm, w3_v)):
            ffn_copies.append(pltpu.make_async_copy(
                src.bitcast(U32).at[:, pl.ds(hf * FH, FH)],
                dst.at[hf, :, pl.ds(0, FH)], sem_w.at[1]))
    for hf in range(2):
        ffn_copies.append(pltpu.make_async_copy(
            w2_hbm.bitcast(U32).at[pl.ds(hf * FH // 2, FH // 2), :],
            w2_v.at[hf, :, pl.ds(0, D)], sem_w.at[1]))
    c_copy = pltpu.make_async_copy(c_hbm, c_v, sem_x.at[2])
    mem0_copy = pltpu.make_async_copy(mem0_hbm, mem0_v, sem_x.at[3])
    x_copy = pltpu.make_async_copy(x_hbm, x_v, sem_x.at[1])
    NXP = 4
    XS = NSEG // NXP

    def xpre_copy(b):
        return pltpu.make_async_copy(
            x_hbm.at[pl.ds(b * XS, XS), pl.ds(0, 8), :],
            xpre_v.at[pl.ds(b * XS, XS)], sem_xp.at[b])

    def out_copy(i, slot):
        return pltpu.make_async_copy(
            stage_v.at[slot], out_hbm.at[pl.ds(i * PAIR, PAIR), :],
            sem_out.at[slot])

    def start_units(j0, j1):
        def step(j, carry):
            for w in range(3):
                start_unit(j, w)
            return carry

        lax.fori_loop(j0, j1, step, 0)

    j1 = NU_FIRST // 3
    for b in range(NXP):
        xpre_copy(b).start()
    c_copy.start()

    def start_chunk(ch, carry):
        for cp in early_mod(ch) + slice_copies(ch):
            cp.start()
        return carry

    lax.fori_loop(0, NCH, start_chunk, 0)
    start_unit(j1, 1)
    start_unit(j1, 2)
    start_units(j1 + 1, j1 + 7)
    x1_v[1] = jnp.zeros((PAIR, D), F32)

    def ln_pre(b, carry):
        @pl.when(b % (XS // 8) == 0)
        def _():
            xpre_copy(b // (XS // 8)).wait()

        x = xpre_v[pl.ds(b * 8, 8)].astype(F32).reshape(64, D)
        xn = _layernorm(x)
        r0 = pl.multiple_of(b * 64, 64)
        for k in range(KD):
            xn_v[k, pl.ds(r0, 64), :] = xn[:, blk(k)]
        return carry

    lax.fori_loop(0, NSEG // 8, ln_pre, 0)

    def relayout_rows(j, w, r):
        rows = pl.ds(r, 8)
        a = w_v[w][j, rows, pl.ds(0, 8, stride=2), :]
        b = w_v[w][j, rows, pl.ds(1, 8, stride=2), :]
        w_v[w][j, rows, 0:8, :] = (a & U32(0xFFFF)) | (b << 16)
        w_v[w][j, rows, 8:16, :] = (a >> 16) | (b & U32(0xFFFF0000))

    def relayout(j, w):
        for k in range(KD):
            relayout_rows(j, w, k * 8)

    def w_head(w, j, p, k0=0, nk=KD):
        p8 = 8 * p if isinstance(p, int) else pl.multiple_of(8 * p, 8)
        t = w_v[w][j, pl.ds(k0 * 8, nk * 8), pl.ds(p8, 8), :]
        return _unpk(t.reshape(nk * LANE // 2, LANE))

    c_copy.wait()
    start_units(j1 + 7, NJ)
    mem0_copy.start()

    c = c_v[...].astype(F32)
    sc = _silu(c).astype(BF16)
    sc = jnp.broadcast_to(sc, (16, D))

    def mod_row(k):
        return jnp.concatenate([mod_blk(k, j) for j in range(KD)], axis=1)

    def mod_blk(k, j):
        return mod_v[k * KD + j, 0:1, :]

    def chunk_body(ch, carry):
        for cp in early_mod(ch) + slice_copies(ch):
            cp.wait()
        k0 = ch * CK
        for kk in range(CK):
            sa = _dot(sc, _unpk(wme_v[ch, 0, :, blk(kk)]))[0:8]
            ca = _dot(sc, _unpk(wme_v[ch, 1, :, blk(kk)]))[0:8] + 1.0
            mod_v[k0 + kk] = sa
            mod_v[KD + k0 + kk] = ca
            for r in range(0, NSEG * 8, 128):
                hpre_v[k0 + kk, r // 2:r // 2 + 64, :] = _pk(
                    xn_v[k0 + kk, r:r + 128, :] * ca[0:1] + sa[0:1])
        for u, (j, w) in enumerate(first_units):
            for kk in range(CK):
                relayout_rows(j, w, (k0 + kk) * 8)
            hp = _cat_pk(hpre_v, [k0 + kk for kk in range(CK)], NPRE)
            wt = jnp.concatenate(
                [w_head(w, j, p, k0, CK) for p in range(2)], axis=1)
            acc = jnp.where(ch > 0, acc0_v[u], 0.0) + _dot(hp, wt)
            acc0_v[u] = acc
            for p in range(2):
                pre_v[w, j, p] = _pk(acc[:, blk(p)])
        return carry

    lax.fori_loop(0, NCH, chunk_body, 0)

    def pre_dot(j, w, p):
        hp = _cat_pk(hpre_v, range(KD), NPRE)
        pre_v[w, j, p] = _pk(_dot(hp, w_head(w, j, p)))

    wait_unit(j1, 1)
    wo_copy.start()
    x_copy.start()
    for cp in late_mod + ffn_copies:
        cp.start()
    relayout(j1, 1)

    def pre_body(j, carry):
        wait_unit(j, 2)
        wait_unit(j + 1, 0)
        wait_unit(j + 1, 1)

        for (dj, dw), (rj, rw) in (((j, 1), (j, 2)), ((j, 2), (j + 1, 0)),
                                   ((j + 1, 0), (j + 1, 1))):
            pre_dot(dj, dw, 0)
            relayout(rj, rw)
            pre_dot(dj, dw, 1)
        return carry

    lax.fori_loop(j1, NJ - 1, pre_body, 0)

    def ln1(seg, sg):
        x = x_v[seg].astype(F32)[8:SEG]
        h = _layernorm(x) * mod_row(1) + mod_row(0)
        for k in range(KD):
            lhs_v[sg, k, 0:8, :] = _pk(h[0:16, blk(k)])
            hs_v[sg, k] = h[16:24, blk(k)]

    L2 = 2 * L
    rr = lax.broadcasted_iota(jnp.int32, (L2, L2), 0)
    cc = lax.broadcasted_iota(jnp.int32, (L2, L2), 1)
    same = (rr >= L) == (cc >= L)
    rr = jnp.where(rr >= L, rr - L, rr)
    cc = jnp.where(cc >= L, cc - L, cc)
    mask = same & ((rr >= SEG) | (cc >= SEG) | (cc <= rr))
    fill_val = jnp.where(same, -1000000000.0, -jnp.inf).astype(F32)

    def scores(q, k):
        s = lax.dot_general(q, k, (((1,), (1,)), ((), ())),
                            preferred_element_type=F32)
        s = jnp.where(mask, s * scale, fill_val)
        m = jnp.max(s, axis=-1, keepdims=True)
        e = jnp.exp(s - m)
        p = e * _recip(jnp.sum(e, axis=-1, keepdims=True))
        return p.astype(BF16)

    def ln2(xs, hs=0):
        h = _layernorm(x1_v[xs]) * mod_row(4) + mod_row(3)
        for k in range(KD):
            h2_v[hs, k, 0:PAIR // 2, :] = _pk(h[:, blk(k)])

    def up_half(hf, f, hs, dst):
        h2 = _cat_pk(h2_v.at[hs], range(KD), PAIR)
        g = _dot(h2, _unpk(w1_v[hf, :, blk(f)]))
        u = _dot(h2, _unpk(w3_v[hf, :, blk(f)]))
        act_v[dst, 0:PAIR // 2, :] = _pk(_silu(g) * u)

    def up(f):
        up_half(f // NH, f % NH, 0, f)

    def down(xs, j, hf):
        a = _cat_pk(act_v, range(hf * NH, (hf + 1) * NH), PAIR)
        y = _dot(a, _unpk(w2_v[hf, :, blk(j)]))
        if hf == 0:
            yh_v[:, blk(j)] = y
        else:
            y = y + yh_v[:, blk(j)]
            stage_v[xs, :, blk(j)] = (
                x1_v[xs, :, blk(j)] + mod_blk(5, j) * y).astype(BF16)

    def segment(i, sg, fill, finish):
        o_v = ob_v if sg else oa_v
        rows = L + 8 if sg else SEG
        prow = pl.multiple_of(i * 8, 8)
        qk, vs, ps = {}, {}, {}

        def proj(g):
            r = []
            for w in range(3):
                parts = []
                for p in range(2):
                    lhs = _cat_pk(lhs_v.at[sg], range(KD), SEG)
                    pre = _unpk(pre_v[w, g, p, pl.ds(prow, 8), :]).astype(F32)
                    parts += [pre[8 * sg:8 * sg + 8],
                              _dot(lhs, w_head(w, g, p))]
                r.append(jnp.concatenate(parts, axis=0).astype(BF16))
            qk[g] = r[0:2]
            vs[g] = r[2]

        def pv(g):
            o2 = _dot(ps.pop(g), vs.pop(g))
            for p in range(2):
                h = 2 * g + p
                o = o2[p * L:(p + 1) * L]
                if sg == 0:
                    o_v[h, 0:16, :] = _pk(
                        jnp.concatenate([o[0:24], o[SEG:L]], axis=0))
                    so_v[h] = o[24:SEG]
                else:
                    o_v[h] = _pk(jnp.concatenate([so_v[h], o], axis=0))

        def wo_part(hs, j):
            lo, hi = hs[0] * (LANE // 2), (hs[-1] + 1) * (LANE // 2)
            return _dot(_cat_pk(o_v, hs, rows), _unpk(wo_v[lo:hi, blk(j)]))

        head_hs = list(range(H - TAIL))
        tail_hs = list(range(H - TAIL, H))
        cuts = (0,) + WO_AT
        wo_at = {NJ + t: range(cuts[t], cuts[t + 1]) for t in range(LP)}
        for g in range(NJ + LP):
            if g < NJ:
                proj(g)
            for j in wo_at.get(g, ()):
                acc_v[j, 0:rows, :] = wo_part(head_hs, j)
            if LS <= g < NJ + LS:
                ps[g - LS] = scores(*qk.pop(g - LS))
            if g >= LP:
                pv(g - LP)
            for fn in fill.get(g, ()):
                fn()
        for j in range(WO_AT[-1], KD):
            acc_v[j, 0:rows, :] = wo_part(head_hs, j)
        for j in range(KD):
            finish(j, acc_v[j, 0:rows, :] + wo_part(tail_hs, j))
        for fn in fill.get(NJ + LP, ()):
            fn()

    def attn_pair(i, fill_a, fill_b):
        xs = i % 2

        def finish_a(j, y):
            ya_v[j] = y[0:24]
            lhs_v[1, j, 8:16, :] = _pk(
                jnp.concatenate([hs_v[1, j], y[24:SEG]], axis=0))

        def finish_b(j, y):
            att = jnp.concatenate([ya_v[j], y[0:L]], axis=0)
            x = x_v[pl.ds(2 * i, 2), :, blk(j)].astype(F32).reshape(PAIR, LANE)
            x1_v[xs, :, blk(j)] = x + mod_blk(2, j) * att
            lhs_v[0, j, 8:16, :] = _pk(
                jnp.concatenate([hs_v[0, j], y[L:L + 8]], axis=0))

        segment(i, 0, fill_a, finish_a)
        segment(i, 1, fill_b, finish_b)

    P = functools.partial

    wait_unit(NJ - 1, 2)
    x_copy.wait()
    for cp in late_mod:
        cp.wait()
    mem0_copy.wait()
    wo_copy.wait()
    relayout(NJ - 1, 2)

    def last_body(p, carry):
        one = p.astype(F32)
        for n, w in enumerate((1, 2)):
            for m in range(KD):
                rows = slice(m * 32, (m + 1) * 32)
                hp = jnp.concatenate(
                    [_unpk(hpre_v[k, rows, :]) for k in range(KD)], axis=1)
                pre_v[w, NJ - 1, p, rows, :] = _pk(
                    _dot(hp, w_head(w, NJ - 1, p)))
                r = _dot(sc, _unpk(wml_v[p, :, blk(n * KD + m)]))[0:8]
                mod_v[(2 + n) * KD + m + 2 * KD * p] = r + one if n == 0 else r
            if n == 0:
                ln1(0, 0)
                mem0 = mem0_v[...].astype(F32)
                for k in range(KD):
                    lhs_v[0, k, 8:16, :] = _pk(jnp.concatenate(
                        [hs_v[0, k], mem0[:, blk(k)]], axis=0))
        return carry

    lax.fori_loop(0, 2, last_body, 0)

    def head_body(i, carry):
        attn_pair(i, {2: [P(ln1, 2 * i + 1, 1)]},
                  {2: [P(ln2, 1 - i)], 8: [P(ln1, 2 * i + 2, 0)]})
        return carry

    lax.fori_loop(0, 2, head_body, 0)
    for cp in ffn_copies:
        cp.wait()
    for f in range(NU0):
        up(f)

    def body(i, carry):
        slot = i % 2

        @pl.when(i >= 4)
        def _():
            out_copy(i - 4, slot).wait()

        fill_a, fill_b = {}, {}
        for f in range(NU0, NF):
            fill_a.setdefault((f - NU0) * NJ // (NF - NU0), []).append(P(up, f))
        downs = [P(down, slot, j, hf) for j in range(KD) for hf in range(2)]
        fill_a[NJ + LP] = downs[0:1]
        for n, fn in enumerate(downs[1:]):
            fill_b.setdefault(n, []).append(fn)
        fill_b.setdefault(2, []).append(P(ln2, 1 - slot))
        fill_a.setdefault(2, []).append(P(ln1, 2 * i + 1, 1))
        fill_b.setdefault(8, []).append(
            P(ln1, jnp.minimum(2 * i + 2, NSEG - 1), 0))
        fill_b.setdefault(NJ + LP - 1, []).append(P(up, 0))
        fill_b[NJ + LP] = [P(up, f) for f in range(1, NU0)]
        attn_pair(i, fill_a, fill_b)
        out_copy(i - 2, slot).start()
        return carry

    lax.fori_loop(2, NP, body, 0)

    out_copy(NP - 4, NP % 2).wait()

    def tail_body(q, carry):
        t, hf = q // 2, q % 2
        xs = (NP + t) % 2

        @pl.when(q == 2)
        def _():
            out_copy(NP - 3, xs).wait()

        for f in range(NH):
            up_half(hf, f, t, f)
        ln2((NP + 1) % 2, 1)
        for j in range(KD):
            y = _dot(_cat_pk(act_v, range(NH), PAIR),
                     _unpk(w2_v[hf, :, blk(j)]))
            y = y + jnp.where(hf == 1, yh_v[:, blk(j)], 0.0)
            yh_v[:, blk(j)] = y
            stage_v[xs, :, blk(j)] = (
                x1_v[xs, :, blk(j)] + mod_blk(5, j) * y).astype(BF16)

        @pl.when(hf == 1)
        def _():
            out_copy(NP - 2 + t, xs).start()

        return carry

    lax.fori_loop(0, 4, tail_body, 0)
    out_copy(NP - 2, NP % 2).wait()
    out_copy(NP - 1, (NP + 1) % 2).wait()


@functools.partial(jax.jit, static_argnames=("A_seg_len",))
def pallas_adaLN_cond__memory_aug_recurrent_mem_tr__glu_gated_swiglu__prompt_kernel(
    A_x: jax.Array,
    A_mem0: jax.Array,
    A_Wq: jax.Array,
    A_Wk: jax.Array,
    A_Wv: jax.Array,
    A_Wo: jax.Array,
    A_seg_len,
    B_x: jax.Array,
    B_w1: jax.Array,
    B_w3: jax.Array,
    B_w2: jax.Array,
    c: jax.Array,
    w_mod: jax.Array,
):
    B, S, D = A_x.shape
    H, Dh = A_Wq.shape[1], A_Wq.shape[2]
    F = B_w1.shape[1]
    assert B == 1 and Dh == LANE and A_seg_len == SEG and A_mem0.shape[1] == MEM
    assert (S, D, H) == (2048, 1024, 32) and F % (2 * LANE) == 0
    KD, NF = D // LANE, F // LANE
    NSEG = S // SEG

    def split(w):
        return w.reshape(D // 16, 16, H // 2, 2, Dh)

    any_spec = pl.BlockSpec(memory_space=pl.ANY)
    out = pl.pallas_call(
        functools.partial(_kernel, S=S, D=D, H=H, F=F),
        out_shape=jax.ShapeDtypeStruct((S, D), A_x.dtype),
        in_specs=[any_spec] * 11,
        out_specs=any_spec,
        scratch_shapes=[
            pltpu.VMEM((1, D), BF16),
            pltpu.VMEM((MEM, D), BF16),
            pltpu.VMEM((NSEG, SEG, D), BF16),
            pltpu.VMEM((NSEG, 8, D), BF16),
            pltpu.VMEM((KD, NSEG * 8, LANE), F32),
            pltpu.VMEM((KD, NSEG * 4 + 8, LANE), U32),
            pltpu.VMEM((NU_FIRST, NSEG * 8, 2 * LANE), F32),
            pltpu.VMEM((3, H // 2, 2, NSEG * 4, LANE), U32),
            pltpu.VMEM((H // 2, D // 16, 16, LANE), U32),
            pltpu.VMEM((H // 2, D // 16, 16, LANE), U32),
            pltpu.VMEM((H // 2, D // 16, 16, LANE), U32),
            pltpu.VMEM((H * Dh // 2, D + LANE), U32),
            pltpu.VMEM((2, D // 2, F // 2 + LANE), U32),
            pltpu.VMEM((2, D // 2, F // 2 + LANE), U32),
            pltpu.VMEM((2, F // 4, D + LANE), U32),
            pltpu.VMEM((4, 2, D // 2, D // 4), U32),
            pltpu.VMEM((2, D // 2, 2 * D), U32),
            pltpu.VMEM((6 * KD, 8, LANE), F32),
            pltpu.VMEM((2, KD, 8, LANE), F32),
            pltpu.VMEM((2, KD, 24, LANE), U32),
            pltpu.VMEM((H, 8, LANE), F32),
            pltpu.VMEM((H, 24, LANE), U32),
            pltpu.VMEM((H, 24, LANE), U32),
            pltpu.VMEM((KD, 48, LANE), F32),
            pltpu.VMEM((KD, 24, LANE), F32),
            pltpu.VMEM((2, PAIR, D), F32),
            pltpu.VMEM((2, KD, PAIR // 2 + 8, LANE), U32),
            pltpu.VMEM((NF, PAIR // 2 + 8, LANE), U32),
            pltpu.VMEM((PAIR, D), F32),
            pltpu.VMEM((2, PAIR, D), BF16),
            pltpu.SemaphoreType.DMA((4,)),
            pltpu.SemaphoreType.DMA((4,)),
            pltpu.SemaphoreType.DMA((5,)),
            pltpu.SemaphoreType.DMA((3 * H // 2,)),
            pltpu.SemaphoreType.DMA((2,)),
            pltpu.SemaphoreType.DMA((2,)),
        ],
        compiler_params=pltpu.CompilerParams(
            vmem_limit_bytes=110 * 1024 * 1024,
            disable_bounds_checks=True,
            disable_semaphore_checks=True),
        name="rmt_block",
    )(A_x.reshape(NSEG, SEG, D), A_mem0.reshape(MEM, D), split(A_Wq),
      split(A_Wk), split(A_Wv), A_Wo.reshape(H * Dh, D), B_w1, B_w3, B_w2, c,
      w_mod)
    return out.reshape(B, S, D)
```

```python
import functools

import jax
import jax.numpy as jnp
from jax import lax
import jax.experimental.pallas as pl
import jax.experimental.pallas.tpu as pltpu

F32 = jnp.float32
BF16 = jnp.bfloat16
U32 = jnp.uint32

LANE = 128
SEG = 32
MEM = 8
PAIR = 2 * SEG
EPS = 1e-5

LS, LP = 1, 3
TAIL = 8
WO_AT = (2, 4, 6)
HEAD_A = (1, 3, 5, 7, 9, 11, 13, 19)
HEAD_B = (1, 3, 6, 9, 12, 18, 19, 19)
NU_FIRST = 7
NU0 = 3


def _dot(a, b):
    return jnp.dot(a, b, preferred_element_type=F32)


def _layernorm(x):
    m = jnp.mean(x, axis=-1, keepdims=True)
    xc = x - m
    v = jnp.mean(xc * xc, axis=-1, keepdims=True)
    return xc * lax.rsqrt(v + EPS)


def _silu(x):
    hx = 0.5 * x
    return hx + hx * jnp.tanh(hx)


def _recip(x):
    r = pl.reciprocal(x, approx=True)
    return r * (2.0 - x * r)


def _pk(x):
    return pltpu.bitcast(x.astype(BF16), U32)


def _unpk(x):
    return pltpu.bitcast(x, BF16)


def _cat_pk(ref, ks, rows):
    return jnp.concatenate(
        [_unpk(ref[k, 0:rows // 2, :]) for k in ks], axis=1)


def _kernel(x_hbm, mem0_hbm, wq_hbm, wk_hbm, wv_hbm, wo_hbm, w1_hbm, w3_hbm,
            w2_hbm, c_hbm, wmod_hbm, out_hbm,
            c_v, mem0_v, x0_v, x_v, xpre_v, xn_v, hpre_v, acc0_v, pre_v,
            wq_v, wk_v, wv_v, wo_v, w1_v, w3_v, w2_v, wme_v, wml_v,
            mod_v, hs_v, lhs_v, so_v, oa_v, ob_v, acc_v, ya_v,
            x1_v, h2_v, act_v, yh_v, stage_v,
            sem_x, sem_xp, sem_mod, sem_qkv, sem_w, sem_out,
            *, S, D, H, F):
    KD = D // LANE
    NF = F // LANE
    NP = S // PAIR
    NSEG = S // SEG
    NJ = H // 2
    NPRE = NSEG * 8
    L = SEG + MEM
    scale = float(LANE) ** -0.5
    w_hbm = (wq_hbm, wk_hbm, wv_hbm)
    w_v = (wq_v, wk_v, wv_v)

    def blk(j):
        return slice(j * LANE, (j + 1) * LANE)

    NCH = 4
    CK = KD // NCH

    def early_mod(ch):
        return [pltpu.make_async_copy(
            wmod_hbm.bitcast(U32).at[:, pl.ds(
                pl.multiple_of(t * D + ch * (CK * LANE), LANE), CK * LANE)],
            wme_v.at[ch, t], sem_mod.at[ch]) for t in range(2)]

    late_mod = [pltpu.make_async_copy(
        wmod_hbm.bitcast(U32).at[:, pl.ds((2 + 2 * t) * D, 2 * D)],
        wml_v.at[t], sem_mod.at[NCH]) for t in range(2)]

    def unit_copy(j, w):
        return pltpu.make_async_copy(
            w_hbm[w].bitcast(U32).at[:, :, j, 0, :],
            w_v[w].at[j], sem_qkv.at[3 * j + w])

    def start_unit(j, w):
        unit_copy(j, w).start()

    def wait_unit(j, w):
        unit_copy(j, w).wait()

    first_units = [(u // 3, u % 3) for u in range(NU_FIRST)]

    def slice_copies(ch):
        rows = pl.ds(ch * (CK * 8), CK * 8)
        return [pltpu.make_async_copy(
            w_hbm[w].bitcast(U32).at[rows, :, j, 0, :], w_v[w].at[j, rows],
            sem_mod.at[ch]) for j, w in first_units]

    wo_copy = pltpu.make_async_copy(
        wo_hbm.bitcast(U32), wo_v.at[:, pl.ds(0, D)], sem_w.at[0])
    FH = F // 2
    NH = NF // 2
    ffn_copies = []
    for hf in range(2):
        for src, dst in ((w1_hbm, w1_v), (w3_hbm, w3_v)):
            ffn_copies.append(pltpu.make_async_copy(
                src.bitcast(U32).at[:, pl.ds(hf * FH, FH)],
                dst.at[hf, :, pl.ds(0, FH)], sem_w.at[1]))
    for hf in range(2):
        ffn_copies.append(pltpu.make_async_copy(
            w2_hbm.bitcast(U32).at[pl.ds(hf * FH // 2, FH // 2), :],
            w2_v.at[hf, :, pl.ds(0, D)], sem_w.at[1]))
    c_copy = pltpu.make_async_copy(c_hbm, c_v, sem_x.at[2])
    mem0_copy = pltpu.make_async_copy(mem0_hbm, mem0_v, sem_x.at[3])
    x_copy = pltpu.make_async_copy(x_hbm, x_v, sem_x.at[1])
    x0_copy = pltpu.make_async_copy(x_hbm.at[0], x0_v, sem_x.at[0])
    NXP = 4
    XS = NSEG // NXP

    def xpre_copy(b):
        return pltpu.make_async_copy(
            x_hbm.at[pl.ds(b * XS, XS), pl.ds(0, 8), :],
            xpre_v.at[pl.ds(b * XS, XS)], sem_xp.at[b])

    def out_copy(i, slot):
        return pltpu.make_async_copy(
            stage_v.at[slot], out_hbm.at[pl.ds(i * PAIR, PAIR), :],
            sem_out.at[slot])

    def start_units(j0, j1):
        def step(j, carry):
            for w in range(3):
                start_unit(j, w)
            return carry

        lax.fori_loop(j0, j1, step, 0)

    j1 = NU_FIRST // 3
    for b in range(NXP):
        xpre_copy(b).start()
    c_copy.start()

    def start_chunk(ch, carry):
        for cp in early_mod(ch) + slice_copies(ch):
            cp.start()
        return carry

    lax.fori_loop(0, NCH, start_chunk, 0)
    mem0_copy.start()
    x0_copy.start()
    start_unit(j1, 1)
    start_unit(j1, 2)
    start_units(j1 + 1, j1 + 7)
    x1_v[1] = jnp.zeros((PAIR, D), F32)
    mod_v[3 * KD:5 * KD] = jnp.zeros((2 * KD, 8, LANE), F32)

    def ln_pre(b, carry):
        @pl.when(b % (XS // 8) == 0)
        def _():
            xpre_copy(b // (XS // 8)).wait()

        x = xpre_v[pl.ds(b * 8, 8)].astype(F32).reshape(64, D)
        xn = _layernorm(x)
        r0 = pl.multiple_of(b * 64, 64)
        for k in range(KD):
            xn_v[k, pl.ds(r0, 64), :] = xn[:, blk(k)]
        return carry

    lax.fori_loop(0, NSEG // 8, ln_pre, 0)

    def relayout_rows(j, w, r, do=None):
        rows = pl.ds(r, 8)
        a = w_v[w][j, rows, pl.ds(0, 8, stride=2), :]
        b = w_v[w][j, rows, pl.ds(1, 8, stride=2), :]
        lo = (a & U32(0xFFFF)) | (b << 16)
        hi = (a >> 16) | (b & U32(0xFFFF0000))
        if do is not None:
            lo = jnp.where(do, lo, w_v[w][j, rows, 0:8, :])
            hi = jnp.where(do, hi, w_v[w][j, rows, 8:16, :])
        w_v[w][j, rows, 0:8, :] = lo
        w_v[w][j, rows, 8:16, :] = hi

    def relayout(j, w, do=None):
        for k in range(KD):
            relayout_rows(j, w, k * 8, do)

    def w_head(w, j, p, k0=0, nk=KD):
        t = w_v[w][j, pl.ds(k0 * 8, nk * 8), 8 * p:8 * p + 8, :]
        return _unpk(t.reshape(nk * LANE // 2, LANE))

    c_copy.wait()
    start_units(j1 + 7, NJ)

    c = c_v[...].astype(F32)
    sc = _silu(c).astype(BF16)
    sc = jnp.broadcast_to(sc, (16, D))

    def mod_row(k):
        return jnp.concatenate([mod_blk(k, j) for j in range(KD)], axis=1)

    def mod_blk(k, j):
        return mod_v[k * KD + j, 0:1, :]

    def chunk_body(ch, carry):
        for cp in early_mod(ch) + slice_copies(ch):
            cp.wait()
        k0 = ch * CK
        for kk in range(CK):
            sa = _dot(sc, _unpk(wme_v[ch, 0, :, blk(kk)]))[0:8]
            ca = _dot(sc, _unpk(wme_v[ch, 1, :, blk(kk)]))[0:8] + 1.0
            mod_v[k0 + kk] = sa
            mod_v[KD + k0 + kk] = ca
            for r in range(0, NSEG * 8, 128):
                hpre_v[k0 + kk, r // 2:r // 2 + 64, :] = _pk(
                    xn_v[k0 + kk, r:r + 128, :] * ca[0:1] + sa[0:1])
        for u, (j, w) in enumerate(first_units):
            for kk in range(CK):
                relayout_rows(j, w, (k0 + kk) * 8)
            hp = _cat_pk(hpre_v, [k0 + kk for kk in range(CK)], NPRE)
            wt = jnp.concatenate(
                [w_head(w, j, p, k0, CK) for p in range(2)], axis=1)
            acc = jnp.where(ch > 0, acc0_v[u], 0.0) + _dot(hp, wt)
            acc0_v[u] = acc
            for p in range(2):
                pre_v[w, j, p] = _pk(acc[:, blk(p)])
        return carry

    lax.fori_loop(0, NCH, chunk_body, 0)

    def ln1(x, sg):
        h = _layernorm(x.astype(F32)[8:SEG]) * mod_row(1) + mod_row(0)
        for k in range(KD):
            lhs_v[sg, k, 0:8, :] = _pk(h[0:16, blk(k)])
            hs_v[sg, k] = h[16:24, blk(k)]

    def ln1_seg(seg, sg):
        ln1(x_v[seg], sg)

    def first_lhs():
        ln1(x0_v[...], 0)
        mem0 = mem0_v[...].astype(F32)
        for k in range(KD):
            lhs_v[0, k, 8:16, :] = _pk(jnp.concatenate(
                [hs_v[0, k], mem0[:, blk(k)]], axis=0))

    def pre_dot(j, w, p):
        hp = _cat_pk(hpre_v, range(KD), NPRE)
        pre_v[w, j, p] = _pk(_dot(hp, w_head(w, j, p)))

    wait_unit(j1, 1)
    mem0_copy.wait()
    x0_copy.wait()
    wo_copy.start()
    x_copy.start()
    for cp in late_mod + ffn_copies:
        cp.start()
    relayout(j1, 1)

    def pre_body(j, carry):
        wait_unit(j, 2)
        wait_unit(j + 1, 0)
        wait_unit(j + 1, 1)

        for (dj, dw), (rj, rw) in (((j, 1), (j, 2)), ((j, 2), (j + 1, 0)),
                                   ((j + 1, 0), (j + 1, 1))):
            pre_dot(dj, dw, 0)
            relayout(rj, rw)
            pre_dot(dj, dw, 1)
        first_lhs()
        return carry

    lax.fori_loop(j1, NJ - 1, pre_body, 0)

    L2 = 2 * L
    rr = lax.broadcasted_iota(jnp.int32, (L2, L2), 0)
    cc = lax.broadcasted_iota(jnp.int32, (L2, L2), 1)
    same = (rr >= L) == (cc >= L)
    rr = jnp.where(rr >= L, rr - L, rr)
    cc = jnp.where(cc >= L, cc - L, cc)
    mask = same & ((rr >= SEG) | (cc >= SEG) | (cc <= rr))
    fill_val = jnp.where(same, -1000000000.0, -jnp.inf).astype(F32)

    def scores(q, k):
        s = lax.dot_general(q, k, (((1,), (1,)), ((), ())),
                            preferred_element_type=F32)
        s = jnp.where(mask, s * scale, fill_val)
        m = jnp.max(s, axis=-1, keepdims=True)
        e = jnp.exp(s - m)
        p = e * _recip(jnp.sum(e, axis=-1, keepdims=True))
        return p.astype(BF16)

    def ln2(xs, hs=0):
        h = _layernorm(x1_v[xs]) * mod_row(4) + mod_row(3)
        for k in range(KD):
            h2_v[hs, k, 0:PAIR // 2, :] = _pk(h[:, blk(k)])

    def up_half(hf, f, hs, dst):
        h2 = _cat_pk(h2_v.at[hs], range(KD), PAIR)
        g = _dot(h2, _unpk(w1_v[hf, :, blk(f)]))
        u = _dot(h2, _unpk(w3_v[hf, :, blk(f)]))
        act_v[dst, 0:PAIR // 2, :] = _pk(_silu(g) * u)

    def up(f):
        up_half(f // NH, f % NH, 0, f)

    def down(xs, j, hf):
        a = _cat_pk(act_v, range(hf * NH, (hf + 1) * NH), PAIR)
        y = _dot(a, _unpk(w2_v[hf, :, blk(j)]))
        if hf == 0:
            yh_v[:, blk(j)] = y
        else:
            y = y + yh_v[:, blk(j)]
            stage_v[xs, :, blk(j)] = (
                x1_v[xs, :, blk(j)] + mod_blk(5, j) * y).astype(BF16)

    def segment(i, sg, fill, finish):
        o_v = ob_v if sg else oa_v
        rows = L + 8 if sg else SEG
        prow = pl.multiple_of(i * 8, 8)
        qk, vs, ps = {}, {}, {}

        def proj(g):
            r = []
            for w in range(3):
                parts = []
                for p in range(2):
                    lhs = _cat_pk(lhs_v.at[sg], range(KD), SEG)
                    pre = _unpk(pre_v[w, g, p, pl.ds(prow, 8), :]).astype(F32)
                    parts += [pre[8 * sg:8 * sg + 8],
                              _dot(lhs, w_head(w, g, p))]
                r.append(jnp.concatenate(parts, axis=0).astype(BF16))
            qk[g] = r[0:2]
            vs[g] = r[2]

        def pv(g):
            o2 = _dot(ps.pop(g), vs.pop(g))
            for p in range(2):
                h = 2 * g + p
                o = o2[p * L:(p + 1) * L]
                if sg == 0:
                    o_v[h, 0:16, :] = _pk(
                        jnp.concatenate([o[0:24], o[SEG:L]], axis=0))
                    so_v[h] = o[24:SEG]
                else:
                    o_v[h] = _pk(jnp.concatenate([so_v[h], o], axis=0))

        def wo_part(hs, j):
            lo, hi = hs[0] * (LANE // 2), (hs[-1] + 1) * (LANE // 2)
            return _dot(_cat_pk(o_v, hs, rows), _unpk(wo_v[lo:hi, blk(j)]))

        def wo_head(j):
            between = fill.get(("head", j))
            if between is None:
                acc_v[j, 0:rows, :] = wo_part(head_hs, j)
                return
            half = len(head_hs) // 2
            acc_v[j, 0:rows, :] = wo_part(head_hs[:half], j)
            between[0]()
            acc_v[j, 0:rows, :] += wo_part(head_hs[half:], j)
            for fn in between[1:]:
                fn()

        head_hs = list(range(H - TAIL))
        tail_hs = list(range(H - TAIL, H))
        cuts = (0,) + WO_AT
        wo_at = {NJ + t: range(cuts[t], cuts[t + 1]) for t in range(LP)}
        for g in range(NJ + LP):
            if g < NJ:
                proj(g)
            for j in wo_at.get(g, ()):
                wo_head(j)
            if LS <= g < NJ + LS:
                ps[g - LS] = scores(*qk.pop(g - LS))
            if g >= LP:
                pv(g - LP)
            for fn in fill.get(g, ()):
                fn()
        for j in range(WO_AT[-1], KD):
            wo_head(j)
        for j in range(KD):
            finish(j, acc_v[j, 0:rows, :] + wo_part(tail_hs, j))
        for fn in fill.get(NJ + LP, ()):
            fn()

    def attn_pair(i, fill_a, fill_b):
        xs = i % 2

        def finish_a(j, y):
            ya_v[j] = y[0:24]
            lhs_v[1, j, 8:16, :] = _pk(
                jnp.concatenate([hs_v[1, j], y[24:SEG]], axis=0))

        def finish_b(j, y):
            att = jnp.concatenate([ya_v[j], y[0:L]], axis=0)
            x = x_v[pl.ds(2 * i, 2), :, blk(j)].astype(F32).reshape(PAIR, LANE)
            x1_v[xs, :, blk(j)] = x + mod_blk(2, j) * att
            lhs_v[0, j, 8:16, :] = _pk(
                jnp.concatenate([hs_v[0, j], y[L:L + 8]], axis=0))

        segment(i, 0, fill_a, finish_a)
        segment(i, 1, fill_b, finish_b)

    P = functools.partial

    wait_unit(NJ - 1, 2)
    x_copy.wait()
    for cp in late_mod:
        cp.wait()
    wo_copy.wait()

    def head_body(i, carry):
        def piece(n):
            m, w, p = n // 4, 1 + n % 4 // 2, n % 2
            r0 = pl.multiple_of(i * (NPRE // 4) + m * 32, 32)
            hp = jnp.concatenate(
                [_unpk(hpre_v[k, pl.ds(r0, 32), :]) for k in range(KD)], axis=1)
            pre_v[w, NJ - 1, p, pl.ds(r0, 32), :] = _pk(
                _dot(hp, w_head(w, NJ - 1, p)))

        def late_mod_col(n):
            r = _dot(sc, _unpk(wml_v[i, :, blk(n)]))[0:8]
            if n < KD:
                r = r + i.astype(F32)
            mod_v[2 * KD * (1 + i) + n] = r

        fill_a = {0: [P(relayout, NJ - 1, 2, i == 0)],
                  2: [P(ln1_seg, 2 * i + 1, 1)]}
        fill_b = {8: [P(ln1_seg, 2 * i + 2, 0)]}
        for j in range(KD):
            fill_b[("head", j)] = [P(late_mod_col, 2 * j + t) for t in range(2)]
        fill_b[("head", KD // 2)].append(P(ln2, 1 - i))
        for n, g in enumerate(HEAD_A):
            fill_a.setdefault(g, []).append(P(piece, n))
        for n, g in enumerate(HEAD_B):
            fill_b.setdefault(g, []).append(P(piece, len(HEAD_A) + n))
        attn_pair(i, fill_a, fill_b)
        return carry

    lax.fori_loop(0, 2, head_body, 0)
    for cp in ffn_copies:
        cp.wait()
    for f in range(NU0):
        up(f)

    def body(i, carry):
        slot = i % 2

        @pl.when(i >= 4)
        def _():
            out_copy(i - 4, slot).wait()

        fill_a, fill_b = {}, {}
        for f in range(NU0, NF):
            fill_a.setdefault((f - NU0) * NJ // (NF - NU0), []).append(P(up, f))
        downs = [P(down, slot, j, hf) for j in range(KD) for hf in range(2)]
        fill_a[NJ + LP] = downs[0:1]
        for n, fn in enumerate(downs[1:]):
            fill_b.setdefault(n, []).append(fn)
        fill_b.setdefault(2, []).append(P(ln2, 1 - slot))
        fill_a.setdefault(2, []).append(P(ln1_seg, 2 * i + 1, 1))
        fill_b.setdefault(8, []).append(
            P(ln1_seg, jnp.minimum(2 * i + 2, NSEG - 1), 0))
        fill_b.setdefault(NJ + LP - 1, []).append(P(up, 0))
        fill_b[NJ + LP] = [P(up, f) for f in range(1, NU0)]
        attn_pair(i, fill_a, fill_b)
        out_copy(i - 2, slot).start()
        return carry

    lax.fori_loop(2, NP, body, 0)

    out_copy(NP - 4, NP % 2).wait()

    def tail_body(q, carry):
        t, hf = q // 2, q % 2
        xs = (NP + t) % 2

        @pl.when(q == 2)
        def _():
            out_copy(NP - 3, xs).wait()

        for f in range(NH):
            up_half(hf, f, t, f)
        ln2((NP + 1) % 2, 1)
        for j in range(KD):
            y = _dot(_cat_pk(act_v, range(NH), PAIR),
                     _unpk(w2_v[hf, :, blk(j)]))
            y = y + jnp.where(hf == 1, yh_v[:, blk(j)], 0.0)
            yh_v[:, blk(j)] = y
            stage_v[xs, :, blk(j)] = (
                x1_v[xs, :, blk(j)] + mod_blk(5, j) * y).astype(BF16)

        @pl.when(hf == 1)
        def _():
            out_copy(NP - 2 + t, xs).start()

        return carry

    lax.fori_loop(0, 4, tail_body, 0)
    out_copy(NP - 2, NP % 2).wait()
    out_copy(NP - 1, (NP + 1) % 2).wait()


@functools.partial(jax.jit, static_argnames=("A_seg_len",))
def pallas_adaLN_cond__memory_aug_recurrent_mem_tr__glu_gated_swiglu__prompt_kernel(
    A_x: jax.Array,
    A_mem0: jax.Array,
    A_Wq: jax.Array,
    A_Wk: jax.Array,
    A_Wv: jax.Array,
    A_Wo: jax.Array,
    A_seg_len,
    B_x: jax.Array,
    B_w1: jax.Array,
    B_w3: jax.Array,
    B_w2: jax.Array,
    c: jax.Array,
    w_mod: jax.Array,
):
    B, S, D = A_x.shape
    H, Dh = A_Wq.shape[1], A_Wq.shape[2]
    F = B_w1.shape[1]
    assert B == 1 and Dh == LANE and A_seg_len == SEG and A_mem0.shape[1] == MEM
    assert (S, D, H) == (2048, 1024, 32) and F % (2 * LANE) == 0
    KD, NF = D // LANE, F // LANE
    NSEG = S // SEG

    def split(w):
        return w.reshape(D // 16, 16, H // 2, 2, Dh)

    any_spec = pl.BlockSpec(memory_space=pl.ANY)
    out = pl.pallas_call(
        functools.partial(_kernel, S=S, D=D, H=H, F=F),
        out_shape=jax.ShapeDtypeStruct((S, D), A_x.dtype),
        in_specs=[any_spec] * 11,
        out_specs=any_spec,
        scratch_shapes=[
            pltpu.VMEM((1, D), BF16),
            pltpu.VMEM((MEM, D), BF16),
            pltpu.VMEM((SEG, D), BF16),
            pltpu.VMEM((NSEG, SEG, D), BF16),
            pltpu.VMEM((NSEG, 8, D), BF16),
            pltpu.VMEM((KD, NSEG * 8, LANE), F32),
            pltpu.VMEM((KD, NSEG * 4 + 8, LANE), U32),
            pltpu.VMEM((NU_FIRST, NSEG * 8, 2 * LANE), F32),
            pltpu.VMEM((3, H // 2, 2, NSEG * 4, LANE), U32),
            pltpu.VMEM((H // 2, D // 16, 16, LANE), U32),
            pltpu.VMEM((H // 2, D // 16, 16, LANE), U32),
            pltpu.VMEM((H // 2, D // 16, 16, LANE), U32),
            pltpu.VMEM((H * Dh // 2, D + LANE), U32),
            pltpu.VMEM((2, D // 2, F // 2 + LANE), U32),
            pltpu.VMEM((2, D // 2, F // 2 + LANE), U32),
            pltpu.VMEM((2, F // 4, D + LANE), U32),
            pltpu.VMEM((4, 2, D // 2, D // 4), U32),
            pltpu.VMEM((2, D // 2, 2 * D), U32),
            pltpu.VMEM((6 * KD, 8, LANE), F32),
            pltpu.VMEM((2, KD, 8, LANE), F32),
            pltpu.VMEM((2, KD, 24, LANE), U32),
            pltpu.VMEM((H, 8, LANE), F32),
            pltpu.VMEM((H, 24, LANE), U32),
            pltpu.VMEM((H, 24, LANE), U32),
            pltpu.VMEM((KD, 48, LANE), F32),
            pltpu.VMEM((KD, 24, LANE), F32),
            pltpu.VMEM((2, PAIR, D), F32),
            pltpu.VMEM((2, KD, PAIR // 2 + 8, LANE), U32),
            pltpu.VMEM((NF, PAIR // 2 + 8, LANE), U32),
            pltpu.VMEM((PAIR, D), F32),
            pltpu.VMEM((2, PAIR, D), BF16),
            pltpu.SemaphoreType.DMA((4,)),
            pltpu.SemaphoreType.DMA((4,)),
            pltpu.SemaphoreType.DMA((5,)),
            pltpu.SemaphoreType.DMA((3 * H // 2,)),
            pltpu.SemaphoreType.DMA((2,)),
            pltpu.SemaphoreType.DMA((2,)),
        ],
        compiler_params=pltpu.CompilerParams(
            vmem_limit_bytes=110 * 1024 * 1024,
            disable_bounds_checks=True,
            disable_semaphore_checks=True),
        name="rmt_block",
    )(A_x.reshape(NSEG, SEG, D), A_mem0.reshape(MEM, D), split(A_Wq),
      split(A_Wk), split(A_Wv), A_Wo.reshape(H * Dh, D), B_w1, B_w3, B_w2, c,
      w_mod)
    return out.reshape(B, S, D)
```

```python
import functools

import jax
import jax.numpy as jnp
from jax import lax
import jax.experimental.pallas as pl
import jax.experimental.pallas.tpu as pltpu

F32 = jnp.float32
BF16 = jnp.bfloat16
U32 = jnp.uint32

LANE = 128
SEG = 32
MEM = 8
PAIR = 2 * SEG
EPS = 1e-5

LS, LP = 1, 3
TAIL = 8
WO_AT = (2, 4, 6)
HEAD_A = (1, 3, 5, 7, 9, 11, 13, 19)
HEAD_B = (1, 3, 6, 9, 12, 18, 19, 19)
NU_FIRST = 7
NU0 = 3


def _dot(a, b):
    return jnp.dot(a, b, preferred_element_type=F32)


def _layernorm(x):
    m = jnp.mean(x, axis=-1, keepdims=True)
    xc = x - m
    v = jnp.mean(xc * xc, axis=-1, keepdims=True)
    return xc * lax.rsqrt(v + EPS)


def _silu(x):
    hx = 0.5 * x
    return hx + hx * jnp.tanh(hx)


def _recip(x):
    r = pl.reciprocal(x, approx=True)
    return r * (2.0 - x * r)


def _pk(x):
    return pltpu.bitcast(x.astype(BF16), U32)


def _unpk(x):
    return pltpu.bitcast(x, BF16)


def _cat_pk(ref, ks, rows):
    return jnp.concatenate(
        [_unpk(ref[k, 0:rows // 2, :]) for k in ks], axis=1)


def _kernel(x_hbm, mem0_hbm, wq_hbm, wk_hbm, wv_hbm, wo_hbm, w1_hbm, w3_hbm,
            w2_hbm, c_hbm, wmod_hbm, out_hbm,
            c_v, mem0_v, x0_v, x_v, xpre_v, xn_v, hpre_v, acc0_v, pre_v, cur_v,
            wq_v, wk_v, wv_v, wo_v, w1_v, w3_v, w2_v, wme_v, wml_v,
            mod_v, hs_v, lhs_v, so_v, oa_v, ob_v, acc_v, ya_v,
            x1_v, h2_v, act_v, yh_v, stage_v,
            sem_x, sem_xp, sem_mod, sem_qkv, sem_w, sem_out,
            *, S, D, H, F):
    KD = D // LANE
    NF = F // LANE
    NP = S // PAIR
    NSEG = S // SEG
    NJ = H // 2
    NPRE = NSEG * 8
    L = SEG + MEM
    scale = float(LANE) ** -0.5
    w_hbm = (wq_hbm, wk_hbm, wv_hbm)
    w_v = (wq_v, wk_v, wv_v)

    def blk(j):
        return slice(j * LANE, (j + 1) * LANE)

    NCH = 4
    CK = KD // NCH

    def early_mod(ch):
        return [pltpu.make_async_copy(
            wmod_hbm.bitcast(U32).at[:, pl.ds(
                pl.multiple_of(t * D + ch * (CK * LANE), LANE), CK * LANE)],
            wme_v.at[ch, t], sem_mod.at[ch]) for t in range(2)]

    late_mod = [pltpu.make_async_copy(
        wmod_hbm.bitcast(U32).at[:, pl.ds((2 + 2 * t) * D, 2 * D)],
        wml_v.at[t], sem_mod.at[NCH]) for t in range(2)]

    def unit_copy(j, w):
        return pltpu.make_async_copy(
            w_hbm[w].bitcast(U32).at[:, :, j, 0, :],
            w_v[w].at[j], sem_qkv.at[3 * j + w])

    def start_unit(j, w):
        unit_copy(j, w).start()

    def wait_unit(j, w):
        unit_copy(j, w).wait()

    first_units = [(u // 3, u % 3) for u in range(NU_FIRST)]

    def slice_copies(ch):
        rows = pl.ds(ch * (CK * 8), CK * 8)
        return [pltpu.make_async_copy(
            w_hbm[w].bitcast(U32).at[rows, :, j, 0, :], w_v[w].at[j, rows],
            sem_mod.at[ch]) for j, w in first_units]

    wo_copy = pltpu.make_async_copy(
        wo_hbm.bitcast(U32), wo_v.at[:, pl.ds(0, D)], sem_w.at[0])
    FH = F // 2
    NH = NF // 2
    ffn_copies = []
    for hf in range(2):
        for src, dst in ((w1_hbm, w1_v), (w3_hbm, w3_v)):
            ffn_copies.append(pltpu.make_async_copy(
                src.bitcast(U32).at[:, pl.ds(hf * FH, FH)],
                dst.at[hf, :, pl.ds(0, FH)], sem_w.at[1]))
    for hf in range(2):
        ffn_copies.append(pltpu.make_async_copy(
            w2_hbm.bitcast(U32).at[pl.ds(hf * FH // 2, FH // 2), :],
            w2_v.at[hf, :, pl.ds(0, D)], sem_w.at[1]))
    c_copy = pltpu.make_async_copy(c_hbm, c_v, sem_x.at[2])
    mem0_copy = pltpu.make_async_copy(mem0_hbm, mem0_v, sem_x.at[3])
    x_copy = pltpu.make_async_copy(x_hbm, x_v, sem_x.at[1])
    x0_copy = pltpu.make_async_copy(x_hbm.at[0], x0_v, sem_x.at[0])
    NXP = 4
    XS = NSEG // NXP

    def xpre_copy(b):
        return pltpu.make_async_copy(
            x_hbm.at[pl.ds(b * XS, XS), pl.ds(0, 8), :],
            xpre_v.at[pl.ds(b * XS, XS)], sem_xp.at[b])

    def out_copy(i, slot):
        return pltpu.make_async_copy(
            stage_v.at[slot], out_hbm.at[pl.ds(i * PAIR, PAIR), :],
            sem_out.at[slot])

    def start_units(j0, j1):
        def step(j, carry):
            for w in range(3):
                start_unit(j, w)
            return carry

        lax.fori_loop(j0, j1, step, 0)

    j1 = NU_FIRST // 3
    for b in range(NXP):
        xpre_copy(b).start()
    c_copy.start()

    def start_chunk(ch, carry):
        for cp in early_mod(ch) + slice_copies(ch):
            cp.start()
        return carry

    lax.fori_loop(0, NCH, start_chunk, 0)
    mem0_copy.start()
    x0_copy.start()
    start_unit(j1, 1)
    start_unit(j1, 2)
    start_units(j1 + 1, j1 + 7)
    x1_v[1] = jnp.zeros((PAIR, D), F32)
    mod_v[3 * KD:5 * KD] = jnp.zeros((2 * KD, 8, LANE), F32)

    def ln_pre(b, carry):
        @pl.when(b % (XS // 8) == 0)
        def _():
            xpre_copy(b // (XS // 8)).wait()

        x = xpre_v[pl.ds(b * 8, 8)].astype(F32).reshape(64, D)
        xn = _layernorm(x)
        r0 = pl.multiple_of(b * 64, 64)
        for k in range(KD):
            xn_v[k, pl.ds(r0, 64), :] = xn[:, blk(k)]
        return carry

    lax.fori_loop(0, NSEG // 8, ln_pre, 0)

    def relayout_rows(j, w, r, do=None):
        rows = pl.ds(r, 8)
        a = w_v[w][j, rows, pl.ds(0, 8, stride=2), :]
        b = w_v[w][j, rows, pl.ds(1, 8, stride=2), :]
        lo = (a & U32(0xFFFF)) | (b << 16)
        hi = (a >> 16) | (b & U32(0xFFFF0000))
        if do is not None:
            lo = jnp.where(do, lo, w_v[w][j, rows, 0:8, :])
            hi = jnp.where(do, hi, w_v[w][j, rows, 8:16, :])
        w_v[w][j, rows, 0:8, :] = lo
        w_v[w][j, rows, 8:16, :] = hi

    def relayout(j, w, do=None):
        for k in range(KD):
            relayout_rows(j, w, k * 8, do)

    def w_head(w, j, p, k0=0, nk=KD):
        t = w_v[w][j, pl.ds(k0 * 8, nk * 8), 8 * p:8 * p + 8, :]
        return _unpk(t.reshape(nk * LANE // 2, LANE))

    c_copy.wait()
    start_units(j1 + 7, NJ)

    c = c_v[...].astype(F32)
    sc = _silu(c).astype(BF16)
    sc = jnp.broadcast_to(sc, (16, D))

    def mod_row(k):
        return jnp.concatenate([mod_blk(k, j) for j in range(KD)], axis=1)

    def mod_blk(k, j):
        return mod_v[k * KD + j, 0:1, :]

    def chunk_body(ch, carry):
        for cp in early_mod(ch) + slice_copies(ch):
            cp.wait()
        k0 = ch * CK
        for kk in range(CK):
            sa = _dot(sc, _unpk(wme_v[ch, 0, :, blk(kk)]))[0:8]
            ca = _dot(sc, _unpk(wme_v[ch, 1, :, blk(kk)]))[0:8] + 1.0
            mod_v[k0 + kk] = sa
            mod_v[KD + k0 + kk] = ca
            for r in range(0, NSEG * 8, 128):
                hpre_v[k0 + kk, r // 2:r // 2 + 64, :] = _pk(
                    xn_v[k0 + kk, r:r + 128, :] * ca[0:1] + sa[0:1])
        for u, (j, w) in enumerate(first_units):
            for kk in range(CK):
                relayout_rows(j, w, (k0 + kk) * 8)
            hp = _cat_pk(hpre_v, [k0 + kk for kk in range(CK)], NPRE)
            wt = jnp.concatenate(
                [w_head(w, j, p, k0, CK) for p in range(2)], axis=1)
            acc = jnp.where(ch > 0, acc0_v[u], 0.0) + _dot(hp, wt)
            acc0_v[u] = acc
            for p in range(2):
                pre_v[w, j, p] = _pk(acc[:, blk(p)])
        return carry

    lax.fori_loop(0, NCH, chunk_body, 0)

    def ln1(x, sg):
        h = _layernorm(x.astype(F32)[8:SEG]) * mod_row(1) + mod_row(0)
        for k in range(KD):
            lhs_v[sg, k, 0:8, :] = _pk(h[0:16, blk(k)])
            hs_v[sg, k] = h[16:24, blk(k)]

    def ln1_seg(seg, sg):
        ln1(x_v[seg], sg)

    def first_lhs():
        ln1(x0_v[...], 0)
        mem0 = mem0_v[...].astype(F32)
        for k in range(KD):
            lhs_v[0, k, 8:16, :] = _pk(jnp.concatenate(
                [hs_v[0, k], mem0[:, blk(k)]], axis=0))

    def pre_dot(j, w, p):
        hp = _cat_pk(hpre_v, range(KD), NPRE)
        pre_v[w, j, p] = _pk(_dot(hp, w_head(w, j, p)))

    wait_unit(j1, 1)
    mem0_copy.wait()
    x0_copy.wait()
    wo_copy.start()
    x_copy.start()
    for cp in late_mod + ffn_copies:
        cp.start()
    relayout(j1, 1)

    def pre_body(j, carry):
        wait_unit(j, 2)
        wait_unit(j + 1, 0)
        wait_unit(j + 1, 1)

        for (dj, dw), (rj, rw) in (((j, 1), (j, 2)), ((j, 2), (j + 1, 0)),
                                   ((j + 1, 0), (j + 1, 1))):
            pre_dot(dj, dw, 0)
            relayout(rj, rw)
            pre_dot(dj, dw, 1)
        first_lhs()
        return carry

    lax.fori_loop(j1, NJ - 1, pre_body, 0)

    L2 = 2 * L
    rr = lax.broadcasted_iota(jnp.int32, (L2, L2), 0)
    cc = lax.broadcasted_iota(jnp.int32, (L2, L2), 1)
    same = (rr >= L) == (cc >= L)
    rr = jnp.where(rr >= L, rr - L, rr)
    cc = jnp.where(cc >= L, cc - L, cc)
    mask = same & ((rr >= SEG) | (cc >= SEG) | (cc <= rr))
    fill_val = jnp.where(same, -1000000000.0, -jnp.inf).astype(F32)

    def scores(q, k):
        s = lax.dot_general(q, k, (((1,), (1,)), ((), ())),
                            preferred_element_type=F32)
        s = jnp.where(mask, s * scale, fill_val)
        m = jnp.max(s, axis=-1, keepdims=True)
        e = jnp.exp(s - m)
        p = e * _recip(jnp.sum(e, axis=-1, keepdims=True))
        return p.astype(BF16)

    def ln2(xs, hs=0):
        h = _layernorm(x1_v[xs]) * mod_row(4) + mod_row(3)
        for k in range(KD):
            h2_v[hs, k, 0:PAIR // 2, :] = _pk(h[:, blk(k)])

    def up_half(hf, f, hs, dst):
        h2 = _cat_pk(h2_v.at[hs], range(KD), PAIR)
        g = _dot(h2, _unpk(w1_v[hf, :, blk(f)]))
        u = _dot(h2, _unpk(w3_v[hf, :, blk(f)]))
        act_v[dst, 0:PAIR // 2, :] = _pk(_silu(g) * u)

    def up(f):
        up_half(f // NH, f % NH, 0, f)

    def down(xs, j, hf):
        a = _cat_pk(act_v, range(hf * NH, (hf + 1) * NH), PAIR)
        y = _dot(a, _unpk(w2_v[hf, :, blk(j)]))
        if hf == 0:
            yh_v[:, blk(j)] = y
        else:
            y = y + yh_v[:, blk(j)]
            stage_v[xs, :, blk(j)] = (
                x1_v[xs, :, blk(j)] + mod_blk(5, j) * y).astype(BF16)

    def segment(i, sg, fill, finish):
        o_v = ob_v if sg else oa_v
        rows = L + 8 if sg else SEG
        prow = pl.multiple_of(i * 8, 8)
        qk, vs, ps = {}, {}, {}

        def proj(g):
            r = []
            for w in range(3):
                parts = []
                for p in range(2):
                    lhs = _cat_pk(lhs_v.at[sg], range(KD), SEG)
                    if sg == 0:
                        pre = pre_v[w, g, p, pl.ds(prow, 8), :]
                        cur_v[w, g, p] = pre
                    else:
                        pre = cur_v[w, g, p]
                    pre = _unpk(pre).astype(F32)
                    parts += [pre[8 * sg:8 * sg + 8],
                              _dot(lhs, w_head(w, g, p))]
                r.append(jnp.concatenate(parts, axis=0).astype(BF16))
            qk[g] = r[0:2]
            vs[g] = r[2]

        def pv(g):
            o2 = _dot(ps.pop(g), vs.pop(g))
            for p in range(2):
                h = 2 * g + p
                o = o2[p * L:(p + 1) * L]
                if sg == 0:
                    o_v[h, 0:16, :] = _pk(
                        jnp.concatenate([o[0:24], o[SEG:L]], axis=0))
                    so_v[h] = o[24:SEG]
                else:
                    o_v[h] = _pk(jnp.concatenate([so_v[h], o], axis=0))

        def wo_part(hs, j):
            lo, hi = hs[0] * (LANE // 2), (hs[-1] + 1) * (LANE // 2)
            return _dot(_cat_pk(o_v, hs, rows), _unpk(wo_v[lo:hi, blk(j)]))

        def wo_head(j):
            between = fill.get(("head", j))
            if between is None:
                acc_v[j, 0:rows, :] = wo_part(head_hs, j)
                return
            half = len(head_hs) // 2
            acc_v[j, 0:rows, :] = wo_part(head_hs[:half], j)
            between[0]()
            acc_v[j, 0:rows, :] += wo_part(head_hs[half:], j)
            for fn in between[1:]:
                fn()

        head_hs = list(range(H - TAIL))
        tail_hs = list(range(H - TAIL, H))
        cuts = (0,) + WO_AT
        wo_at = {NJ + t: range(cuts[t], cuts[t + 1]) for t in range(LP)}
        for g in range(NJ + LP):
            if g < NJ:
                proj(g)
            for j in wo_at.get(g, ()):
                wo_head(j)
            if LS <= g < NJ + LS:
                ps[g - LS] = scores(*qk.pop(g - LS))
            if g >= LP:
                pv(g - LP)
            for fn in fill.get(g, ()):
                fn()
        for j in range(WO_AT[-1], KD):
            wo_head(j)
        for j in range(KD):
            finish(j, acc_v[j, 0:rows, :] + wo_part(tail_hs, j))
        for fn in fill.get(NJ + LP, ()):
            fn()

    def attn_pair(i, fill_a, fill_b):
        xs = i % 2

        def finish_a(j, y):
            ya_v[j] = y[0:24]
            lhs_v[1, j, 8:16, :] = _pk(
                jnp.concatenate([hs_v[1, j], y[24:SEG]], axis=0))

        def finish_b(j, y):
            att = jnp.concatenate([ya_v[j], y[0:L]], axis=0)
            x = x_v[pl.ds(2 * i, 2), :, blk(j)].astype(F32).reshape(PAIR, LANE)
            x1_v[xs, :, blk(j)] = x + mod_blk(2, j) * att
            lhs_v[0, j, 8:16, :] = _pk(
                jnp.concatenate([hs_v[0, j], y[L:L + 8]], axis=0))

        segment(i, 0, fill_a, finish_a)
        segment(i, 1, fill_b, finish_b)

    P = functools.partial

    wait_unit(NJ - 1, 2)
    x_copy.wait()
    for cp in late_mod:
        cp.wait()
    wo_copy.wait()

    def head_body(i, carry):
        def piece(n):
            m, w, p = n // 4, 1 + n % 4 // 2, n % 2
            r0 = pl.multiple_of(i * (NPRE // 4) + m * 32, 32)
            hp = jnp.concatenate(
                [_unpk(hpre_v[k, pl.ds(r0, 32), :]) for k in range(KD)], axis=1)
            pre_v[w, NJ - 1, p, pl.ds(r0, 32), :] = _pk(
                _dot(hp, w_head(w, NJ - 1, p)))

        def late_mod_col(n):
            r = _dot(sc, _unpk(wml_v[i, :, blk(n)]))[0:8]
            if n < KD:
                r = r + i.astype(F32)
            mod_v[2 * KD * (1 + i) + n] = r

        fill_a = {0: [P(relayout, NJ - 1, 2, i == 0)],
                  2: [P(ln1_seg, 2 * i + 1, 1)]}
        fill_b = {8: [P(ln1_seg, 2 * i + 2, 0)]}
        for j in range(KD):
            fill_b[("head", j)] = [P(late_mod_col, 2 * j + t) for t in range(2)]
        fill_b[("head", KD // 2)].append(P(ln2, 1 - i))
        for n, g in enumerate(HEAD_A):
            fill_a.setdefault(g, []).append(P(piece, n))
        for n, g in enumerate(HEAD_B):
            fill_b.setdefault(g, []).append(P(piece, len(HEAD_A) + n))
        attn_pair(i, fill_a, fill_b)
        return carry

    lax.fori_loop(0, 2, head_body, 0)
    for cp in ffn_copies:
        cp.wait()
    for f in range(NU0):
        up(f)

    def body(i, carry):
        slot = i % 2

        @pl.when(i >= 4)
        def _():
            out_copy(i - 4, slot).wait()

        fill_a, fill_b = {}, {}
        for f in range(NU0, NF):
            fill_a.setdefault((f - NU0) * NJ // (NF - NU0), []).append(P(up, f))
        downs = [P(down, slot, j, hf) for j in range(KD) for hf in range(2)]
        fill_a[NJ + LP] = downs[0:1]
        for n, fn in enumerate(downs[1:]):
            fill_b.setdefault(n, []).append(fn)
        fill_b.setdefault(2, []).append(P(ln2, 1 - slot))
        fill_a.setdefault(2, []).append(P(ln1_seg, 2 * i + 1, 1))
        fill_b.setdefault(8, []).append(
            P(ln1_seg, jnp.minimum(2 * i + 2, NSEG - 1), 0))
        fill_b.setdefault(NJ + LP - 1, []).append(P(up, 0))
        fill_b[NJ + LP] = [P(up, f) for f in range(1, NU0)]
        attn_pair(i, fill_a, fill_b)
        out_copy(i - 2, slot).start()
        return carry

    lax.fori_loop(2, NP, body, 0)

    out_copy(NP - 4, NP % 2).wait()

    def tail_body(q, carry):
        t, hf = q // 2, q % 2
        xs = (NP + t) % 2

        @pl.when(q == 2)
        def _():
            out_copy(NP - 3, xs).wait()

        for f in range(NH):
            up_half(hf, f, t, f)
        ln2((NP + 1) % 2, 1)
        for j in range(KD):
            y = _dot(_cat_pk(act_v, range(NH), PAIR),
                     _unpk(w2_v[hf, :, blk(j)]))
            y = y + jnp.where(hf == 1, yh_v[:, blk(j)], 0.0)
            yh_v[:, blk(j)] = y
            stage_v[xs, :, blk(j)] = (
                x1_v[xs, :, blk(j)] + mod_blk(5, j) * y).astype(BF16)

        @pl.when(hf == 1)
        def _():
            out_copy(NP - 2 + t, xs).start()

        return carry

    lax.fori_loop(0, 4, tail_body, 0)
    out_copy(NP - 2, NP % 2).wait()
    out_copy(NP - 1, (NP + 1) % 2).wait()


@functools.partial(jax.jit, static_argnames=("A_seg_len",))
def pallas_adaLN_cond__memory_aug_recurrent_mem_tr__glu_gated_swiglu__prompt_kernel(
    A_x: jax.Array,
    A_mem0: jax.Array,
    A_Wq: jax.Array,
    A_Wk: jax.Array,
    A_Wv: jax.Array,
    A_Wo: jax.Array,
    A_seg_len,
    B_x: jax.Array,
    B_w1: jax.Array,
    B_w3: jax.Array,
    B_w2: jax.Array,
    c: jax.Array,
    w_mod: jax.Array,
):
    B, S, D = A_x.shape
    H, Dh = A_Wq.shape[1], A_Wq.shape[2]
    F = B_w1.shape[1]
    assert B == 1 and Dh == LANE and A_seg_len == SEG and A_mem0.shape[1] == MEM
    assert (S, D, H) == (2048, 1024, 32) and F % (2 * LANE) == 0
    KD, NF = D // LANE, F // LANE
    NSEG = S // SEG

    def split(w):
        return w.reshape(D // 16, 16, H // 2, 2, Dh)

    any_spec = pl.BlockSpec(memory_space=pl.ANY)
    out = pl.pallas_call(
        functools.partial(_kernel, S=S, D=D, H=H, F=F),
        out_shape=jax.ShapeDtypeStruct((S, D), A_x.dtype),
        in_specs=[any_spec] * 11,
        out_specs=any_spec,
        scratch_shapes=[
            pltpu.VMEM((1, D), BF16),
            pltpu.VMEM((MEM, D), BF16),
            pltpu.VMEM((SEG, D), BF16),
            pltpu.VMEM((NSEG, SEG, D), BF16),
            pltpu.VMEM((NSEG, 8, D), BF16),
            pltpu.VMEM((KD, NSEG * 8, LANE), F32),
            pltpu.VMEM((KD, NSEG * 4 + 8, LANE), U32),
            pltpu.VMEM((NU_FIRST, NSEG * 8, 2 * LANE), F32),
            pltpu.VMEM((3, H // 2, 2, NSEG * 4, LANE), U32),
            pltpu.VMEM((3, H // 2, 2, 8, LANE), U32),
            pltpu.VMEM((H // 2, D // 16, 16, LANE), U32),
            pltpu.VMEM((H // 2, D // 16, 16, LANE), U32),
            pltpu.VMEM((H // 2, D // 16, 16, LANE), U32),
            pltpu.VMEM((H * Dh // 2, D + LANE), U32),
            pltpu.VMEM((2, D // 2, F // 2 + LANE), U32),
            pltpu.VMEM((2, D // 2, F // 2 + LANE), U32),
            pltpu.VMEM((2, F // 4, D + LANE), U32),
            pltpu.VMEM((4, 2, D // 2, D // 4), U32),
            pltpu.VMEM((2, D // 2, 2 * D), U32),
            pltpu.VMEM((6 * KD, 8, LANE), F32),
            pltpu.VMEM((2, KD, 8, LANE), F32),
            pltpu.VMEM((2, KD, 24, LANE), U32),
            pltpu.VMEM((H, 8, LANE), F32),
            pltpu.VMEM((H, 24, LANE), U32),
            pltpu.VMEM((H, 24, LANE), U32),
            pltpu.VMEM((KD, 48, LANE), F32),
            pltpu.VMEM((KD, 24, LANE), F32),
            pltpu.VMEM((2, PAIR, D), F32),
            pltpu.VMEM((2, KD, PAIR // 2 + 8, LANE), U32),
            pltpu.VMEM((NF, PAIR // 2 + 8, LANE), U32),
            pltpu.VMEM((PAIR, D), F32),
            pltpu.VMEM((2, PAIR, D), BF16),
            pltpu.SemaphoreType.DMA((4,)),
            pltpu.SemaphoreType.DMA((4,)),
            pltpu.SemaphoreType.DMA((5,)),
            pltpu.SemaphoreType.DMA((3 * H // 2,)),
            pltpu.SemaphoreType.DMA((2,)),
            pltpu.SemaphoreType.DMA((2,)),
        ],
        compiler_params=pltpu.CompilerParams(
            vmem_limit_bytes=110 * 1024 * 1024,
            disable_bounds_checks=True,
            disable_semaphore_checks=True),
        name="rmt_block",
    )(A_x.reshape(NSEG, SEG, D), A_mem0.reshape(MEM, D), split(A_Wq),
      split(A_Wk), split(A_Wv), A_Wo.reshape(H * Dh, D), B_w1, B_w3, B_w2, c,
      w_mod)
    return out.reshape(B, S, D)
```

```python
import functools

import jax
import jax.numpy as jnp
from jax import lax
import jax.experimental.pallas as pl
import jax.experimental.pallas.tpu as pltpu

F32 = jnp.float32
BF16 = jnp.bfloat16
U32 = jnp.uint32

LANE = 128
SEG = 32
MEM = 8
PAIR = 2 * SEG
EPS = 1e-5

LS, LP = 1, 3
TAIL = 10
WO_AT = (1, 3, 5)
HEAD_A = (1, 3, 5, 7, 9, 11, 13, 19)
HEAD_B = (1, 3, 6, 9, 12, 18, 19, 19)
NU_FIRST = 7
NU0 = 1


def _dot(a, b):
    return jnp.dot(a, b, preferred_element_type=F32)


def _layernorm(x):
    m = jnp.mean(x, axis=-1, keepdims=True)
    xc = x - m
    v = jnp.mean(xc * xc, axis=-1, keepdims=True)
    return xc * lax.rsqrt(v + EPS)


def _silu(x):
    hx = 0.5 * x
    return hx + hx * jnp.tanh(hx)


def _recip(x):
    r = pl.reciprocal(x, approx=True)
    return r * (2.0 - x * r)


def _pk(x):
    return pltpu.bitcast(x.astype(BF16), U32)


def _unpk(x):
    return pltpu.bitcast(x, BF16)


def _cat_pk(ref, ks, rows):
    return jnp.concatenate(
        [_unpk(ref[k, 0:rows // 2, :]) for k in ks], axis=1)


def _kernel(x_hbm, mem0_hbm, wq_hbm, wk_hbm, wv_hbm, wo_hbm, w1_hbm, w3_hbm,
            w2_hbm, c_hbm, wmod_hbm, out_hbm,
            c_v, mem0_v, x0_v, x_v, xpre_v, xn_v, hpre_v, acc0_v, pre_v, cur_v,
            wq_v, wk_v, wv_v, wo_v, w1_v, w3_v, w2_v, wme_v, wml_v,
            mod_v, hs_v, lhs_v, so_v, oa_v, ob_v, acc_v, ya_v,
            x1_v, h2_v, act_v, yh_v, stage_v,
            sem_x, sem_xp, sem_mod, sem_qkv, sem_w, sem_out,
            *, S, D, H, F):
    KD = D // LANE
    NF = F // LANE
    NP = S // PAIR
    NSEG = S // SEG
    NJ = H // 2
    NPRE = NSEG * 8
    L = SEG + MEM
    scale = float(LANE) ** -0.5
    w_hbm = (wq_hbm, wk_hbm, wv_hbm)
    w_v = (wq_v, wk_v, wv_v)

    def blk(j):
        return slice(j * LANE, (j + 1) * LANE)

    NCH = 4
    CK = KD // NCH

    def early_mod(ch):
        return [pltpu.make_async_copy(
            wmod_hbm.bitcast(U32).at[:, pl.ds(
                pl.multiple_of(t * D + ch * (CK * LANE), LANE), CK * LANE)],
            wme_v.at[ch, t], sem_mod.at[ch]) for t in range(2)]

    late_mod = [pltpu.make_async_copy(
        wmod_hbm.bitcast(U32).at[:, pl.ds((2 + 2 * t) * D, 2 * D)],
        wml_v.at[t], sem_mod.at[NCH]) for t in range(2)]

    def unit_copy(j, w):
        return pltpu.make_async_copy(
            w_hbm[w].bitcast(U32).at[:, :, j, 0, :],
            w_v[w].at[j], sem_qkv.at[3 * j + w])

    def start_unit(j, w):
        unit_copy(j, w).start()

    def wait_unit(j, w):
        unit_copy(j, w).wait()

    first_units = [(u // 3, u % 3) for u in range(NU_FIRST)]

    def slice_copies(ch):
        rows = pl.ds(ch * (CK * 8), CK * 8)
        return [pltpu.make_async_copy(
            w_hbm[w].bitcast(U32).at[rows, :, j, 0, :], w_v[w].at[j, rows],
            sem_mod.at[ch]) for j, w in first_units]

    wo_copy = pltpu.make_async_copy(
        wo_hbm.bitcast(U32), wo_v.at[:, pl.ds(0, D)], sem_w.at[0])
    FH = F // 2
    NH = NF // 2
    ffn_copies = []
    for hf in range(2):
        for src, dst in ((w1_hbm, w1_v), (w3_hbm, w3_v)):
            ffn_copies.append(pltpu.make_async_copy(
                src.bitcast(U32).at[:, pl.ds(hf * FH, FH)],
                dst.at[hf, :, pl.ds(0, FH)], sem_w.at[1]))
    for hf in range(2):
        ffn_copies.append(pltpu.make_async_copy(
            w2_hbm.bitcast(U32).at[pl.ds(hf * FH // 2, FH // 2), :],
            w2_v.at[hf, :, pl.ds(0, D)], sem_w.at[1]))
    c_copy = pltpu.make_async_copy(c_hbm, c_v, sem_x.at[2])
    mem0_copy = pltpu.make_async_copy(mem0_hbm, mem0_v, sem_x.at[3])
    x_copy = pltpu.make_async_copy(x_hbm, x_v, sem_x.at[1])
    x0_copy = pltpu.make_async_copy(x_hbm.at[0], x0_v, sem_x.at[0])
    NXP = 4
    XS = NSEG // NXP

    def xpre_copy(b):
        return pltpu.make_async_copy(
            x_hbm.at[pl.ds(b * XS, XS), pl.ds(0, 8), :],
            xpre_v.at[pl.ds(b * XS, XS)], sem_xp.at[b])

    def out_copy(i, slot):
        return pltpu.make_async_copy(
            stage_v.at[slot], out_hbm.at[pl.ds(i * PAIR, PAIR), :],
            sem_out.at[slot])

    def start_units(j0, j1):
        def step(j, carry):
            for w in range(3):
                start_unit(j, w)
            return carry

        lax.fori_loop(j0, j1, step, 0)

    j1 = NU_FIRST // 3
    for b in range(NXP):
        xpre_copy(b).start()
    c_copy.start()

    def start_chunk(ch, carry):
        for cp in early_mod(ch) + slice_copies(ch):
            cp.start()
        return carry

    lax.fori_loop(0, NCH, start_chunk, 0)
    mem0_copy.start()
    x0_copy.start()
    start_unit(j1, 1)
    start_unit(j1, 2)
    start_units(j1 + 1, j1 + 7)
    x1_v[1] = jnp.zeros((PAIR, D), F32)
    mod_v[3 * KD:5 * KD] = jnp.zeros((2 * KD, 8, LANE), F32)

    def ln_pre(b, carry):
        @pl.when(b % (XS // 8) == 0)
        def _():
            xpre_copy(b // (XS // 8)).wait()

        x = xpre_v[pl.ds(b * 8, 8)].astype(F32).reshape(64, D)
        xn = _layernorm(x)
        r0 = pl.multiple_of(b * 64, 64)
        for k in range(KD):
            xn_v[k, pl.ds(r0, 64), :] = xn[:, blk(k)]
        return carry

    lax.fori_loop(0, NSEG // 8, ln_pre, 0)

    def relayout_rows(j, w, r, do=None):
        rows = pl.ds(r, 8)
        a = w_v[w][j, rows, pl.ds(0, 8, stride=2), :]
        b = w_v[w][j, rows, pl.ds(1, 8, stride=2), :]
        lo = (a & U32(0xFFFF)) | (b << 16)
        hi = (a >> 16) | (b & U32(0xFFFF0000))
        if do is not None:
            lo = jnp.where(do, lo, w_v[w][j, rows, 0:8, :])
            hi = jnp.where(do, hi, w_v[w][j, rows, 8:16, :])
        w_v[w][j, rows, 0:8, :] = lo
        w_v[w][j, rows, 8:16, :] = hi

    def relayout(j, w, do=None):
        for k in range(KD):
            relayout_rows(j, w, k * 8, do)

    def w_head(w, j, p, k0=0, nk=KD):
        t = w_v[w][j, pl.ds(k0 * 8, nk * 8), 8 * p:8 * p + 8, :]
        return _unpk(t.reshape(nk * LANE // 2, LANE))

    c_copy.wait()
    start_units(j1 + 7, NJ)

    c = c_v[...].astype(F32)
    sc = _silu(c).astype(BF16)
    sc = jnp.broadcast_to(sc, (16, D))

    def mod_row(k):
        return jnp.concatenate([mod_blk(k, j) for j in range(KD)], axis=1)

    def mod_blk(k, j):
        return mod_v[k * KD + j, 0:1, :]

    def chunk_body(ch, carry):
        for cp in early_mod(ch) + slice_copies(ch):
            cp.wait()
        k0 = ch * CK
        for kk in range(CK):
            sa = _dot(sc, _unpk(wme_v[ch, 0, :, blk(kk)]))[0:8]
            ca = _dot(sc, _unpk(wme_v[ch, 1, :, blk(kk)]))[0:8] + 1.0
            mod_v[k0 + kk] = sa
            mod_v[KD + k0 + kk] = ca
            for r in range(0, NSEG * 8, 128):
                hpre_v[k0 + kk, r // 2:r // 2 + 64, :] = _pk(
                    xn_v[k0 + kk, r:r + 128, :] * ca[0:1] + sa[0:1])
        for u, (j, w) in enumerate(first_units):
            for kk in range(CK):
                relayout_rows(j, w, (k0 + kk) * 8)
            hp = _cat_pk(hpre_v, [k0 + kk for kk in range(CK)], NPRE)
            wt = jnp.concatenate(
                [w_head(w, j, p, k0, CK) for p in range(2)], axis=1)
            acc = jnp.where(ch > 0, acc0_v[u], 0.0) + _dot(hp, wt)
            acc0_v[u] = acc
            for p in range(2):
                pre_v[w, j, p] = _pk(acc[:, blk(p)])
        return carry

    lax.fori_loop(0, NCH, chunk_body, 0)

    def ln1(x, sg):
        h = _layernorm(x.astype(F32)[8:SEG]) * mod_row(1) + mod_row(0)
        for k in range(KD):
            lhs_v[sg, k, 0:8, :] = _pk(h[0:16, blk(k)])
            hs_v[sg, k] = h[16:24, blk(k)]

    def ln1_seg(seg, sg):
        ln1(x_v[seg], sg)

    def first_lhs():
        ln1(x0_v[...], 0)
        mem0 = mem0_v[...].astype(F32)
        for k in range(KD):
            lhs_v[0, k, 8:16, :] = _pk(jnp.concatenate(
                [hs_v[0, k], mem0[:, blk(k)]], axis=0))

    def pre_dot(j, w, p):
        hp = _cat_pk(hpre_v, range(KD), NPRE)
        pre_v[w, j, p] = _pk(_dot(hp, w_head(w, j, p)))

    wait_unit(j1, 1)
    mem0_copy.wait()
    x0_copy.wait()
    wo_copy.start()
    x_copy.start()
    for cp in late_mod + ffn_copies:
        cp.start()
    relayout(j1, 1)

    def pre_body(j, carry):
        wait_unit(j, 2)
        wait_unit(j + 1, 0)
        wait_unit(j + 1, 1)

        for (dj, dw), (rj, rw) in (((j, 1), (j, 2)), ((j, 2), (j + 1, 0)),
                                   ((j + 1, 0), (j + 1, 1))):
            pre_dot(dj, dw, 0)
            relayout(rj, rw)
            pre_dot(dj, dw, 1)
        first_lhs()
        return carry

    lax.fori_loop(j1, NJ - 1, pre_body, 0)

    L2 = 2 * L
    rr = lax.broadcasted_iota(jnp.int32, (L2, L2), 0)
    cc = lax.broadcasted_iota(jnp.int32, (L2, L2), 1)
    same = (rr >= L) == (cc >= L)
    rr = jnp.where(rr >= L, rr - L, rr)
    cc = jnp.where(cc >= L, cc - L, cc)
    mask = same & ((rr >= SEG) | (cc >= SEG) | (cc <= rr))
    fill_val = jnp.where(same, -1000000000.0, -jnp.inf).astype(F32)

    def scores(q, k):
        s = lax.dot_general(q, k, (((1,), (1,)), ((), ())),
                            preferred_element_type=F32)
        s = jnp.where(mask, s * scale, fill_val)
        m = jnp.max(s, axis=-1, keepdims=True)
        e = jnp.exp(s - m)
        p = e * _recip(jnp.sum(e, axis=-1, keepdims=True))
        return p.astype(BF16)

    def ln2(xs, hs=0):
        h = _layernorm(x1_v[xs]) * mod_row(4) + mod_row(3)
        for k in range(KD):
            h2_v[hs, k, 0:PAIR // 2, :] = _pk(h[:, blk(k)])

    def up_half(hf, f, hs, dst):
        h2 = _cat_pk(h2_v.at[hs], range(KD), PAIR)
        g = _dot(h2, _unpk(w1_v[hf, :, blk(f)]))
        u = _dot(h2, _unpk(w3_v[hf, :, blk(f)]))
        act_v[dst, 0:PAIR // 2, :] = _pk(_silu(g) * u)

    def up(f):
        up_half(f // NH, f % NH, 0, f)

    def down(xs, j, hf):
        a = _cat_pk(act_v, range(hf * NH, (hf + 1) * NH), PAIR)
        y = _dot(a, _unpk(w2_v[hf, :, blk(j)]))
        if hf == 0:
            yh_v[:, blk(j)] = y
        else:
            y = y + yh_v[:, blk(j)]
            stage_v[xs, :, blk(j)] = (
                x1_v[xs, :, blk(j)] + mod_blk(5, j) * y).astype(BF16)

    def segment(i, sg, fill, finish):
        o_v = ob_v if sg else oa_v
        rows = L + 8 if sg else SEG
        prow = pl.multiple_of(i * 8, 8)
        qk, vs, ps = {}, {}, {}

        def proj(g):
            r = []
            for w in range(3):
                parts = []
                for p in range(2):
                    lhs = _cat_pk(lhs_v.at[sg], range(KD), SEG)
                    if sg == 0:
                        pre = pre_v[w, g, p, pl.ds(prow, 8), :]
                        cur_v[w, g, p] = pre
                    else:
                        pre = cur_v[w, g, p]
                    pre = _unpk(pre).astype(F32)
                    parts += [pre[8 * sg:8 * sg + 8],
                              _dot(lhs, w_head(w, g, p))]
                r.append(jnp.concatenate(parts, axis=0).astype(BF16))
            qk[g] = r[0:2]
            vs[g] = r[2]

        def pv(g):
            o2 = _dot(ps.pop(g), vs.pop(g))
            for p in range(2):
                h = 2 * g + p
                o = o2[p * L:(p + 1) * L]
                if sg == 0:
                    o_v[h, 0:16, :] = _pk(
                        jnp.concatenate([o[0:24], o[SEG:L]], axis=0))
                    so_v[h] = o[24:SEG]
                else:
                    o_v[h] = _pk(jnp.concatenate([so_v[h], o], axis=0))

        def wo_part(hs, j):
            lo, hi = hs[0] * (LANE // 2), (hs[-1] + 1) * (LANE // 2)
            return _dot(_cat_pk(o_v, hs, rows), _unpk(wo_v[lo:hi, blk(j)]))

        def wo_head(j):
            between = fill.get(("head", j))
            if between is None:
                acc_v[j, 0:rows, :] = wo_part(head_hs, j)
                return
            half = len(head_hs) // 2
            acc_v[j, 0:rows, :] = wo_part(head_hs[:half], j)
            between[0]()
            acc_v[j, 0:rows, :] += wo_part(head_hs[half:], j)
            for fn in between[1:]:
                fn()

        head_hs = list(range(H - TAIL))
        tail_hs = list(range(H - TAIL, H))
        cuts = (0,) + WO_AT
        wo_at = {NJ + t: range(cuts[t], cuts[t + 1]) for t in range(LP)}
        for g in range(NJ + LP):
            if g < NJ:
                proj(g)
            for j in wo_at.get(g, ()):
                wo_head(j)
            if LS <= g < NJ + LS:
                ps[g - LS] = scores(*qk.pop(g - LS))
            if g >= LP:
                pv(g - LP)
            for fn in fill.get(g, ()):
                fn()
        for j in range(WO_AT[-1], KD):
            wo_head(j)
        for j in range(KD):
            finish(j, acc_v[j, 0:rows, :] + wo_part(tail_hs, j))
        for fn in fill.get(NJ + LP, ()):
            fn()

    def attn_pair(i, fill_a, fill_b):
        xs = i % 2

        def finish_a(j, y):
            ya_v[j] = y[0:24]
            lhs_v[1, j, 8:16, :] = _pk(
                jnp.concatenate([hs_v[1, j], y[24:SEG]], axis=0))

        def finish_b(j, y):
            att = jnp.concatenate([ya_v[j], y[0:L]], axis=0)
            x = x_v[pl.ds(2 * i, 2), :, blk(j)].astype(F32).reshape(PAIR, LANE)
            x1_v[xs, :, blk(j)] = x + mod_blk(2, j) * att
            lhs_v[0, j, 8:16, :] = _pk(
                jnp.concatenate([hs_v[0, j], y[L:L + 8]], axis=0))

        segment(i, 0, fill_a, finish_a)
        segment(i, 1, fill_b, finish_b)

    P = functools.partial

    wait_unit(NJ - 1, 2)
    x_copy.wait()
    for cp in late_mod:
        cp.wait()
    wo_copy.wait()

    def head_body(i, carry):
        def piece(n):
            m, w, p = n // 4, 1 + n % 4 // 2, n % 2
            r0 = pl.multiple_of(i * (NPRE // 4) + m * 32, 32)
            hp = jnp.concatenate(
                [_unpk(hpre_v[k, pl.ds(r0, 32), :]) for k in range(KD)], axis=1)
            pre_v[w, NJ - 1, p, pl.ds(r0, 32), :] = _pk(
                _dot(hp, w_head(w, NJ - 1, p)))

        def late_mod_col(n):
            r = _dot(sc, _unpk(wml_v[i, :, blk(n)]))[0:8]
            if n < KD:
                r = r + i.astype(F32)
            mod_v[2 * KD * (1 + i) + n] = r

        fill_a = {0: [P(relayout, NJ - 1, 2, i == 0)],
                  2: [P(ln1_seg, 2 * i + 1, 1)]}
        fill_b = {8: [P(ln1_seg, 2 * i + 2, 0)]}
        for j in range(KD):
            fill_b[("head", j)] = [P(late_mod_col, 2 * j + t) for t in range(2)]
        fill_b[("head", KD // 2)].append(P(ln2, 1 - i))
        for n, g in enumerate(HEAD_A):
            fill_a.setdefault(g, []).append(P(piece, n))
        for n, g in enumerate(HEAD_B):
            fill_b.setdefault(g, []).append(P(piece, len(HEAD_A) + n))
        attn_pair(i, fill_a, fill_b)
        return carry

    lax.fori_loop(0, 2, head_body, 0)
    for cp in ffn_copies:
        cp.wait()
    for f in range(NU0):
        up(f)

    def body(i, carry):
        slot = i % 2

        @pl.when(i >= 4)
        def _():
            out_copy(i - 4, slot).wait()

        fill_a, fill_b = {}, {}
        for f in range(NU0, NF):
            fill_a.setdefault((f - NU0) * NJ // (NF - NU0), []).append(P(up, f))
        downs = [P(down, slot, j, hf) for j in range(KD) for hf in range(2)]
        fill_a[NJ + LP] = downs[0:1]
        for n, fn in enumerate(downs[1:]):
            fill_b.setdefault(n, []).append(fn)
        fill_b.setdefault(2, []).append(P(ln2, 1 - slot))
        fill_a.setdefault(2, []).append(P(ln1_seg, 2 * i + 1, 1))
        fill_b.setdefault(8, []).append(
            P(ln1_seg, jnp.minimum(2 * i + 2, NSEG - 1), 0))
        fill_b[NJ + LP] = [P(up, f) for f in range(NU0)]
        attn_pair(i, fill_a, fill_b)
        out_copy(i - 2, slot).start()
        return carry

    lax.fori_loop(2, NP, body, 0)

    out_copy(NP - 4, NP % 2).wait()

    def tail_body(q, carry):
        t, hf = q // 2, q % 2
        xs = (NP + t) % 2

        @pl.when(q == 2)
        def _():
            out_copy(NP - 3, xs).wait()

        for f in range(NH):
            up_half(hf, f, t, f)
        ln2((NP + 1) % 2, 1)
        for j in range(KD):
            y = _dot(_cat_pk(act_v, range(NH), PAIR),
                     _unpk(w2_v[hf, :, blk(j)]))
            y = y + jnp.where(hf == 1, yh_v[:, blk(j)], 0.0)
            yh_v[:, blk(j)] = y
            stage_v[xs, :, blk(j)] = (
                x1_v[xs, :, blk(j)] + mod_blk(5, j) * y).astype(BF16)

        @pl.when(hf == 1)
        def _():
            out_copy(NP - 2 + t, xs).start()

        return carry

    lax.fori_loop(0, 4, tail_body, 0)
    out_copy(NP - 2, NP % 2).wait()
    out_copy(NP - 1, (NP + 1) % 2).wait()


@functools.partial(jax.jit, static_argnames=("A_seg_len",))
def pallas_adaLN_cond__memory_aug_recurrent_mem_tr__glu_gated_swiglu__prompt_kernel(
    A_x: jax.Array,
    A_mem0: jax.Array,
    A_Wq: jax.Array,
    A_Wk: jax.Array,
    A_Wv: jax.Array,
    A_Wo: jax.Array,
    A_seg_len,
    B_x: jax.Array,
    B_w1: jax.Array,
    B_w3: jax.Array,
    B_w2: jax.Array,
    c: jax.Array,
    w_mod: jax.Array,
):
    B, S, D = A_x.shape
    H, Dh = A_Wq.shape[1], A_Wq.shape[2]
    F = B_w1.shape[1]
    assert B == 1 and Dh == LANE and A_seg_len == SEG and A_mem0.shape[1] == MEM
    assert (S, D, H) == (2048, 1024, 32) and F % (2 * LANE) == 0
    KD, NF = D // LANE, F // LANE
    NSEG = S // SEG

    def split(w):
        return w.reshape(D // 16, 16, H // 2, 2, Dh)

    any_spec = pl.BlockSpec(memory_space=pl.ANY)
    out = pl.pallas_call(
        functools.partial(_kernel, S=S, D=D, H=H, F=F),
        out_shape=jax.ShapeDtypeStruct((S, D), A_x.dtype),
        in_specs=[any_spec] * 11,
        out_specs=any_spec,
        scratch_shapes=[
            pltpu.VMEM((1, D), BF16),
            pltpu.VMEM((MEM, D), BF16),
            pltpu.VMEM((SEG, D), BF16),
            pltpu.VMEM((NSEG, SEG, D), BF16),
            pltpu.VMEM((NSEG, 8, D), BF16),
            pltpu.VMEM((KD, NSEG * 8, LANE), F32),
            pltpu.VMEM((KD, NSEG * 4 + 8, LANE), U32),
            pltpu.VMEM((NU_FIRST, NSEG * 8, 2 * LANE), F32),
            pltpu.VMEM((3, H // 2, 2, NSEG * 4, LANE), U32),
            pltpu.VMEM((3, H // 2, 2, 8, LANE), U32),
            pltpu.VMEM((H // 2, D // 16, 16, LANE), U32),
            pltpu.VMEM((H // 2, D // 16, 16, LANE), U32),
            pltpu.VMEM((H // 2, D // 16, 16, LANE), U32),
            pltpu.VMEM((H * Dh // 2, D + LANE), U32),
            pltpu.VMEM((2, D // 2, F // 2 + LANE), U32),
            pltpu.VMEM((2, D // 2, F // 2 + LANE), U32),
            pltpu.VMEM((2, F // 4, D + LANE), U32),
            pltpu.VMEM((4, 2, D // 2, D // 4), U32),
            pltpu.VMEM((2, D // 2, 2 * D), U32),
            pltpu.VMEM((6 * KD, 8, LANE), F32),
            pltpu.VMEM((2, KD, 8, LANE), F32),
            pltpu.VMEM((2, KD, 24, LANE), U32),
            pltpu.VMEM((H, 8, LANE), F32),
            pltpu.VMEM((H, 24, LANE), U32),
            pltpu.VMEM((H, 24, LANE), U32),
            pltpu.VMEM((KD, 48, LANE), F32),
            pltpu.VMEM((KD, 24, LANE), F32),
            pltpu.VMEM((2, PAIR, D), F32),
            pltpu.VMEM((2, KD, PAIR // 2 + 8, LANE), U32),
            pltpu.VMEM((NF, PAIR // 2 + 8, LANE), U32),
            pltpu.VMEM((PAIR, D), F32),
            pltpu.VMEM((2, PAIR, D), BF16),
            pltpu.SemaphoreType.DMA((4,)),
            pltpu.SemaphoreType.DMA((4,)),
            pltpu.SemaphoreType.DMA((5,)),
            pltpu.SemaphoreType.DMA((3 * H // 2,)),
            pltpu.SemaphoreType.DMA((2,)),
            pltpu.SemaphoreType.DMA((2,)),
        ],
        compiler_params=pltpu.CompilerParams(
            vmem_limit_bytes=110 * 1024 * 1024,
            disable_bounds_checks=True,
            disable_semaphore_checks=True),
        name="rmt_block",
    )(A_x.reshape(NSEG, SEG, D), A_mem0.reshape(MEM, D), split(A_Wq),
      split(A_Wk), split(A_Wv), A_Wo.reshape(H * Dh, D), B_w1, B_w3, B_w2, c,
      w_mod)
    return out.reshape(B, S, D)
```

```python
import functools

import jax
import jax.numpy as jnp
from jax import lax
import jax.experimental.pallas as pl
import jax.experimental.pallas.tpu as pltpu

F32 = jnp.float32
BF16 = jnp.bfloat16
U32 = jnp.uint32

LANE = 128
SEG = 32
MEM = 8
PAIR = 2 * SEG
EPS = 1e-5

LS, LP = 1, 3
WO_MAIN = (10, (1, 3, 5))
WO_HEAD = (8, (2, 4, 6))
HEAD_A = (1, 3, 5, 7, 9, 11, 13, 19)
HEAD_B = (1, 3, 6, 9, 12, 18, 19, 19)
NU_FIRST = 7
NU0 = 1


def _dot(a, b):
    return jnp.dot(a, b, preferred_element_type=F32)


def _layernorm(x):
    m = jnp.mean(x, axis=-1, keepdims=True)
    xc = x - m
    v = jnp.mean(xc * xc, axis=-1, keepdims=True)
    return xc * lax.rsqrt(v + EPS)


def _silu(x):
    hx = 0.5 * x
    return hx + hx * jnp.tanh(hx)


def _recip(x):
    r = pl.reciprocal(x, approx=True)
    return r * (2.0 - x * r)


def _pk(x):
    return pltpu.bitcast(x.astype(BF16), U32)


def _unpk(x):
    return pltpu.bitcast(x, BF16)


def _cat_pk(ref, ks, rows):
    return jnp.concatenate(
        [_unpk(ref[k, 0:rows // 2, :]) for k in ks], axis=1)


def _kernel(x_hbm, mem0_hbm, wq_hbm, wk_hbm, wv_hbm, wo_hbm, w1_hbm, w3_hbm,
            w2_hbm, c_hbm, wmod_hbm, out_hbm,
            c_v, mem0_v, x0_v, x_v, xpre_v, xn_v, hpre_v, acc0_v, pre_v, cur_v,
            wq_v, wk_v, wv_v, wo_v, w1_v, w3_v, w2_v, wme_v, wml_v,
            mod_v, hs_v, lhs_v, so_v, oa_v, ob_v, acc_v, ya_v,
            x1_v, h2_v, act_v, yh_v, stage_v,
            sem_x, sem_xp, sem_mod, sem_qkv, sem_w, sem_out,
            *, S, D, H, F):
    KD = D // LANE
    NF = F // LANE
    NP = S // PAIR
    NSEG = S // SEG
    NJ = H // 2
    NPRE = NSEG * 8
    L = SEG + MEM
    scale = float(LANE) ** -0.5
    w_hbm = (wq_hbm, wk_hbm, wv_hbm)
    w_v = (wq_v, wk_v, wv_v)

    def blk(j):
        return slice(j * LANE, (j + 1) * LANE)

    NCH = 4
    CK = KD // NCH

    def early_mod(ch):
        return [pltpu.make_async_copy(
            wmod_hbm.bitcast(U32).at[:, pl.ds(
                pl.multiple_of(t * D + ch * (CK * LANE), LANE), CK * LANE)],
            wme_v.at[ch, t], sem_mod.at[ch]) for t in range(2)]

    late_mod = [pltpu.make_async_copy(
        wmod_hbm.bitcast(U32).at[:, pl.ds((2 + 2 * t) * D, 2 * D)],
        wml_v.at[t], sem_mod.at[NCH]) for t in range(2)]

    def unit_copy(j, w):
        return pltpu.make_async_copy(
            w_hbm[w].bitcast(U32).at[:, :, j, 0, :],
            w_v[w].at[j], sem_qkv.at[3 * j + w])

    def start_unit(j, w):
        unit_copy(j, w).start()

    def wait_unit(j, w):
        unit_copy(j, w).wait()

    first_units = [(u // 3, u % 3) for u in range(NU_FIRST)]

    def slice_copies(ch):
        rows = pl.ds(ch * (CK * 8), CK * 8)
        return [pltpu.make_async_copy(
            w_hbm[w].bitcast(U32).at[rows, :, j, 0, :], w_v[w].at[j, rows],
            sem_mod.at[ch]) for j, w in first_units]

    wo_copy = pltpu.make_async_copy(
        wo_hbm.bitcast(U32), wo_v.at[:, pl.ds(0, D)], sem_w.at[0])
    FH = F // 2
    NH = NF // 2
    ffn_copies = []
    for hf in range(2):
        for src, dst in ((w1_hbm, w1_v), (w3_hbm, w3_v)):
            ffn_copies.append(pltpu.make_async_copy(
                src.bitcast(U32).at[:, pl.ds(hf * FH, FH)],
                dst.at[hf, :, pl.ds(0, FH)], sem_w.at[1]))
    for hf in range(2):
        ffn_copies.append(pltpu.make_async_copy(
            w2_hbm.bitcast(U32).at[pl.ds(hf * FH // 2, FH // 2), :],
            w2_v.at[hf, :, pl.ds(0, D)], sem_w.at[1]))
    c_copy = pltpu.make_async_copy(c_hbm, c_v, sem_x.at[2])
    mem0_copy = pltpu.make_async_copy(mem0_hbm, mem0_v, sem_x.at[3])
    x_copy = pltpu.make_async_copy(x_hbm, x_v, sem_x.at[1])
    x0_copy = pltpu.make_async_copy(x_hbm.at[0], x0_v, sem_x.at[0])
    NXP = 4
    XS = NSEG // NXP

    def xpre_copy(b):
        return pltpu.make_async_copy(
            x_hbm.at[pl.ds(b * XS, XS), pl.ds(0, 8), :],
            xpre_v.at[pl.ds(b * XS, XS)], sem_xp.at[b])

    def out_copy(i, slot):
        return pltpu.make_async_copy(
            stage_v.at[slot], out_hbm.at[pl.ds(i * PAIR, PAIR), :],
            sem_out.at[slot])

    def start_units(j0, j1):
        def step(j, carry):
            for w in range(3):
                start_unit(j, w)
            return carry

        lax.fori_loop(j0, j1, step, 0)

    j1 = NU_FIRST // 3
    for b in range(NXP):
        xpre_copy(b).start()
    c_copy.start()

    def start_chunk(ch, carry):
        for cp in early_mod(ch) + slice_copies(ch):
            cp.start()
        return carry

    lax.fori_loop(0, NCH, start_chunk, 0)
    mem0_copy.start()
    x0_copy.start()
    start_unit(j1, 1)
    start_unit(j1, 2)
    start_units(j1 + 1, j1 + 7)
    x1_v[1] = jnp.zeros((PAIR, D), F32)
    mod_v[3 * KD:5 * KD] = jnp.zeros((2 * KD, 8, LANE), F32)

    def ln_pre(b, carry):
        @pl.when(b % (XS // 8) == 0)
        def _():
            xpre_copy(b // (XS // 8)).wait()

        x = xpre_v[pl.ds(b * 8, 8)].astype(F32).reshape(64, D)
        xn = _layernorm(x)
        r0 = pl.multiple_of(b * 64, 64)
        for k in range(KD):
            xn_v[k, pl.ds(r0, 64), :] = xn[:, blk(k)]
        return carry

    lax.fori_loop(0, NSEG // 8, ln_pre, 0)

    def relayout_rows(j, w, r, do=None):
        rows = pl.ds(r, 8)
        a = w_v[w][j, rows, pl.ds(0, 8, stride=2), :]
        b = w_v[w][j, rows, pl.ds(1, 8, stride=2), :]
        lo = (a & U32(0xFFFF)) | (b << 16)
        hi = (a >> 16) | (b & U32(0xFFFF0000))
        if do is not None:
            lo = jnp.where(do, lo, w_v[w][j, rows, 0:8, :])
            hi = jnp.where(do, hi, w_v[w][j, rows, 8:16, :])
        w_v[w][j, rows, 0:8, :] = lo
        w_v[w][j, rows, 8:16, :] = hi

    def relayout(j, w, do=None):
        for k in range(KD):
            relayout_rows(j, w, k * 8, do)

    def w_head(w, j, p, k0=0, nk=KD):
        t = w_v[w][j, pl.ds(k0 * 8, nk * 8), 8 * p:8 * p + 8, :]
        return _unpk(t.reshape(nk * LANE // 2, LANE))

    c_copy.wait()
    start_units(j1 + 7, NJ)

    c = c_v[...].astype(F32)
    sc = _silu(c).astype(BF16)
    sc = jnp.broadcast_to(sc, (16, D))

    def mod_row(k):
        return jnp.concatenate([mod_blk(k, j) for j in range(KD)], axis=1)

    def mod_blk(k, j):
        return mod_v[k * KD + j, 0:1, :]

    def chunk_body(ch, carry):
        for cp in early_mod(ch) + slice_copies(ch):
            cp.wait()
        k0 = ch * CK
        for kk in range(CK):
            sa = _dot(sc, _unpk(wme_v[ch, 0, :, blk(kk)]))[0:8]
            ca = _dot(sc, _unpk(wme_v[ch, 1, :, blk(kk)]))[0:8] + 1.0
            mod_v[k0 + kk] = sa
            mod_v[KD + k0 + kk] = ca
            for r in range(0, NSEG * 8, 128):
                hpre_v[k0 + kk, r // 2:r // 2 + 64, :] = _pk(
                    xn_v[k0 + kk, r:r + 128, :] * ca[0:1] + sa[0:1])
        for u, (j, w) in enumerate(first_units):
            for kk in range(CK):
                relayout_rows(j, w, (k0 + kk) * 8)
            hp = _cat_pk(hpre_v, [k0 + kk for kk in range(CK)], NPRE)
            wt = jnp.concatenate(
                [w_head(w, j, p, k0, CK) for p in range(2)], axis=1)
            acc = jnp.where(ch > 0, acc0_v[u], 0.0) + _dot(hp, wt)
            acc0_v[u] = acc
            for p in range(2):
                pre_v[w, j, p] = _pk(acc[:, blk(p)])
        return carry

    lax.fori_loop(0, NCH, chunk_body, 0)

    def ln1(x, sg):
        h = _layernorm(x.astype(F32)[8:SEG]) * mod_row(1) + mod_row(0)
        for k in range(KD):
            lhs_v[sg, k, 0:8, :] = _pk(h[0:16, blk(k)])
            hs_v[sg, k] = h[16:24, blk(k)]

    def ln1_seg(seg, sg):
        ln1(x_v[seg], sg)

    def first_lhs():
        ln1(x0_v[...], 0)
        mem0 = mem0_v[...].astype(F32)
        for k in range(KD):
            lhs_v[0, k, 8:16, :] = _pk(jnp.concatenate(
                [hs_v[0, k], mem0[:, blk(k)]], axis=0))

    def pre_dot(j, w, p):
        hp = _cat_pk(hpre_v, range(KD), NPRE)
        pre_v[w, j, p] = _pk(_dot(hp, w_head(w, j, p)))

    wait_unit(j1, 1)
    mem0_copy.wait()
    x0_copy.wait()
    wo_copy.start()
    x_copy.start()
    for cp in late_mod + ffn_copies:
        cp.start()
    relayout(j1, 1)

    def pre_body(j, carry):
        wait_unit(j, 2)
        wait_unit(j + 1, 0)
        wait_unit(j + 1, 1)

        for (dj, dw), (rj, rw) in (((j, 1), (j, 2)), ((j, 2), (j + 1, 0)),
                                   ((j + 1, 0), (j + 1, 1))):
            pre_dot(dj, dw, 0)
            relayout(rj, rw)
            pre_dot(dj, dw, 1)
        first_lhs()
        return carry

    lax.fori_loop(j1, NJ - 1, pre_body, 0)

    L2 = 2 * L
    rr = lax.broadcasted_iota(jnp.int32, (L2, L2), 0)
    cc = lax.broadcasted_iota(jnp.int32, (L2, L2), 1)
    same = (rr >= L) == (cc >= L)
    rr = jnp.where(rr >= L, rr - L, rr)
    cc = jnp.where(cc >= L, cc - L, cc)
    mask = same & ((rr >= SEG) | (cc >= SEG) | (cc <= rr))
    fill_val = jnp.where(same, -1000000000.0, -jnp.inf).astype(F32)

    def scores(q, k):
        s = lax.dot_general(q, k, (((1,), (1,)), ((), ())),
                            preferred_element_type=F32)
        s = jnp.where(mask, s * scale, fill_val)
        m = jnp.max(s, axis=-1, keepdims=True)
        e = jnp.exp(s - m)
        p = e * _recip(jnp.sum(e, axis=-1, keepdims=True))
        return p.astype(BF16)

    def ln2(xs, hs=0):
        h = _layernorm(x1_v[xs]) * mod_row(4) + mod_row(3)
        for k in range(KD):
            h2_v[hs, k, 0:PAIR // 2, :] = _pk(h[:, blk(k)])

    def up_half(hf, f, hs, dst):
        h2 = _cat_pk(h2_v.at[hs], range(KD), PAIR)
        g = _dot(h2, _unpk(w1_v[hf, :, blk(f)]))
        u = _dot(h2, _unpk(w3_v[hf, :, blk(f)]))
        act_v[dst, 0:PAIR // 2, :] = _pk(_silu(g) * u)

    def up(f):
        up_half(f // NH, f % NH, 0, f)

    def down(xs, j, hf):
        a = _cat_pk(act_v, range(hf * NH, (hf + 1) * NH), PAIR)
        y = _dot(a, _unpk(w2_v[hf, :, blk(j)]))
        if hf == 0:
            yh_v[:, blk(j)] = y
        else:
            y = y + yh_v[:, blk(j)]
            stage_v[xs, :, blk(j)] = (
                x1_v[xs, :, blk(j)] + mod_blk(5, j) * y).astype(BF16)

    def segment(i, sg, fill, finish, wo_plan):
        tail, wo_cuts = wo_plan
        o_v = ob_v if sg else oa_v
        rows = L + 8 if sg else SEG
        prow = pl.multiple_of(i * 8, 8)
        qk, vs, ps = {}, {}, {}

        def proj(g):
            r = []
            for w in range(3):
                parts = []
                for p in range(2):
                    lhs = _cat_pk(lhs_v.at[sg], range(KD), SEG)
                    if sg == 0:
                        pre = pre_v[w, g, p, pl.ds(prow, 8), :]
                        cur_v[w, g, p] = pre
                    else:
                        pre = cur_v[w, g, p]
                    pre = _unpk(pre).astype(F32)
                    parts += [pre[8 * sg:8 * sg + 8],
                              _dot(lhs, w_head(w, g, p))]
                r.append(jnp.concatenate(parts, axis=0).astype(BF16))
            qk[g] = r[0:2]
            vs[g] = r[2]

        def pv(g):
            o2 = _dot(ps.pop(g), vs.pop(g))
            for p in range(2):
                h = 2 * g + p
                o = o2[p * L:(p + 1) * L]
                if sg == 0:
                    o_v[h, 0:16, :] = _pk(
                        jnp.concatenate([o[0:24], o[SEG:L]], axis=0))
                    so_v[h] = o[24:SEG]
                else:
                    o_v[h] = _pk(jnp.concatenate([so_v[h], o], axis=0))

        def wo_part(hs, j):
            lo, hi = hs[0] * (LANE // 2), (hs[-1] + 1) * (LANE // 2)
            return _dot(_cat_pk(o_v, hs, rows), _unpk(wo_v[lo:hi, blk(j)]))

        def wo_head(j):
            between = fill.get(("head", j))
            if between is None:
                acc_v[j, 0:rows, :] = wo_part(head_hs, j)
                return
            half = len(head_hs) // 2
            acc_v[j, 0:rows, :] = wo_part(head_hs[:half], j)
            between[0]()
            acc_v[j, 0:rows, :] += wo_part(head_hs[half:], j)
            for fn in between[1:]:
                fn()

        head_hs = list(range(H - tail))
        tail_hs = list(range(H - tail, H))
        cuts = (0,) + wo_cuts
        wo_at = {NJ + t: range(cuts[t], cuts[t + 1]) for t in range(LP)}
        for g in range(NJ + LP):
            if g < NJ:
                proj(g)
            for j in wo_at.get(g, ()):
                wo_head(j)
            if LS <= g < NJ + LS:
                ps[g - LS] = scores(*qk.pop(g - LS))
            if g >= LP:
                pv(g - LP)
            for fn in fill.get(g, ()):
                fn()
        for j in range(wo_cuts[-1], KD):
            wo_head(j)
        for j in range(KD):
            finish(j, acc_v[j, 0:rows, :] + wo_part(tail_hs, j))
        for fn in fill.get(NJ + LP, ()):
            fn()

    def attn_pair(i, fill_a, fill_b, wo_plan):
        xs = i % 2

        def finish_a(j, y):
            ya_v[j] = y[0:24]
            lhs_v[1, j, 8:16, :] = _pk(
                jnp.concatenate([hs_v[1, j], y[24:SEG]], axis=0))

        def finish_b(j, y):
            att = jnp.concatenate([ya_v[j], y[0:L]], axis=0)
            x = x_v[pl.ds(2 * i, 2), :, blk(j)].astype(F32).reshape(PAIR, LANE)
            x1_v[xs, :, blk(j)] = x + mod_blk(2, j) * att
            lhs_v[0, j, 8:16, :] = _pk(
                jnp.concatenate([hs_v[0, j], y[L:L + 8]], axis=0))

        segment(i, 0, fill_a, finish_a, wo_plan)
        segment(i, 1, fill_b, finish_b, wo_plan)

    P = functools.partial

    wait_unit(NJ - 1, 2)
    x_copy.wait()
    for cp in late_mod:
        cp.wait()
    wo_copy.wait()

    def head_body(i, carry):
        def piece(n):
            m, w, p = n // 4, 1 + n % 4 // 2, n % 2
            r0 = pl.multiple_of(i * (NPRE // 4) + m * 32, 32)
            hp = jnp.concatenate(
                [_unpk(hpre_v[k, pl.ds(r0, 32), :]) for k in range(KD)], axis=1)
            pre_v[w, NJ - 1, p, pl.ds(r0, 32), :] = _pk(
                _dot(hp, w_head(w, NJ - 1, p)))

        def late_mod_col(n):
            r = _dot(sc, _unpk(wml_v[i, :, blk(n)]))[0:8]
            if n < KD:
                r = r + i.astype(F32)
            mod_v[2 * KD * (1 + i) + n] = r

        fill_a = {0: [P(relayout, NJ - 1, 2, i == 0)],
                  2: [P(ln1_seg, 2 * i + 1, 1)]}
        fill_b = {8: [P(ln1_seg, 2 * i + 2, 0)]}
        for j in range(KD):
            fill_b[("head", j)] = [P(late_mod_col, 2 * j + t) for t in range(2)]
        fill_b[("head", KD // 2)].append(P(ln2, 1 - i))
        for n, g in enumerate(HEAD_A):
            fill_a.setdefault(g, []).append(P(piece, n))
        for n, g in enumerate(HEAD_B):
            fill_b.setdefault(g, []).append(P(piece, len(HEAD_A) + n))
        attn_pair(i, fill_a, fill_b, WO_HEAD)
        return carry

    lax.fori_loop(0, 2, head_body, 0)
    for cp in ffn_copies:
        cp.wait()
    for f in range(NU0):
        up(f)

    def body(i, carry):
        slot = i % 2

        @pl.when(i >= 4)
        def _():
            out_copy(i - 4, slot).wait()

        fill_a, fill_b = {}, {}
        for f in range(NU0, NF):
            fill_a.setdefault((f - NU0) * NJ // (NF - NU0), []).append(P(up, f))
        downs = [P(down, slot, j, hf) for j in range(KD) for hf in range(2)]
        fill_a[NJ + LP] = downs[0:1]
        for n, fn in enumerate(downs[1:]):
            fill_b.setdefault(n, []).append(fn)
        fill_b.setdefault(2, []).append(P(ln2, 1 - slot))
        fill_a.setdefault(2, []).append(P(ln1_seg, 2 * i + 1, 1))
        fill_b.setdefault(8, []).append(
            P(ln1_seg, jnp.minimum(2 * i + 2, NSEG - 1), 0))
        fill_b[NJ + LP] = [P(up, f) for f in range(NU0)]
        attn_pair(i, fill_a, fill_b, WO_MAIN)
        out_copy(i - 2, slot).start()
        return carry

    lax.fori_loop(2, NP, body, 0)

    out_copy(NP - 4, NP % 2).wait()

    def tail_body(q, carry):
        t, hf = q // 2, q % 2
        xs = (NP + t) % 2

        @pl.when(q == 2)
        def _():
            out_copy(NP - 3, xs).wait()

        for f in range(NH):
            up_half(hf, f, t, f)
        ln2((NP + 1) % 2, 1)
        for j in range(KD):
            y = _dot(_cat_pk(act_v, range(NH), PAIR),
                     _unpk(w2_v[hf, :, blk(j)]))
            y = y + jnp.where(hf == 1, yh_v[:, blk(j)], 0.0)
            yh_v[:, blk(j)] = y
            stage_v[xs, :, blk(j)] = (
                x1_v[xs, :, blk(j)] + mod_blk(5, j) * y).astype(BF16)

        @pl.when(hf == 1)
        def _():
            out_copy(NP - 2 + t, xs).start()

        return carry

    lax.fori_loop(0, 4, tail_body, 0)
    out_copy(NP - 2, NP % 2).wait()
    out_copy(NP - 1, (NP + 1) % 2).wait()


@functools.partial(jax.jit, static_argnames=("A_seg_len",))
def pallas_adaLN_cond__memory_aug_recurrent_mem_tr__glu_gated_swiglu__prompt_kernel(
    A_x: jax.Array,
    A_mem0: jax.Array,
    A_Wq: jax.Array,
    A_Wk: jax.Array,
    A_Wv: jax.Array,
    A_Wo: jax.Array,
    A_seg_len,
    B_x: jax.Array,
    B_w1: jax.Array,
    B_w3: jax.Array,
    B_w2: jax.Array,
    c: jax.Array,
    w_mod: jax.Array,
):
    B, S, D = A_x.shape
    H, Dh = A_Wq.shape[1], A_Wq.shape[2]
    F = B_w1.shape[1]
    assert B == 1 and Dh == LANE and A_seg_len == SEG and A_mem0.shape[1] == MEM
    assert (S, D, H) == (2048, 1024, 32) and F % (2 * LANE) == 0
    KD, NF = D // LANE, F // LANE
    NSEG = S // SEG

    def split(w):
        return w.reshape(D // 16, 16, H // 2, 2, Dh)

    any_spec = pl.BlockSpec(memory_space=pl.ANY)
    out = pl.pallas_call(
        functools.partial(_kernel, S=S, D=D, H=H, F=F),
        out_shape=jax.ShapeDtypeStruct((S, D), A_x.dtype),
        in_specs=[any_spec] * 11,
        out_specs=any_spec,
        scratch_shapes=[
            pltpu.VMEM((1, D), BF16),
            pltpu.VMEM((MEM, D), BF16),
            pltpu.VMEM((SEG, D), BF16),
            pltpu.VMEM((NSEG, SEG, D), BF16),
            pltpu.VMEM((NSEG, 8, D), BF16),
            pltpu.VMEM((KD, NSEG * 8, LANE), F32),
            pltpu.VMEM((KD, NSEG * 4 + 8, LANE), U32),
            pltpu.VMEM((NU_FIRST, NSEG * 8, 2 * LANE), F32),
            pltpu.VMEM((3, H // 2, 2, NSEG * 4, LANE), U32),
            pltpu.VMEM((3, H // 2, 2, 8, LANE), U32),
            pltpu.VMEM((H // 2, D // 16, 16, LANE), U32),
            pltpu.VMEM((H // 2, D // 16, 16, LANE), U32),
            pltpu.VMEM((H // 2, D // 16, 16, LANE), U32),
            pltpu.VMEM((H * Dh // 2, D + LANE), U32),
            pltpu.VMEM((2, D // 2, F // 2 + LANE), U32),
            pltpu.VMEM((2, D // 2, F // 2 + LANE), U32),
            pltpu.VMEM((2, F // 4, D + LANE), U32),
            pltpu.VMEM((4, 2, D // 2, D // 4), U32),
            pltpu.VMEM((2, D // 2, 2 * D), U32),
            pltpu.VMEM((6 * KD, 8, LANE), F32),
            pltpu.VMEM((2, KD, 8, LANE), F32),
            pltpu.VMEM((2, KD, 24, LANE), U32),
            pltpu.VMEM((H, 8, LANE), F32),
            pltpu.VMEM((H, 24, LANE), U32),
            pltpu.VMEM((H, 24, LANE), U32),
            pltpu.VMEM((KD, 48, LANE), F32),
            pltpu.VMEM((KD, 24, LANE), F32),
            pltpu.VMEM((2, PAIR, D), F32),
            pltpu.VMEM((2, KD, PAIR // 2 + 8, LANE), U32),
            pltpu.VMEM((NF, PAIR // 2 + 8, LANE), U32),
            pltpu.VMEM((PAIR, D), F32),
            pltpu.VMEM((2, PAIR, D), BF16),
            pltpu.SemaphoreType.DMA((4,)),
            pltpu.SemaphoreType.DMA((4,)),
            pltpu.SemaphoreType.DMA((5,)),
            pltpu.SemaphoreType.DMA((3 * H // 2,)),
            pltpu.SemaphoreType.DMA((2,)),
            pltpu.SemaphoreType.DMA((2,)),
        ],
        compiler_params=pltpu.CompilerParams(
            vmem_limit_bytes=110 * 1024 * 1024,
            disable_bounds_checks=True,
            disable_semaphore_checks=True),
        name="rmt_block",
    )(A_x.reshape(NSEG, SEG, D), A_mem0.reshape(MEM, D), split(A_Wq),
      split(A_Wk), split(A_Wv), A_Wo.reshape(H * Dh, D), B_w1, B_w3, B_w2, c,
      w_mod)
    return out.reshape(B, S, D)
```
